```python
import jax
import jax.numpy as jnp

def _softmax(x, axis=-1):
    return jax.nn.softmax(x, axis=axis)
def _gelu(x):
    return jax.nn.gelu(x, approximate=True)
def _silu(x):
    return jax.nn.silu(x)
def _sigmoid(x):
    return jax.nn.sigmoid(x)
def _layernorm(x, axis=-1, eps=1e-5):
    m = jnp.mean(x, axis=axis, keepdims=True)
    v = jnp.var(x, axis=axis, keepdims=True)
    return (x - m) / jnp.sqrt(v + eps)
def _scatter_add(tgt, idx, src, axis=0):
    return tgt.at[idx].add(src)
def _segment_sum(src, seg, n):
    return jax.ops.segment_sum(src, seg, n)
class _Rng:
    def __init__(self, key):
        self._k = key
    def _next(self):
        self._k, sub = jax.random.split(self._k)
        return sub
    def normal(self, shape):
        return jax.random.normal(self._next(), shape, dtype=jnp.bfloat16)
    def randint(self, lo, hi, shape):
        return jax.random.randint(self._next(), shape, lo, hi, dtype=jnp.int32)
    def uniform(self, shape, lo=0.0, hi=1.0):
        return jax.random.uniform(self._next(), shape, jnp.bfloat16, lo, hi)
    def permutation(self, n):
        return jax.random.permutation(self._next(), n)


kernel_name = 'parallel_sum__linear_attn_block__moe_arch_mod__prompt'

def setup_inputs():
    _rng = _Rng(jax.random.key(int.from_bytes(__import__("os").urandom(4), "little")))
    _w = (lambda a: (lambda t: t.astype(jnp.bfloat16) if jnp.issubdtype(t.dtype, jnp.floating) else t)(jnp.asarray(a)))
    def _A_setup():
        B, S, D = 1, 2048, 1024
        return {
            "x": _w((lambda *s: _rng.normal(s) * 0.05)(B, S, D)),
            "wqkv": _w((lambda *s: _rng.normal(s) * 0.05)(D, 3 * D)),
            "wo": _w((lambda *s: _rng.normal(s) * 0.05)(D, D)),
        }
    _A_in = _A_setup()

    def _B_setup():
        B, S, D, F, C = 1, 2048, 1024, 3584, 1
        return {
            "x": _w((lambda *s: _rng.normal(s) * 0.05)(B, S, D)),
            "w_r": _w((lambda *s: _rng.normal(s) * 0.05)(D)),
            "w_gate": _w((lambda *s: _rng.normal(s) * 0.05)(D, F)),
            "w_up": _w((lambda *s: _rng.normal(s) * 0.05)(D, F)),
            "w_down": _w((lambda *s: _rng.normal(s) * 0.05)(F, D)),
        }
    _B_in = _B_setup()

    return {
        "A_x": _A_in["x"],
        "A_wqkv": _A_in["wqkv"],
        "A_wo": _A_in["wo"],
        "B_x": _B_in["x"],
        "B_w_r": _B_in["w_r"],
        "B_w_gate": _B_in["w_gate"],
        "B_w_up": _B_in["w_up"],
        "B_w_down": _B_in["w_down"],
    }

def reference(A_x, A_wqkv, A_wo, B_x, B_w_r, B_w_gate, B_w_up, B_w_down):
    def _A_ref(x, wqkv, wo):
        B, S, D = x.shape
        H = 32; Dh = D // H
        qkv = (lambda x, *d: x.transpose(*d))((x @ wqkv).reshape(B, S, 3, H, Dh), 2, 0, 3, 1, 4)
        q, k, v = qkv[0], qkv[1], qkv[2]
        phi = lambda t: jnp.where(t > 0, t + 1, jnp.exp(t)) + 1e-6
        pq, pk = phi(q), phi(k)
        kv = jnp.einsum("bhsd,bhse->bhde", pk, v)
        z = jnp.einsum("bhsd->bhd", pk)
        num = jnp.einsum("bhqd,bhde->bhqe", pq, kv)
        den = jnp.einsum("bhqd,bhd->bhq", pq, z)[..., None] + 1e-6
        o = num / den
        return (lambda x, *d: x.transpose(*d))(o, 0, 2, 1, 3).reshape(B, S, D) @ wo

    def _B_ref(x, w_r, w_gate, w_up, w_down):
        B, S, D = x.shape
        C = 1
        r = x @ w_r
        idx = jnp.argsort(-r, axis=-1)[:, :C]
        idx_e = jnp.repeat(idx.reshape(B, C, 1), D, axis=2)
        x_sel = jnp.take_along_axis(x, idx_e, axis=1)
        g = _silu(x_sel @ w_gate)
        u = x_sel @ w_up
        y = (g * u) @ w_down
        r_sel = _sigmoid(jnp.take_along_axis(r, idx, axis=1))
        y = y * r_sel.reshape(B, C, 1)
        b_off = (jnp.arange(B) * S).reshape(B, 1)
        flat_idx = (idx + b_off).reshape(B * C)
        zero = (x * 0.0).reshape(B * S, D)
        upd = _scatter_add(zero, flat_idx, y.reshape(B * C, D), axis=0)
        return x + upd.reshape(B, S, D)

    x = A_x
    xn = _layernorm(x, axis=-1)
    return x + _A_ref(xn, A_wqkv, A_wo) + _B_ref(xn, B_w_r, B_w_gate, B_w_up, B_w_down)
```

```python
import functools

import jax
import jax.numpy as jnp
import jax.experimental.pallas as pl
import jax.experimental.pallas.tpu as pltpu

_H = 32
_LN_EPS = 1e-5
_PHI_EPS = 1e-6
_DEN_EPS = 1e-6
_SUB = 256
_CB = 256
_LNR = 32
_G = 128
_PAD = 128

_F32 = jnp.float32
_BF16 = jnp.bfloat16
_U32 = jnp.uint32


def _dot(a, b):
    return jnp.dot(a, b, preferred_element_type=_F32)


def _dot_tn(a, b):
    return jax.lax.dot_general(a, b, (((0,), (0,)), ((), ())), preferred_element_type=_F32)


def _dot_nt(a, b):
    return jax.lax.dot_general(a, b, (((1,), (1,)), ((), ())), preferred_element_type=_F32)


def _phi(t):
    return jnp.where(t > 0, t + 1.0, jnp.exp(t)) + _PHI_EPS


def _pack(v):
    return pltpu.bitcast(v, _U32)


def _unpack(v):
    return pltpu.bitcast(v, _BF16)


def _col_bcast(row):
    return jnp.broadcast_to(row, (_G, _G)).T


def _kernel(x_hbm, wqkv_hbm, wo_hbm, wr_ref, wg_hbm, wu_hbm, wd_hbm, out_hbm,
            x_v, wq_v, wk_v, wv_v, wo_v, wg_v, wu_v, wd_v,
            xn_v, wqt_v, g_v, zcol_v, xcol_v, m_v, out_v,
            sem_x, sem_k, sem_w, sem_o, sem_l, sem_b, *, S, D, F):
    n_sub = S // _SUB
    n_cb = D // _CB
    n_groups = D // _G
    dh = D // _H

    cols = lambda c: pl.ds(c * _CB, _CB)
    dcols = pl.ds(0, D)

    x_parts = [(0, 1), (1, 2), (2, 4), (4, n_sub)]
    x_cp = [pltpu.make_async_copy(x_hbm.at[pl.ds(a * _SUB, (b - a) * _SUB), :],
                                  x_v.at[pl.ds(a * _SUB, (b - a) * _SUB), :], sem_x.at[j])
            for j, (a, b) in enumerate(x_parts)]
    k_parts = [(0, 1), (1, 2), (2, n_cb)]
    k_cp = [pltpu.make_async_copy(wqkv_hbm.at[:, pl.ds(D + a * _CB, (b - a) * _CB)],
                                  wk_v.at[:, pl.ds(a * _CB, (b - a) * _CB)], sem_k.at[j])
            for j, (a, b) in enumerate(k_parts)]
    w_cp = dict(
        q=pltpu.make_async_copy(wqkv_hbm.at[:, pl.ds(0, D)], wq_v.at[:, dcols], sem_w.at[0]),
        v=pltpu.make_async_copy(wqkv_hbm.at[:, pl.ds(2 * D, D)], wv_v.at[:, dcols], sem_w.at[1]),
        o=pltpu.make_async_copy(wo_hbm, wo_v.at[:, dcols], sem_w.at[2]),
        g=pltpu.make_async_copy(wg_hbm, wg_v, sem_w.at[3]),
        u=pltpu.make_async_copy(wu_hbm, wu_v, sem_w.at[4]),
        d=pltpu.make_async_copy(wd_hbm, wd_v.at[:, dcols], sem_w.at[5]),
    )

    def fence():
        pl.semaphore_signal(sem_b, 1)
        pl.semaphore_wait(sem_b, 1)

    for cp in (x_cp[0], k_cp[0], k_cp[1], k_cp[2], x_cp[1], x_cp[2], w_cp["q"], x_cp[3],
               w_cp["v"], w_cp["o"], w_cp["g"], w_cp["u"], w_cp["d"]):
        cp.start()
        fence()

    st = {}
    st["best"] = jnp.full((8, 1), -jnp.inf, _F32)
    st["besti"] = jnp.zeros((8, 1), jnp.int32)
    st["z"] = [None] * n_cb
    pk = {}
    wr = wr_ref[...].astype(_F32)
    wr_sum = jnp.sum(wr, axis=-1, keepdims=True)
    sub_iota = jax.lax.broadcasted_iota(jnp.int32, (8, 1), 0)

    def ln_chunk(s, j):
        r0 = s * _SUB + j * _LNR
        x = x_v[pl.ds(r0, _LNR), :].astype(_F32)
        m = jnp.sum(x, axis=-1, keepdims=True) * (1.0 / D)
        ex2 = jnp.sum(x * x, axis=-1, keepdims=True) * (1.0 / D)
        xw = jnp.sum(x * wr, axis=-1, keepdims=True)
        v = jnp.maximum(ex2 - m * m, 0.0)
        rstd = jax.lax.rsqrt(v + _LN_EPS)
        r = (xw - m * wr_sum) * rstd
        r = r.astype(_BF16).astype(_F32)
        rstd = jnp.where(r != r, r, rstd)
        for t in range(_LNR // 8):
            rt = r[t * 8:(t + 1) * 8, :]
            upd = rt > st["best"]
            st["best"] = jnp.where(upd, rt, st["best"])
            st["besti"] = jnp.where(upd, sub_iota + (r0 + t * 8), st["besti"])
        for c in range(n_cb):
            xc = x_v[pl.ds(r0, _LNR), cols(c)].astype(_F32)
            xn_v[pl.ds(r0 // 2, _LNR // 2), cols(c)] = _pack(((xc - m) * rstd).astype(_BF16))

    def xn_rows(r0, n):
        return _unpack(xn_v[pl.ds(r0 // 2, n // 2), :])

    def k_job(s, c):
        p = _phi(_dot(xn_rows(s * _SUB, _SUB), wk_v[:, cols(c)]))
        zs = jnp.sum(p.reshape(_SUB // 8, 8, _CB), axis=0)
        st["z"][c] = zs if st["z"][c] is None else st["z"][c] + zs
        pk[s, c] = p.astype(_BF16)

    def g_job(s, c):
        upd = _dot_tn(pk.pop((s, c)), xn_rows(s * _SUB, _SUB))
        if s == 0:
            g_v[cols(c), :] = upd
        else:
            g_v[cols(c), :] += upd

    def wqt_job(a, b):
        wqt_v[pl.ds(b * _CB // 2, _CB // 2), cols(a)] = _pack(wq_v[cols(a), cols(b)].T)

    n_ln = _SUB // _LNR
    lpc = n_ln // n_cb
    x_cp[0].wait()
    for j in range(n_ln):
        ln_chunk(0, j)
    k_cp[0].wait()
    k_job(0, 0)
    k_cp[1].wait()
    k_job(0, 1)
    g_job(0, 0)
    g_job(0, 1)
    k_cp[2].wait()
    x_cp[1].wait()
    k_job(0, 2)
    for j in range(n_ln // 2):
        ln_chunk(1, j)
    k_job(0, 3)
    for j in range(n_ln // 2, n_ln):
        ln_chunk(1, j)
    g_job(0, 2)
    pending = [(0, 3)]
    wqt_q = [(a, b) for a in range(n_cb) for b in range(n_cb)]
    for s in range(1, n_sub):
        for c in range(n_cb):
            late = s in (1, 3)
            if late and c == 2:
                if s == 1:
                    x_cp[2].wait()
                    w_cp["q"].wait()
                else:
                    x_cp[3].wait()
                    w_cp["v"].wait()
                    w_cp["o"].wait()
            k_job(s, c)
            if s + 1 < n_sub and (not late or c >= 2):
                if late:
                    js = range(2 * lpc * (c - 2), 2 * lpc * (c - 1))
                else:
                    js = range(lpc * c, lpc * (c + 1))
                for j in js:
                    ln_chunk(s + 1, j)
            if (s, c) >= (1, 2):
                for _ in range(2):
                    if wqt_q:
                        wqt_job(*wqt_q.pop(0))
            g_job(*pending.pop(0))
            pending.append((s, c))

    rmax = jnp.max(st["best"], axis=0, keepdims=True)
    idx = jnp.min(jnp.where(st["best"] == rmax, st["besti"], S - 1))
    idx16 = pl.multiple_of((idx // 16) * 16, 16)
    idx_tile = idx // _SUB
    row0 = [pl.multiple_of(((idx_tile + 1 + t) % n_sub) * _SUB, _SUB) for t in range(n_sub)]
    half0 = [pl.multiple_of(((idx_tile + 1 + t) % n_sub) * (_SUB // 2), _SUB // 2) for t in range(n_sub)]
    rows = lambda t: pl.ds(row0[t], _SUB)
    hrows = lambda t: pl.ds(half0[t], _SUB // 2)
    o_cp = [pltpu.make_async_copy(out_v.at[rows(t), :], out_hbm.at[rows(t), :], sem_o.at[t])
            for t in range(n_sub - 1)]
    l_cp = [pltpu.make_async_copy(out_v.at[rows(n_sub - 1), cols(c)], out_hbm.at[rows(n_sub - 1), cols(c)],
                                  sem_l.at[c]) for c in range(n_cb)]

    rr = jax.lax.broadcasted_iota(jnp.int32, (_G, _G), 0) // dh
    cc = jax.lax.broadcasted_iota(jnp.int32, (_G, _G), 1) // dh
    same_head = rr == cc

    ob = {}
    kvb = {}
    ffn_q = []

    def ffn_step():
        if ffn_q:
            ffn_q.pop(0)()

    def q_job(t, c):
        xn = _unpack(xn_v[hrows(t), :])
        p = _phi(_dot_nt(_unpack(wqt_v[pl.ds(c * _CB // 2, _CB // 2), :]), xn))
        zc = zcol_v[cols(c), :]
        zc = jnp.concatenate([zc] * (_SUB // _G), axis=1)
        p3 = p.reshape(_CB // dh, dh, _SUB)
        den = jnp.sum(p3 * zc.reshape(_CB // dh, dh, _SUB), axis=1, keepdims=True) + _DEN_EPS
        o = (p3 * pl.reciprocal(den, approx=True)).reshape(_CB, _SUB).astype(_BF16)
        ob[t, c] = o.T
        ffn_step()

    def z_job(g):
        c, j = divmod(g, _CB // _G)
        z = jnp.sum(st["z"][c][:, j * _G:(j + 1) * _G], axis=0, keepdims=True)
        zcol_v[pl.ds(g * _G, _G), :] = _col_bcast(z)

    def kv_job(g):
        gs = pl.ds(g * _G, _G)
        kv = _dot(g_v[gs, :].astype(_BF16), wv_v[:, gs])
        kvb[g] = jnp.where(same_head, kv, 0.0).astype(_BF16)

    def m_job(g):
        m_v[pl.ds(g * _G // 2, _G // 2), :] = _pack(_dot(kvb.pop(g), wo_v[pl.ds(g * _G, _G), dcols]).astype(_BF16))

    def out_job(t, c):
        if c == 0:
            ob[t] = jnp.concatenate([ob.pop((t, cb)) for cb in range(n_cb)], axis=1)
        a = _dot(ob[t], _unpack(m_v[:, cols(c)]))
        res = x_v[rows(t), cols(c)].astype(_F32) + a + _unpack(xn_v[hrows(t), cols(c)]).astype(_F32)
        if t == n_sub - 1:
            sel = jax.lax.broadcasted_iota(jnp.int32, (_SUB, _CB), 0) == (idx - row0[t])
            res = res + jnp.where(sel, st["y"][:, c * _CB:(c + 1) * _CB], 0.0)
        out_v[rows(t), cols(c)] = res.astype(_BF16)
        if t == n_sub - 1:
            l_cp[c].start()
        elif c == n_cb - 1:
            o_cp[t].start()
        ffn_step()

    def build_ffn():
        xs = _unpack(xn_v[pl.ds(pl.multiple_of(idx16 // 2, 8), 8), :]).astype(_F32)
        sel = jax.lax.broadcasted_iota(jnp.int32, (16, D), 0) == (idx - idx16)
        xs = jnp.sum(jnp.where(sel, xs, 0.0), axis=0, keepdims=True)
        for g in range(n_groups):
            xcol_v[pl.ds(g * _G, _G), :] = _col_bcast(xs[:, g * _G:(g + 1) * _G])
        fs = {}
        n_f = F // _CB

        def matvec(w):
            xc = xcol_v[...]
            xc = jnp.concatenate([xc] * (_CB // _G), axis=1)
            acc = jnp.sum((w.astype(_F32) * xc).reshape(D // 8, 8, _CB), axis=0)
            return jnp.sum(acc, axis=0, keepdims=True)

        def piece(f):
            fsl = pl.ds(f * _CB, _CB)
            g = matvec(wg_v[:, fsl])
            u = matvec(wu_v[:, fsl])
            h = g * jax.nn.sigmoid(g) * u
            fs["h"] = h

        def down(f, j):
            hb = jnp.broadcast_to(fs["h"][:, j * _G:(j + 1) * _G], (16, _G)).astype(_BF16)
            part = _dot(hb, wd_v[pl.ds(f * _CB + j * _G, _G), dcols])
            fs["y"] = part if "y" not in fs else fs["y"] + part
            if f == n_f - 1 and j == _CB // _G - 1:
                st["y"] = fs["y"][0:1, :] * jax.nn.sigmoid(rmax)

        for f in range(n_f):
            ffn_q.append(lambda: None)
            ffn_q.append(lambda f=f: (piece(f), down(f, 0)))
            ffn_q.append(functools.partial(down, f, 1))

    for g in range(n_groups):
        z_job(g)
    q_job(0, 0)
    g_job(*pending.pop(0))
    q_job(0, 1)
    for g in range(n_groups):
        kv_job(g)
    q_job(0, 2)
    for g in range(n_groups):
        m_job(g)
    q_job(0, 3)
    for name in ("g", "u", "d"):
        w_cp[name].wait()
    build_ffn()
    for t in range(1, n_sub + 1):
        if t == n_sub:
            while ffn_q:
                ffn_step()
        for c in range(n_cb):
            if t < n_sub:
                q_job(t, c)
            out_job(t - 1, c)
    for cp in o_cp + l_cp:
        cp.wait()


@jax.jit
def pallas_parallel_sum__linear_attn_block__moe_arch_mod__prompt_kernel(
    A_x: jax.Array,
    A_wqkv: jax.Array,
    A_wo: jax.Array,
    B_x: jax.Array,
    B_w_r: jax.Array,
    B_w_gate: jax.Array,
    B_w_up: jax.Array,
    B_w_down: jax.Array,
):
    del B_x
    B, S, D = A_x.shape
    assert B == 1
    F = B_w_gate.shape[1]
    any_spec = pl.BlockSpec(memory_space=pl.ANY)
    out = pl.pallas_call(
        functools.partial(_kernel, S=S, D=D, F=F),
        out_shape=jax.ShapeDtypeStruct((S, D), A_x.dtype),
        in_specs=[any_spec, any_spec, any_spec,
                  pl.BlockSpec(memory_space=pltpu.VMEM),
                  any_spec, any_spec, any_spec],
        out_specs=any_spec,
        scratch_shapes=[
            pltpu.VMEM((S, D), _BF16),
            pltpu.VMEM((D, D + _PAD), _BF16),
            pltpu.VMEM((D, D + _PAD), _BF16),
            pltpu.VMEM((D, D + _PAD), _BF16),
            pltpu.VMEM((D, D + _PAD), _BF16),
            pltpu.VMEM((D, F), _BF16),
            pltpu.VMEM((D, F), _BF16),
            pltpu.VMEM((F, D + _PAD), _BF16),
            pltpu.VMEM((S // 2, D), _U32),
            pltpu.VMEM((D // 2, D), _U32),
            pltpu.VMEM((D, D), _F32),
            pltpu.VMEM((D, _G), _F32),
            pltpu.VMEM((D, _G), _F32),
            pltpu.VMEM((D // 2, D), _U32),
            pltpu.VMEM((S, D), _BF16),
            pltpu.SemaphoreType.DMA((4,)),
            pltpu.SemaphoreType.DMA((3,)),
            pltpu.SemaphoreType.DMA((6,)),
            pltpu.SemaphoreType.DMA((S // _SUB - 1,)),
            pltpu.SemaphoreType.DMA((D // _CB,)),
            pltpu.SemaphoreType.REGULAR,
        ],
        compiler_params=pltpu.CompilerParams(vmem_limit_bytes=100 * 1024 * 1024),
    )(A_x.reshape(S, D), A_wqkv, A_wo, B_w_r.reshape(1, D), B_w_gate, B_w_up, B_w_down)
    return out.reshape(B, S, D)
```

```python
import contextlib
import functools
import os

import jax
import jax.numpy as jnp
import jax.experimental.pallas as pl
import jax.experimental.pallas.tpu as pltpu

_H = 32
_LN_EPS = 1e-5
_PHI_EPS = 1e-6
_DEN_EPS = 1e-6
_SUB = 256
_CB = 256
_LNR = 16
_G = 128
_PAD = 128

_SCOPES = bool(os.environ.get("KSCOPES"))


def _scope(name):
    return jax.named_scope(name) if _SCOPES else contextlib.nullcontext()


_F32 = jnp.float32
_BF16 = jnp.bfloat16
_U32 = jnp.uint32


def _dot(a, b):
    return jnp.dot(a, b, preferred_element_type=_F32)


def _dot_tn(a, b):
    return jax.lax.dot_general(a, b, (((0,), (0,)), ((), ())), preferred_element_type=_F32)


def _dot_nt(a, b):
    return jax.lax.dot_general(a, b, (((1,), (1,)), ((), ())), preferred_element_type=_F32)


def _phi(t):
    return jnp.where(t > 0, t + 1.0, jnp.exp(t)) + _PHI_EPS


def _pack(v):
    return pltpu.bitcast(v, _U32)


def _unpack(v):
    return pltpu.bitcast(v, _BF16)


def _col_bcast(row):
    return jnp.broadcast_to(row, (_G, _G)).T


def _kernel(x_hbm, wqkv_hbm, wo_hbm, wr_hbm, wg_hbm, wu_hbm, wd_hbm, out_hbm,
            x_v, wq_v, wk_v, wv_v, wo_v, wr_v, gu_v, wd_v,
            sa_v, sb_v, xn_v, wqt_v, g_v, zcol_v, xcol_v, hcol_v, m_v, out_v,
            sem_i, sem_o, sem_b, *, S, D, F):
    n_sub = S // _SUB
    n_cb = D // _CB
    n_groups = D // _G
    dh = D // _H
    n_it = n_sub // 2
    fc = F // n_it
    hs = _SUB // 2

    cols = lambda c: pl.ds(c * _CB, _CB)
    dcols = pl.ds(0, D)

    def x_cp(a, b, s):
        sl = pl.ds(a * _SUB, (b - a) * _SUB)
        return pltpu.make_async_copy(x_hbm.at[sl, :], x_v.at[sl, :], sem_i.at[s])

    def k_cp(a, b, s):
        return pltpu.make_async_copy(wqkv_hbm.at[:, pl.ds(D + a * _CB, (b - a) * _CB)],
                                     wk_v.at[:, pl.ds(a * _CB, (b - a) * _CB)], sem_i.at[s])

    def gu_cps(j, s):
        return [pltpu.make_async_copy(wg_hbm.at[:, pl.ds(j * fc, fc)], gu_v.at[j, :, pl.ds(0, fc)], sem_i.at[s]),
                pltpu.make_async_copy(wu_hbm.at[:, pl.ds(j * fc, fc)], gu_v.at[j, :, pl.ds(fc, fc)], sem_i.at[s])]

    def d_cp(j, s):
        return pltpu.make_async_copy(wd_hbm.at[pl.ds(j * fc, fc), :], wd_v.at[j, :, dcols], sem_i.at[s])

    groups = [
        [pltpu.make_async_copy(wr_hbm, wr_v, sem_i.at[0]), x_cp(0, 1, 0)],
        [k_cp(0, 1, 1)],
        [k_cp(1, 2, 2)],
        [k_cp(2, n_cb, 3), x_cp(1, 2, 3)],
        [x_cp(2, 4, 4)],
        [x_cp(4, n_sub, 5)],
        [pltpu.make_async_copy(wqkv_hbm.at[:, pl.ds(0, D)], wq_v.at[:, dcols], sem_i.at[6]),
         pltpu.make_async_copy(wqkv_hbm.at[:, pl.ds(2 * D, D)], wv_v.at[:, dcols], sem_i.at[6]),
         pltpu.make_async_copy(wo_hbm, wo_v.at[:, dcols], sem_i.at[6])] + gu_cps(0, 6),
        gu_cps(1, 7) + [d_cp(0, 7)],
        sum([gu_cps(j, 8) for j in range(2, n_it)], []) + [d_cp(j, 8) for j in range(1, n_it)],
    ]

    def start(cps):
        for cp in cps:
            cp.start()
            pl.semaphore_signal(sem_b, 1)
            pl.semaphore_wait(sem_b, 1)

    def wait(name, cps):
        with _scope(name):
            for cp in cps:
                cp.wait()

    for grp in groups:
        start(grp)

    zero = pl.semaphore_read(sem_b)
    zero8 = pl.multiple_of(zero * 8, 8)
    zero_u = zero.astype(_U32)
    zero_f = zero.astype(_F32)

    def zero_like(v):
        return pltpu.bitcast(pltpu.bitcast(v, _U32) & zero_u, _F32)

    wait("w_x0", groups[0])
    wr8 = wr_v[...].astype(_F32)
    wr = jnp.concatenate([wr8[g:g + 1, :] for g in range(n_groups)], axis=1)
    wr_sum = jnp.sum(wr, axis=-1, keepdims=True)
    sub_iota = jax.lax.broadcasted_iota(jnp.int32, (8, 1), 0)

    def ln_tile(st, tile, stage, chain_from=0, rows=_LNR, throttle=True):
        gsl = lambda g: slice(g * _G, (g + 1) * _G)
        for j in range(_SUB // rows):
            if isinstance(tile, int):
                r0 = tile * _SUB + j * rows
                h0 = r0 // 2
            else:
                r0 = pl.multiple_of(tile * _SUB + j * rows, rows)
                h0 = pl.multiple_of(tile * hs + j * (rows // 2), rows // 2)
            x = x_v[pl.ds(r0, rows), :].astype(_F32)

            def lane_partial(terms, dep):
                acc = terms[0] if dep is None else dep + terms[0]
                for t in terms[1:]:
                    acc = acc + t
                return acc

            dep = None
            if j >= chain_from:
                dep = pltpu.bitcast(stage[pl.ds(zero8, 8), pl.ds(0, _G)] & zero_u, _F32)
                dep = jnp.concatenate([dep] * (rows // 8), axis=0)
            s1 = lane_partial([x[:, gsl(g)] for g in range(n_groups)], dep)
            s2 = lane_partial([x[:, gsl(g)] * x[:, gsl(g)] for g in range(n_groups)],
                              zero_like(s1) if throttle else None)
            s3 = lane_partial([x[:, gsl(g)] * wr[:, gsl(g)] for g in range(n_groups)],
                              zero_like(s2) if throttle else None)
            m = jnp.sum(s1, axis=-1, keepdims=True) * (1.0 / D)
            ex2 = jnp.sum(s2, axis=-1, keepdims=True) * (1.0 / D)
            xw = jnp.sum(s3, axis=-1, keepdims=True)
            v = jnp.maximum(ex2 - m * m, 0.0)
            rstd = jax.lax.rsqrt(v + _LN_EPS)
            r = (xw - m * wr_sum) * rstd
            r = r.astype(_BF16).astype(_F32)
            rstd = jnp.where(r != r, r, rstd)
            for t in range(rows // 8):
                rt = r[t * 8:(t + 1) * 8, :]
                upd = rt > st["best"]
                st["best"] = jnp.where(upd, rt, st["best"])
                st["besti"] = jnp.where(upd, sub_iota + (r0 + t * 8), st["besti"])
            mb = jnp.broadcast_to(m, (rows, _G))
            for c in range(n_cb):
                xc = x_v[pl.ds(pl.multiple_of(r0 + zero * rows, rows), rows), cols(c)].astype(_F32)
                xn = _pack(((xc - jnp.concatenate([mb] * (_CB // _G), axis=1)) * rstd).astype(_BF16))
                stage[pl.ds(j * rows // 2, rows // 2), cols(c)] = xn
                xn_v[pl.ds(h0, rows // 2), cols(c)] = xn
                if throttle and c + 1 < n_cb:
                    d = pltpu.bitcast((xn[:, :_G] | xn[:, _G:]) & zero_u, _F32)
                    mb = mb + jnp.concatenate([d, d], axis=0)

    def k_job(st, stage, c):
        p = _phi(_dot(_unpack(stage[...]), wk_v[:, cols(c)]))
        zs = jnp.sum(p.reshape(_SUB // 8, 8, _CB), axis=0)
        st["z"][c] = zs if st["z"][c] is None else st["z"][c] + zs
        return p.astype(_BF16)

    def g_job(pk, stage, c, first=False):
        upd = _dot_tn(pk, _unpack(stage[...]))
        if first:
            g_v[cols(c), :] = upd
        else:
            g_v[cols(c), :] += upd

    st = dict(best=jnp.full((8, 1), -jnp.inf, _F32), besti=jnp.zeros((8, 1), jnp.int32), z=[None] * n_cb)
    ln_tile(st, 0, sb_v, chain_from=_SUB, throttle=False)
    wait("w_k0", groups[1])
    p0 = k_job(st, sb_v, 0)
    wait("w_k1", groups[2])
    p1 = k_job(st, sb_v, 1)
    g_job(p0, sb_v, 0, True)
    g_job(p1, sb_v, 1, True)
    wait("w_k2x1", groups[3])
    ln_tile(st, 1, sa_v, chain_from=1, rows=2 * _LNR)
    p2 = k_job(st, sb_v, 2)
    p3 = k_job(st, sb_v, 3)
    g_job(p2, sb_v, 2, True)
    g_job(p3, sb_v, 3, True)
    wait("w_x23", groups[4])

    def phase1(i, carry):
        st = dict(best=carry[0], besti=carry[1], z=list(carry[2:]))

        @pl.when(i == 1)
        def _():
            wait("w_x47", groups[5])

        ln_tile(st, 2 * i + 2, sb_v)
        seq = [(sa_v, c) for c in range(n_cb)] + [(sb_v, c) for c in range(n_cb)]
        pend = []
        for n, (stage, c) in enumerate(seq):
            pend.append((k_job(st, stage, c), stage, c))
            if n >= 1:
                g_job(*pend.pop(0))
            if n == n_cb:
                ln_tile(st, 2 * i + 3, sa_v)
        g_job(*pend.pop(0))
        return (st["best"], st["besti"], *st["z"])

    carry = jax.lax.fori_loop(0, (n_sub - 2) // 2, phase1, (st["best"], st["besti"], *st["z"]))
    st = dict(best=carry[0], besti=carry[1], z=list(carry[2:]))
    wait("w_qvo", groups[6])

    rmax = jnp.max(st["best"], axis=0, keepdims=True)
    idx = jnp.min(jnp.where(st["best"] == rmax, st["besti"], S - 1))
    idx16 = (idx // 16) * 16
    idx_tile = idx // _SUB
    gate_r = jax.nn.sigmoid(rmax)

    xs = _unpack(xn_v[pl.ds(pl.multiple_of(idx16 // 2, 8), 8), :]).astype(_F32)
    sel = jax.lax.broadcasted_iota(jnp.int32, (16, D), 0) == (idx - idx16)
    xs = jnp.sum(jnp.where(sel, xs, 0.0), axis=0, keepdims=True)
    for g in range(n_groups):
        xcol_v[pl.ds(g * _G, _G), :] = _col_bcast(xs[:, g * _G:(g + 1) * _G])

    def chain_matvec(w, colv, acc0):
        colv = jnp.concatenate([colv] * (w.shape[1] // _G), axis=1)
        n = w.shape[0] // 8
        prod = (w.astype(_F32) * colv).reshape(n, 1, 8, w.shape[1])
        pad = jnp.broadcast_to(zero_f, prod.shape)
        prod = jnp.concatenate([prod, pad], axis=1).reshape(2 * n, 8, w.shape[1])
        return jnp.sum(jnp.concatenate([acc0[None], prod], axis=0), axis=0)

    def gate_up(j):
        dep = jnp.zeros((8, _CB), _F32)
        accs = []
        for f in range(2 * fc // _CB):
            accs.append(chain_matvec(gu_v[j, :, cols(f)], xcol_v[...], dep))
            dep = zero_like(accs[-1])
        gu = jnp.sum(jnp.concatenate(accs, axis=1), axis=0, keepdims=True)
        g, u = gu[:, :fc], gu[:, fc:]
        return (g * jax.nn.sigmoid(g) * u).astype(_BF16).astype(_F32), dep

    def store_hcol(h, fs=range(fc // _G)):
        for f in fs:
            hcol_v[pl.ds(f * _G, _G), :] = _col_bcast(h[:, f * _G:(f + 1) * _G])

    store_hcol(gate_up(0)[0])

    rr = jax.lax.broadcasted_iota(jnp.int32, (_G, _G), 0) // dh
    cc = jax.lax.broadcasted_iota(jnp.int32, (_G, _G), 1) // dh
    same_head = rr == cc

    for a in range(n_cb):
        for b in range(n_cb):
            wqt_v[pl.ds(b * _CB // 2, _CB // 2), cols(a)] = _pack(wq_v[cols(a), cols(b)].T)

    kvb = {}

    def kv_job(c):
        for g in range(c * _CB // _G, (c + 1) * _CB // _G):
            gs = pl.ds(g * _G, _G)
            kv = _dot(g_v[gs, :].astype(_BF16), wv_v[:, gs])
            kvb[g] = jnp.where(same_head, kv, 0.0).astype(_BF16)

    def m_job(c):
        for g in range(c * _CB // _G, (c + 1) * _CB // _G):
            m_v[pl.ds(g * _G // 2, _G // 2), :] = _pack(
                _dot(kvb.pop(g), wo_v[pl.ds(g * _G, _G), dcols]).astype(_BF16))

    pk = [k_job(st, sa_v, 0), k_job(st, sa_v, 1)]
    g_job(pk[0], sa_v, 0)
    pk.append(k_job(st, sa_v, 2))
    g_job(pk[1], sa_v, 1)
    pk.append(k_job(st, sa_v, 3))
    kv_job(0)
    g_job(pk[2], sa_v, 2)
    kv_job(1)
    m_job(0)
    g_job(pk[3], sa_v, 3)
    kv_job(2)
    m_job(1)
    kv_job(3)
    m_job(2)
    m_job(3)
    for g in range(n_groups):
        c, j = divmod(g, _CB // _G)
        z = jnp.sum(st["z"][c][:, j * _G:(j + 1) * _G], axis=0, keepdims=True)
        zcol_v[pl.ds(g * _G, _G), :] = _col_bcast(z)

    wait("w_f0", groups[7])

    def phase2(i, yacc):
        @pl.when(i == 1)
        def _():
            wait("w_f1", groups[8])

        tiles = [(idx_tile + 1 + 2 * i + t) % n_sub for t in range(2)]
        row0 = [pl.multiple_of(t * _SUB, _SUB) for t in tiles]
        half0 = [pl.multiple_of(t * hs, hs) for t in tiles]

        hnext, dep = gate_up(jnp.minimum(i + 1, n_it - 1))
        ys = []
        for c in range(n_cb):
            ys.append(chain_matvec(wd_v[i, :, cols(c)], hcol_v[...], yacc[:, c * _CB:(c + 1) * _CB] + dep))
            dep = zero_like(ys[-1])
        yacc = jnp.concatenate(ys, axis=1)
        yrow = jnp.sum(yacc, axis=0, keepdims=True) * gate_r

        ob = {}

        def q_job(t, c):
            xn = _unpack(xn_v[pl.ds(half0[t], hs), :])
            p = _phi(_dot_nt(_unpack(wqt_v[pl.ds(c * _CB // 2, _CB // 2), :]), xn))
            zc = zcol_v[cols(c), :]
            zc = jnp.concatenate([zc] * (_SUB // _G), axis=1)
            p3 = p.reshape(_CB // dh, dh, _SUB)
            den = jnp.sum(p3 * zc.reshape(_CB // dh, dh, _SUB), axis=1, keepdims=True) + _DEN_EPS
            o = (p3 * pl.reciprocal(den, approx=True)).reshape(_CB, _SUB).astype(_BF16)
            ob[t, c] = o.T

        def out_job(t, c):
            if c == 0:
                ob[t] = jnp.concatenate([ob.pop((t, cb)) for cb in range(n_cb)], axis=1)
            rows = pl.ds(row0[t], _SUB)
            a = _dot(ob[t], _unpack(m_v[:, cols(c)]))
            res = x_v[rows, cols(c)].astype(_F32) + a + _unpack(xn_v[pl.ds(half0[t], hs), cols(c)]).astype(_F32)
            if t == 1:
                sel = jax.lax.broadcasted_iota(jnp.int32, (_SUB, _CB), 0) == (idx - row0[t])
                store_hcol(hnext, range(2 * c, min(2 * c + 2, fc // _G)))
                pin = zero_like(hcol_v[pl.ds(zero8, 1), :])
                yc = yrow[:, c * _CB:(c + 1) * _CB] + jnp.concatenate([pin] * (_CB // _G), axis=1)
                res = res + jnp.where(sel, yc, 0.0)
            out_v[rows, cols(c)] = res.astype(_BF16)
            if t == 1:
                pltpu.make_async_copy(out_v.at[rows, cols(c)], out_hbm.at[rows, cols(c)], sem_o).start()
            elif c == n_cb - 1:
                pltpu.make_async_copy(out_v.at[rows, :], out_hbm.at[rows, :], sem_o).start()

        for c in range(n_cb):
            q_job(0, c)
        for c in range(n_cb):
            q_job(1, c)
            out_job(0, c)
        for c in range(n_cb):
            out_job(1, c)
        return yacc

    jax.lax.fori_loop(0, n_it, phase2, jnp.zeros((8, D), _F32))
    wait("w_out", [pltpu.make_async_copy(out_v, out_hbm, sem_o)])


@jax.jit
def pallas_parallel_sum__linear_attn_block__moe_arch_mod__prompt_kernel(
    A_x: jax.Array,
    A_wqkv: jax.Array,
    A_wo: jax.Array,
    B_x: jax.Array,
    B_w_r: jax.Array,
    B_w_gate: jax.Array,
    B_w_up: jax.Array,
    B_w_down: jax.Array,
):
    del B_x
    B, S, D = A_x.shape
    assert B == 1
    F = B_w_gate.shape[1]
    n_it = S // _SUB // 2
    fc = F // n_it
    any_spec = pl.BlockSpec(memory_space=pl.ANY)
    out = pl.pallas_call(
        functools.partial(_kernel, S=S, D=D, F=F),
        out_shape=jax.ShapeDtypeStruct((S, D), A_x.dtype),
        in_specs=[any_spec] * 7,
        out_specs=any_spec,
        scratch_shapes=[
            pltpu.VMEM((S, D), _BF16),
            pltpu.VMEM((D, D + _PAD), _BF16),
            pltpu.VMEM((D, D + _PAD), _BF16),
            pltpu.VMEM((D, D + _PAD), _BF16),
            pltpu.VMEM((D, D + _PAD), _BF16),
            pltpu.VMEM((D // _G, _G), _BF16),
            pltpu.VMEM((n_it, D, 2 * fc), _BF16),
            pltpu.VMEM((n_it, fc, D + _PAD), _BF16),
            pltpu.VMEM((_SUB // 2, D), _U32),
            pltpu.VMEM((_SUB // 2, D), _U32),
            pltpu.VMEM((S // 2, D), _U32),
            pltpu.VMEM((D // 2, D), _U32),
            pltpu.VMEM((D, D), _F32),
            pltpu.VMEM((D, _G), _F32),
            pltpu.VMEM((D, _G), _F32),
            pltpu.VMEM((fc, _G), _F32),
            pltpu.VMEM((D // 2, D), _U32),
            pltpu.VMEM((S, D), _BF16),
            pltpu.SemaphoreType.DMA((9,)),
            pltpu.SemaphoreType.DMA,
            pltpu.SemaphoreType.REGULAR,
        ],
        compiler_params=pltpu.CompilerParams(vmem_limit_bytes=100 * 1024 * 1024),
    )(A_x.reshape(S, D), A_wqkv, A_wo, B_w_r.reshape(D // _G, _G), B_w_gate, B_w_up, B_w_down)
    return out.reshape(B, S, D)
```

```python
import contextlib
import functools
import os

import jax
import jax.numpy as jnp
import jax.experimental.pallas as pl
import jax.experimental.pallas.tpu as pltpu

_H = 32
_LN_EPS = 1e-5
_PHI_EPS = 1e-6
_DEN_EPS = 1e-6
_SUB = 256
_CB = 256
_LNR = 16
_G = 128
_BLK = int(os.environ.get('BLK', 8))
_PAD = 128

_SCOPES = bool(os.environ.get("KSCOPES"))


def _scope(name):
    return jax.named_scope(name) if _SCOPES else contextlib.nullcontext()


_F32 = jnp.float32
_BF16 = jnp.bfloat16
_U32 = jnp.uint32


def _dot(a, b):
    return jnp.dot(a, b, preferred_element_type=_F32)


def _dot_tn(a, b):
    return jax.lax.dot_general(a, b, (((0,), (0,)), ((), ())), preferred_element_type=_F32)


def _dot_nt(a, b):
    return jax.lax.dot_general(a, b, (((1,), (1,)), ((), ())), preferred_element_type=_F32)


def _phi(t):
    return jnp.where(t > 0, t + 1.0, jnp.exp(t)) + _PHI_EPS


def _pack(v):
    return pltpu.bitcast(v, _U32)


def _unpack(v):
    return pltpu.bitcast(v, _BF16)


def _col_bcast(row):
    return jnp.broadcast_to(row, (_G, _G)).T


def _kernel(x_hbm, wqkv_hbm, wo_hbm, wr_hbm, wg_hbm, wu_hbm, wd_hbm, out_hbm,
            x_v, wq_v, wk_v, wv_v, wo_v, wr_v, gu_v, wd_v,
            sa_v, sb_v, xn_v, wqt_v, g_v, zcol_v, xcol_v, hcol_v, m_v, out_v,
            sem_i, sem_o, sem_b, *, S, D, F):
    n_sub = S // _SUB
    n_cb = D // _CB
    n_groups = D // _G
    dh = D // _H
    n_it = n_sub // 2
    fc = F // n_it
    hs = _SUB // 2

    cols = lambda c: pl.ds(c * _CB, _CB)
    dcols = pl.ds(0, D)

    def x_cp(a, b, s):
        sl = pl.ds(a * _SUB, (b - a) * _SUB)
        return pltpu.make_async_copy(x_hbm.at[sl, :], x_v.at[sl, :], sem_i.at[s])

    def k_cp(a, b, s):
        return pltpu.make_async_copy(wqkv_hbm.at[:, pl.ds(D + a * _CB, (b - a) * _CB)],
                                     wk_v.at[:, pl.ds(a * _CB, (b - a) * _CB)], sem_i.at[s])

    def gu_cps(j, s):
        return [pltpu.make_async_copy(wg_hbm.at[:, pl.ds(j * fc, fc)], gu_v.at[j, :, pl.ds(0, fc)], sem_i.at[s]),
                pltpu.make_async_copy(wu_hbm.at[:, pl.ds(j * fc, fc)], gu_v.at[j, :, pl.ds(fc, fc)], sem_i.at[s])]

    def d_cp(j, s):
        return pltpu.make_async_copy(wd_hbm.at[pl.ds(j * fc, fc), :], wd_v.at[j, :, dcols], sem_i.at[s])

    groups = [
        [pltpu.make_async_copy(wr_hbm, wr_v, sem_i.at[0]), x_cp(0, 1, 0)],
        [k_cp(0, 1, 1)],
        [k_cp(1, 2, 2)],
        [k_cp(2, n_cb, 3), x_cp(1, 2, 3)],
        [x_cp(2, 4, 4)],
        [x_cp(4, n_sub, 5)],
        [pltpu.make_async_copy(wqkv_hbm.at[:, pl.ds(0, D)], wq_v.at[:, dcols], sem_i.at[6]),
         pltpu.make_async_copy(wqkv_hbm.at[:, pl.ds(2 * D, D)], wv_v.at[:, dcols], sem_i.at[6]),
         pltpu.make_async_copy(wo_hbm, wo_v.at[:, dcols], sem_i.at[6])] + gu_cps(0, 6),
        gu_cps(1, 7) + [d_cp(0, 7)],
        sum([gu_cps(j, 8) for j in range(2, n_it)], []) + [d_cp(j, 8) for j in range(1, n_it)],
    ]

    def start(cps):
        for cp in cps:
            cp.start()
            pl.semaphore_signal(sem_b, 1)
            pl.semaphore_wait(sem_b, 1)

    def wait(name, cps):
        with _scope(name):
            for cp in cps:
                cp.wait()

    for grp in groups:
        start(grp)

    zero = pl.semaphore_read(sem_b)
    zero8 = pl.multiple_of(zero * 8, 8)
    zero_u = zero.astype(_U32)
    zero_f = zero.astype(_F32)

    def zero_like(v):
        return pltpu.bitcast(pltpu.bitcast(v, _U32) & zero_u, _F32)

    def zero_link(v):
        d = pltpu.bitcast(v, _U32)
        d = pltpu.bitcast((d[:, :_G] | d[:, _G:]) & zero_u, _F32)
        return jnp.concatenate([d, d], axis=1)

    wait("w_x0", groups[0])
    wr8 = wr_v[...].astype(_F32)
    wr = jnp.concatenate([wr8[g:g + 1, :] for g in range(n_groups)], axis=1)
    wr_sum = jnp.sum(wr, axis=-1, keepdims=True)
    sub_iota = jax.lax.broadcasted_iota(jnp.int32, (8, 1), 0)

    def ln_tile(st, tile, stage, chain_from=0, rows=_LNR, throttle=True):
        gsl = lambda g: slice(g * _G, (g + 1) * _G)
        for j in range(_SUB // rows):
            if isinstance(tile, int):
                r0 = tile * _SUB + j * rows
                h0 = r0 // 2
            else:
                r0 = pl.multiple_of(tile * _SUB + j * rows, rows)
                h0 = pl.multiple_of(tile * hs + j * (rows // 2), rows // 2)
            x = x_v[pl.ds(r0, rows), :].astype(_F32)

            def lane_partial(terms, dep):
                acc = terms[0] if dep is None else dep + terms[0]
                for t in terms[1:]:
                    acc = acc + t
                return acc

            dep = None
            if j >= chain_from:
                dep = pltpu.bitcast(stage[pl.ds(zero8, 8), pl.ds(0, _G)] & zero_u, _F32)
                dep = jnp.concatenate([dep] * (rows // 8), axis=0)
            s1 = lane_partial([x[:, gsl(g)] for g in range(n_groups)], dep)
            s2 = lane_partial([x[:, gsl(g)] * x[:, gsl(g)] for g in range(n_groups)],
                              zero_like(s1) if throttle else None)
            s3 = lane_partial([x[:, gsl(g)] * wr[:, gsl(g)] for g in range(n_groups)],
                              zero_like(s2) if throttle else None)
            m = jnp.sum(s1, axis=-1, keepdims=True) * (1.0 / D)
            ex2 = jnp.sum(s2, axis=-1, keepdims=True) * (1.0 / D)
            xw = jnp.sum(s3, axis=-1, keepdims=True)
            v = jnp.maximum(ex2 - m * m, 0.0)
            rstd = jax.lax.rsqrt(v + _LN_EPS)
            r = (xw - m * wr_sum) * rstd
            r = r.astype(_BF16).astype(_F32)
            rstd = jnp.where(r != r, r, rstd)
            for t in range(rows // 8):
                rt = r[t * 8:(t + 1) * 8, :]
                upd = rt > st["best"]
                st["best"] = jnp.where(upd, rt, st["best"])
                st["besti"] = jnp.where(upd, sub_iota + (r0 + t * 8), st["besti"])
            mb = jnp.broadcast_to(m, (rows, _G))
            for c in range(n_cb):
                xc = x_v[pl.ds(pl.multiple_of(r0 + zero * rows, rows), rows), cols(c)].astype(_F32)
                xn = _pack(((xc - jnp.concatenate([mb] * (_CB // _G), axis=1)) * rstd).astype(_BF16))
                stage[pl.ds(j * rows // 2, rows // 2), cols(c)] = xn
                xn_v[pl.ds(h0, rows // 2), cols(c)] = xn
                if throttle and c + 1 < n_cb:
                    d = pltpu.bitcast((xn[:, :_G] | xn[:, _G:]) & zero_u, _F32)
                    mb = mb + jnp.concatenate([d, d], axis=0)

    def k_job(st, stage, c):
        p = _phi(_dot(_unpack(stage[...]), wk_v[:, cols(c)]))
        zs = jnp.sum(p.reshape(_SUB // 8, 8, _CB), axis=0)
        st["z"][c] = zs if st["z"][c] is None else st["z"][c] + zs
        return p.astype(_BF16)

    def g_job(pk, stage, c, first=False):
        upd = _dot_tn(pk, _unpack(stage[...]))
        if first:
            g_v[cols(c), :] = upd
        else:
            g_v[cols(c), :] += upd

    st = dict(best=jnp.full((8, 1), -jnp.inf, _F32), besti=jnp.zeros((8, 1), jnp.int32), z=[None] * n_cb)
    ln_tile(st, 0, sb_v, chain_from=_SUB, throttle=False)
    wait("w_k0", groups[1])
    p0 = k_job(st, sb_v, 0)
    wait("w_k1", groups[2])
    p1 = k_job(st, sb_v, 1)
    g_job(p0, sb_v, 0, True)
    g_job(p1, sb_v, 1, True)
    wait("w_k2x1", groups[3])
    ln_tile(st, 1, sa_v, chain_from=1, rows=2 * _LNR)
    p2 = k_job(st, sb_v, 2)
    p3 = k_job(st, sb_v, 3)
    g_job(p2, sb_v, 2, True)
    g_job(p3, sb_v, 3, True)
    wait("w_x23", groups[4])

    def phase1(i, carry):
        st = dict(best=carry[0], besti=carry[1], z=list(carry[2:]))

        @pl.when(i == 1)
        def _():
            wait("w_x47", groups[5])

        ln_tile(st, 2 * i + 2, sb_v)
        seq = [(sa_v, c) for c in range(n_cb)] + [(sb_v, c) for c in range(n_cb)]
        pend = []
        for n, (stage, c) in enumerate(seq):
            pend.append((k_job(st, stage, c), stage, c))
            if n >= 1:
                g_job(*pend.pop(0))
            if n == n_cb:
                ln_tile(st, 2 * i + 3, sa_v)
        g_job(*pend.pop(0))
        return (st["best"], st["besti"], *st["z"])

    carry = jax.lax.fori_loop(0, (n_sub - 2) // 2, phase1, (st["best"], st["besti"], *st["z"]))
    st = dict(best=carry[0], besti=carry[1], z=list(carry[2:]))
    wait("w_qvo", groups[6])

    rmax = jnp.max(st["best"], axis=0, keepdims=True)
    idx = jnp.min(jnp.where(st["best"] == rmax, st["besti"], S - 1))
    idx16 = (idx // 16) * 16
    idx_tile = idx // _SUB
    gate_r = jax.nn.sigmoid(rmax)

    xs = _unpack(xn_v[pl.ds(pl.multiple_of(idx16 // 2, 8), 8), :]).astype(_F32)
    sel = jax.lax.broadcasted_iota(jnp.int32, (16, D), 0) == (idx - idx16)
    xs = jnp.sum(jnp.where(sel, xs, 0.0), axis=0, keepdims=True)
    for g in range(n_groups):
        xcol_v[pl.ds(g * _G, _G), :] = _col_bcast(xs[:, g * _G:(g + 1) * _G])

    def chain_matvec(w_ref, lead, cb, col_ref, acc0, off=0):
        n = col_ref.shape[0] // 8
        acc = [acc0[:, :_G], acc0[:, _G:]]
        link = None
        for k0 in range(0, n, _BLK):
            rows = pl.ds(k0 * 8, _BLK * 8)
            w = w_ref[lead, rows, cols(cb)].astype(_F32)
            colv = col_ref[rows if isinstance(off, int) else pl.ds(pl.multiple_of(k0 * 8 + off, 8), _BLK * 8), :]
            for h in range(2):
                prod = (w[:, h * _G:(h + 1) * _G] * colv).reshape(_BLK, 8, _G)
                start = acc[h] if link is None else acc[h] + link
                acc[h] = jnp.sum(jnp.concatenate([start[None], prod], axis=0), axis=0)
                link = zero_like(acc[h])
        return jnp.concatenate(acc, axis=1)

    def gate_up(j, off=0):
        dep = jnp.zeros((8, _CB), _F32)
        accs = []
        for f in range(2 * fc // _CB):
            accs.append(chain_matvec(gu_v, j, f, xcol_v, dep, off))
            dep = zero_link(accs[-1])
        gu = jnp.sum(jnp.concatenate(accs, axis=1), axis=0, keepdims=True)
        g, u = gu[:, :fc], gu[:, fc:]
        return (g * jax.nn.sigmoid(g) * u).astype(_BF16).astype(_F32), dep

    def store_hcol(h, fs=range(fc // _G)):
        for f in fs:
            hcol_v[pl.ds(f * _G, _G), :] = _col_bcast(h[:, f * _G:(f + 1) * _G])

    rr = jax.lax.broadcasted_iota(jnp.int32, (_G, _G), 0) // dh
    cc = jax.lax.broadcasted_iota(jnp.int32, (_G, _G), 1) // dh
    same_head = rr == cc

    for a in range(n_cb):
        for b in range(n_cb):
            wqt_v[pl.ds(b * _CB // 2, _CB // 2), cols(a)] = _pack(wq_v[cols(a), cols(b)].T)

    kvb = {}

    def kv_job(c):
        for g in range(c * _CB // _G, (c + 1) * _CB // _G):
            gs = pl.ds(g * _G, _G)
            kv = _dot(g_v[gs, :].astype(_BF16), wv_v[:, gs])
            kvb[g] = jnp.where(same_head, kv, 0.0).astype(_BF16)

    def m_job(c):
        for g in range(c * _CB // _G, (c + 1) * _CB // _G):
            m_v[pl.ds(g * _G // 2, _G // 2), :] = _pack(
                _dot(kvb.pop(g), wo_v[pl.ds(g * _G, _G), dcols]).astype(_BF16))

    pk = [k_job(st, sa_v, 0), k_job(st, sa_v, 1)]
    g_job(pk[0], sa_v, 0)
    pk.append(k_job(st, sa_v, 2))
    g_job(pk[1], sa_v, 1)
    pk.append(k_job(st, sa_v, 3))
    kv_job(0)
    g_job(pk[2], sa_v, 2)
    kv_job(1)
    m_job(0)
    g_job(pk[3], sa_v, 3)
    kv_job(2)
    m_job(1)
    kv_job(3)
    m_job(2)
    m_job(3)
    for g in range(n_groups):
        c, j = divmod(g, _CB // _G)
        z = jnp.sum(st["z"][c][:, j * _G:(j + 1) * _G], axis=0, keepdims=True)
        zcol_v[pl.ds(g * _G, _G), :] = _col_bcast(z)

    store_hcol(gate_up(0, zero8)[0])
    wait("w_f0", groups[7])

    def phase2(i, yacc):
        @pl.when(i == 1)
        def _():
            wait("w_f1", groups[8])

        tiles = [(idx_tile + 1 + 2 * i + t) % n_sub for t in range(2)]
        row0 = [pl.multiple_of(t * _SUB, _SUB) for t in tiles]
        half0 = [pl.multiple_of(t * hs, hs) for t in tiles]

        hnext, dep = gate_up(jnp.minimum(i + 1, n_it - 1))
        ys = []
        for c in range(n_cb):
            ys.append(chain_matvec(wd_v, i, c, hcol_v, yacc[:, c * _CB:(c + 1) * _CB] + dep))
            dep = zero_link(ys[-1])
        yacc = jnp.concatenate([y + dep for y in ys], axis=1)
        yrow = jnp.sum(yacc, axis=0, keepdims=True) * gate_r

        ob = {}

        def q_job(t, c):
            xn = _unpack(xn_v[pl.ds(half0[t], hs), :])
            p = _phi(_dot_nt(_unpack(wqt_v[pl.ds(c * _CB // 2, _CB // 2), :]), xn))
            zc = zcol_v[cols(c), :]
            zc = jnp.concatenate([zc] * (_SUB // _G), axis=1)
            p3 = p.reshape(_CB // dh, dh, _SUB)
            den = jnp.sum(p3 * zc.reshape(_CB // dh, dh, _SUB), axis=1, keepdims=True) + _DEN_EPS
            o = (p3 * pl.reciprocal(den, approx=True)).reshape(_CB, _SUB).astype(_BF16)
            ob[t, c] = o.T

        def out_job(t, c):
            if c == 0:
                ob[t] = jnp.concatenate([ob.pop((t, cb)) for cb in range(n_cb)], axis=1)
            rows = pl.ds(row0[t], _SUB)
            a = _dot(ob[t], _unpack(m_v[:, cols(c)]))
            res = x_v[rows, cols(c)].astype(_F32) + a + _unpack(xn_v[pl.ds(half0[t], hs), cols(c)]).astype(_F32)
            if t == 1:
                sel = jax.lax.broadcasted_iota(jnp.int32, (_SUB, _CB), 0) == (idx - row0[t])
                yc = yrow[:, c * _CB:(c + 1) * _CB]
                if c in (1, 2):
                    store_hcol(hnext, range(4 * (c - 1), min(4 * c, fc // _G)))
                    pin = zero_like(hcol_v[pl.ds(zero8, 1), :])
                    yc = yc + jnp.concatenate([pin] * (_CB // _G), axis=1)
                res = res + jnp.where(sel, yc, 0.0)
            out_v[rows, cols(c)] = res.astype(_BF16)
            if t == 1:
                pltpu.make_async_copy(out_v.at[rows, cols(c)], out_hbm.at[rows, cols(c)], sem_o).start()
            elif c == n_cb - 1:
                pltpu.make_async_copy(out_v.at[rows, :], out_hbm.at[rows, :], sem_o).start()

        for c in range(n_cb):
            q_job(0, c)
        for c in range(n_cb):
            q_job(1, c)
            out_job(0, c)
        for c in range(n_cb):
            out_job(1, c)
        return yacc

    jax.lax.fori_loop(0, n_it, phase2, jnp.zeros((8, D), _F32))
    wait("w_out", [pltpu.make_async_copy(out_v, out_hbm, sem_o)])


@jax.jit
def pallas_parallel_sum__linear_attn_block__moe_arch_mod__prompt_kernel(
    A_x: jax.Array,
    A_wqkv: jax.Array,
    A_wo: jax.Array,
    B_x: jax.Array,
    B_w_r: jax.Array,
    B_w_gate: jax.Array,
    B_w_up: jax.Array,
    B_w_down: jax.Array,
):
    del B_x
    B, S, D = A_x.shape
    assert B == 1
    F = B_w_gate.shape[1]
    n_it = S // _SUB // 2
    fc = F // n_it
    any_spec = pl.BlockSpec(memory_space=pl.ANY)
    out = pl.pallas_call(
        functools.partial(_kernel, S=S, D=D, F=F),
        out_shape=jax.ShapeDtypeStruct((S, D), A_x.dtype),
        in_specs=[any_spec] * 7,
        out_specs=any_spec,
        scratch_shapes=[
            pltpu.VMEM((S, D), _BF16),
            pltpu.VMEM((D, D + _PAD), _BF16),
            pltpu.VMEM((D, D + _PAD), _BF16),
            pltpu.VMEM((D, D + _PAD), _BF16),
            pltpu.VMEM((D, D + _PAD), _BF16),
            pltpu.VMEM((D // _G, _G), _BF16),
            pltpu.VMEM((n_it, D, 2 * fc), _BF16),
            pltpu.VMEM((n_it, fc, D + _PAD), _BF16),
            pltpu.VMEM((_SUB // 2, D), _U32),
            pltpu.VMEM((_SUB // 2, D), _U32),
            pltpu.VMEM((S // 2, D), _U32),
            pltpu.VMEM((D // 2, D), _U32),
            pltpu.VMEM((D, D), _F32),
            pltpu.VMEM((D, _G), _F32),
            pltpu.VMEM((D, _G), _F32),
            pltpu.VMEM((fc, _G), _F32),
            pltpu.VMEM((D // 2, D), _U32),
            pltpu.VMEM((S, D), _BF16),
            pltpu.SemaphoreType.DMA((9,)),
            pltpu.SemaphoreType.DMA,
            pltpu.SemaphoreType.REGULAR,
        ],
        compiler_params=pltpu.CompilerParams(vmem_limit_bytes=100 * 1024 * 1024),
    )(A_x.reshape(S, D), A_wqkv, A_wo, B_w_r.reshape(D // _G, _G), B_w_gate, B_w_up, B_w_down)
    return out.reshape(B, S, D)
```

```python
import contextlib
import functools
import os

import jax
import jax.numpy as jnp
import jax.experimental.pallas as pl
import jax.experimental.pallas.tpu as pltpu

_H = 32
_LN_EPS = 1e-5
_PHI_EPS = 1e-6
_DEN_EPS = 1e-6
_SUB = 256
_CB = 256
_LNR = 16
_G = 128
_BLK = 8
_PAD = 128

_SCOPES = bool(os.environ.get("KSCOPES"))
_CHECKS = bool(os.environ.get("KCHECKS"))


def _scope(name):
    return jax.named_scope(name) if _SCOPES else contextlib.nullcontext()


_F32 = jnp.float32
_BF16 = jnp.bfloat16
_U32 = jnp.uint32


def _dot(a, b):
    return jnp.dot(a, b, preferred_element_type=_F32)


def _dot_tn(a, b):
    return jax.lax.dot_general(a, b, (((0,), (0,)), ((), ())), preferred_element_type=_F32)


def _dot_nt(a, b):
    return jax.lax.dot_general(a, b, (((1,), (1,)), ((), ())), preferred_element_type=_F32)


def _phi(t):
    return jnp.where(t > 0, t + 1.0, jnp.exp(t)) + _PHI_EPS


def _pack(v):
    return pltpu.bitcast(v, _U32)


def _unpack(v):
    return pltpu.bitcast(v, _BF16)


def _col_bcast(row):
    return jnp.broadcast_to(row, (_G, _G)).T


def _ffn_chunks(F, n):
    nb = F // _G
    per = -(-nb // n)
    starts = [min(j * per, nb - per) if j == n - 1 else None for j in range(n)]
    step = (nb - per) // (n - 1)
    assert step * (n - 1) == nb - per and per - step <= per
    return per * _G, [j * step * _G for j in range(n)], (per - step) * _G


def _kernel(x_hbm, wqkv_hbm, wo_hbm, wr_hbm, wg_hbm, wu_hbm, wd_hbm, out_hbm,
            x_v, wq_v, wk_v, wv_v, wo_v, wr_v, gu_v, wd_v,
            sa_v, sb_v, xn_v, wqt_v, g_v, z_v, best_v, besti_v, zcol_v, xcol_v, hcol_v, y_v, m_v, out_v,
            sem_i, sem_o, sem_b, *, S, D, F):
    n_sub = S // _SUB
    n_cb = D // _CB
    n_groups = D // _G
    dh = D // _H
    n_it = n_sub // 2
    n_fc = n_it - 1
    fc, f_start, f_dup = _ffn_chunks(F, n_fc)
    hs = _SUB // 2

    cols = lambda c: pl.ds(c * _CB, _CB)
    dcols = pl.ds(0, D)

    def x_cp(a, b, s):
        sl = pl.ds(a * _SUB, (b - a) * _SUB)
        return pltpu.make_async_copy(x_hbm.at[sl, :], x_v.at[sl, :], sem_i.at[s])

    def k_cp(a, b, s):
        return pltpu.make_async_copy(wqkv_hbm.at[:, pl.ds(D + a * _CB, (b - a) * _CB)],
                                     wk_v.at[:, pl.ds(a * _CB, (b - a) * _CB)], sem_i.at[s])

    def gu_cps(j, s):
        src = pl.ds(f_start[j], fc)
        return [pltpu.make_async_copy(wg_hbm.at[:, src], gu_v.at[j, :, pl.ds(0, fc)], sem_i.at[s]),
                pltpu.make_async_copy(wu_hbm.at[:, src], gu_v.at[j, :, pl.ds(fc, fc)], sem_i.at[s])]

    def d_cp(j, s):
        return pltpu.make_async_copy(wd_hbm.at[pl.ds(f_start[j], fc), :], wd_v.at[j, :, dcols], sem_i.at[s])

    groups = [
        [pltpu.make_async_copy(wr_hbm, wr_v, sem_i.at[0]), x_cp(0, 1, 0)],
        [k_cp(0, 1, 1)],
        [k_cp(1, 2, 2)],
        [k_cp(2, n_cb, 3), x_cp(1, 2, 3)],
        [x_cp(2, 4, 4)],
        [x_cp(4, n_sub, 5)],
        [pltpu.make_async_copy(wqkv_hbm.at[:, pl.ds(0, D)], wq_v.at[:, dcols], sem_i.at[6]),
         pltpu.make_async_copy(wqkv_hbm.at[:, pl.ds(2 * D, D)], wv_v.at[:, dcols], sem_i.at[6]),
         pltpu.make_async_copy(wo_hbm, wo_v.at[:, dcols], sem_i.at[6])],
        gu_cps(0, 7) + [d_cp(0, 7)],
        sum([gu_cps(j, 8) + [d_cp(j, 8)] for j in range(1, n_fc)], []),
    ]

    def start(cps):
        for cp in cps:
            cp.start()
            pl.semaphore_signal(sem_b, 1)
            pl.semaphore_wait(sem_b, 1)

    def wait(name, cps):
        with _scope(name):
            for cp in cps:
                cp.wait()

    for grp in groups:
        start(grp)

    zero = pl.semaphore_read(sem_b)
    zero8 = pl.multiple_of(zero * 8, 8)
    zero_u = zero.astype(_U32)

    def zero_like(v):
        return pltpu.bitcast(pltpu.bitcast(v, _U32) & zero_u, _F32)

    def zero_link(v):
        d = pltpu.bitcast(v, _U32)
        d = pltpu.bitcast((d[:, :_G] | d[:, _G:]) & zero_u, _F32)
        return jnp.concatenate([d, d], axis=1)

    hcol_v[...] = jnp.zeros_like(hcol_v)
    y_v[...] = jnp.zeros_like(y_v)
    best_v[...] = jnp.full(best_v.shape, -jnp.inf, _F32)
    besti_v[...] = jnp.zeros_like(besti_v)

    wait("w_x0", groups[0])
    wr8 = wr_v[...].astype(_F32)
    wr = jnp.concatenate([wr8[g:g + 1, :] for g in range(n_groups)], axis=1)
    wr_sum = jnp.sum(wr, axis=-1, keepdims=True)
    sub_iota = jax.lax.broadcasted_iota(jnp.int32, (8, 1), 0)

    def ln_tile(tile, stage, chain_from=0, rows=_LNR, throttle=True):
        gsl = lambda g: slice(g * _G, (g + 1) * _G)
        best, besti = best_v[...], besti_v[...]
        for j in range(_SUB // rows):
            if isinstance(tile, int):
                r0 = tile * _SUB + j * rows
                h0 = r0 // 2
            else:
                r0 = pl.multiple_of(tile * _SUB + j * rows, rows)
                h0 = pl.multiple_of(tile * hs + j * (rows // 2), rows // 2)
            x = x_v[pl.ds(r0, rows), :].astype(_F32)

            def lane_partial(terms, dep):
                acc = terms[0] if dep is None else dep + terms[0]
                for t in terms[1:]:
                    acc = acc + t
                return acc

            dep = None
            if j >= chain_from:
                dep = pltpu.bitcast(stage[pl.ds(zero8, 8), pl.ds(0, _G)] & zero_u, _F32)
                dep = jnp.concatenate([dep] * (rows // 8), axis=0)
            s1 = lane_partial([x[:, gsl(g)] for g in range(n_groups)], dep)
            s2 = lane_partial([x[:, gsl(g)] * x[:, gsl(g)] for g in range(n_groups)],
                              zero_like(s1) if throttle else None)
            s3 = lane_partial([x[:, gsl(g)] * wr[:, gsl(g)] for g in range(n_groups)],
                              zero_like(s2) if throttle else None)
            m = jnp.sum(s1, axis=-1, keepdims=True) * (1.0 / D)
            ex2 = jnp.sum(s2, axis=-1, keepdims=True) * (1.0 / D)
            xw = jnp.sum(s3, axis=-1, keepdims=True)
            v = jnp.maximum(ex2 - m * m, 0.0)
            rstd = jax.lax.rsqrt(v + _LN_EPS)
            r = (xw - m * wr_sum) * rstd
            r = r.astype(_BF16).astype(_F32)
            rstd = jnp.where(r != r, r, rstd)
            for t in range(rows // 8):
                rt = r[t * 8:(t + 1) * 8, :]
                upd = rt > best
                best = jnp.where(upd, rt, best)
                besti = jnp.where(upd, sub_iota + (r0 + t * 8), besti)
            mb = jnp.broadcast_to(m, (rows, _G))
            for c in range(n_cb):
                xc = x_v[pl.ds(pl.multiple_of(r0 + zero * rows, rows), rows), cols(c)].astype(_F32)
                xn = _pack(((xc - jnp.concatenate([mb] * (_CB // _G), axis=1)) * rstd).astype(_BF16))
                stage[pl.ds(j * rows // 2, rows // 2), cols(c)] = xn
                xn_v[pl.ds(h0, rows // 2), cols(c)] = xn
                if throttle and c + 1 < n_cb:
                    d = pltpu.bitcast((xn[:, :_G] | xn[:, _G:]) & zero_u, _F32)
                    mb = mb + jnp.concatenate([d, d], axis=0)
        best_v[...] = best
        besti_v[...] = besti

    def k_job(stage, c, first=False):
        p = _phi(_dot(_unpack(stage[...]), wk_v[:, cols(c)]))
        zs = jnp.sum(p.reshape(_SUB // 8, 8, _CB), axis=0)
        if first:
            z_v[:, cols(c)] = zs
        else:
            z_v[:, cols(c)] += zs
        return p.astype(_BF16)

    def g_job(pk, stage, c, first=False):
        upd = _dot_tn(pk, _unpack(stage[...]))
        if first:
            g_v[cols(c), :] = upd
        else:
            g_v[cols(c), :] += upd

    ln_tile(0, sb_v, chain_from=_SUB, throttle=False)
    wait("w_k0", groups[1])
    p0 = k_job(sb_v, 0, True)
    wait("w_k1", groups[2])
    p1 = k_job(sb_v, 1, True)
    g_job(p0, sb_v, 0, True)
    g_job(p1, sb_v, 1, True)
    wait("w_k2x1", groups[3])
    ln_tile(1, sa_v, chain_from=1, rows=2 * _LNR)
    p2 = k_job(sb_v, 2, True)
    p3 = k_job(sb_v, 3, True)
    g_job(p2, sb_v, 2, True)
    g_job(p3, sb_v, 3, True)
    wait("w_x23", groups[4])

    def phase1(i, carry):
        @pl.when(i == 1)
        def _():
            wait("w_x47", groups[5])

        ln_tile(2 * i + 2, sb_v)
        seq = [(sa_v, c) for c in range(n_cb)] + [(sb_v, c) for c in range(n_cb)]
        pend = []
        for n, (stage, c) in enumerate(seq):
            pend.append((k_job(stage, c), stage, c))
            if n >= 1:
                g_job(*pend.pop(0))
            if n == n_cb:
                ln_tile(2 * i + 3, sa_v)
        g_job(*pend.pop(0))
        return carry

    jax.lax.fori_loop(0, (n_sub - 2) // 2, phase1, 0)
    wait("w_qvo", groups[6])

    best, besti = best_v[...], besti_v[...]
    rmax = jnp.max(best, axis=0, keepdims=True)
    idx = jnp.min(jnp.where(best == rmax, besti, S - 1))
    idx8 = pl.multiple_of((idx >> 4) * 8, 8)
    first_tile = idx // _SUB + 1
    gate_r = jax.nn.sigmoid(rmax)

    xs = _unpack(xn_v[pl.ds(idx8, 8), :]).astype(_F32)
    sel = jax.lax.broadcasted_iota(jnp.int32, (16, D), 0) == (idx & 15)
    xs = jnp.sum(jnp.where(sel, xs, 0.0), axis=0, keepdims=True)
    for g in range(n_groups):
        xcol_v[pl.ds(g * _G, _G), :] = _col_bcast(xs[:, g * _G:(g + 1) * _G])

    rr = jax.lax.broadcasted_iota(jnp.int32, (_G, _G), 0) // dh
    cc = jax.lax.broadcasted_iota(jnp.int32, (_G, _G), 1) // dh
    same_head = rr == cc

    for a in range(n_cb):
        for b in range(n_cb):
            wqt_v[pl.ds(b * _CB // 2, _CB // 2), cols(a)] = _pack(wq_v[cols(a), cols(b)].T)

    kvb = {}

    def kv_job(c):
        for g in range(c * _CB // _G, (c + 1) * _CB // _G):
            gs = pl.ds(g * _G, _G)
            kv = _dot(g_v[gs, :].astype(_BF16), wv_v[:, gs])
            kvb[g] = jnp.where(same_head, kv, 0.0).astype(_BF16)

    def m_job(c):
        for g in range(c * _CB // _G, (c + 1) * _CB // _G):
            m_v[pl.ds(g * _G // 2, _G // 2), :] = _pack(
                _dot(kvb.pop(g), wo_v[pl.ds(g * _G, _G), dcols]).astype(_BF16))

    pk = [k_job(sa_v, 0), k_job(sa_v, 1)]
    g_job(pk[0], sa_v, 0)
    pk.append(k_job(sa_v, 2))
    g_job(pk[1], sa_v, 1)
    pk.append(k_job(sa_v, 3))
    kv_job(0)
    g_job(pk[2], sa_v, 2)
    kv_job(1)
    m_job(0)
    g_job(pk[3], sa_v, 3)
    kv_job(2)
    m_job(1)
    kv_job(3)
    m_job(2)
    m_job(3)
    for g in range(n_groups):
        z = jnp.sum(z_v[:, pl.ds(g * _G, _G)], axis=0, keepdims=True)
        zcol_v[pl.ds(g * _G, _G), :] = _col_bcast(z)
    wait("w_f0", groups[7])

    def chain_matvec(w_ref, lead, cb, col_ref, acc0):
        n = col_ref.shape[0] // 8
        acc = [acc0[:, :_G], acc0[:, _G:]]
        link = None
        for k0 in range(0, n, _BLK):
            rows = pl.ds(k0 * 8, _BLK * 8)
            w = w_ref[lead, rows, cols(cb)].astype(_F32)
            colv = col_ref[rows, :]
            for h in range(2):
                prod = (w[:, h * _G:(h + 1) * _G] * colv).reshape(_BLK, 8, _G)
                first = acc[h] if link is None else acc[h] + link
                acc[h] = jnp.sum(jnp.concatenate([first[None], prod], axis=0), axis=0)
                link = zero_like(acc[h])
        return jnp.concatenate(acc, axis=1)

    def phase2(i, carry):
        @pl.when(i == 1)
        def _():
            wait("w_f1", groups[8])

        tiles = [(first_tile + 2 * i + t) & (n_sub - 1) for t in range(2)]
        row0 = [pl.multiple_of(t * _SUB, _SUB) for t in tiles]
        half0 = [pl.multiple_of(t * hs, hs) for t in tiles]

        dep = jnp.zeros((8, _CB), _F32)
        accs = []
        for f in range(2 * fc // _CB):
            accs.append(chain_matvec(gu_v, jnp.minimum(i, n_fc - 1), f, xcol_v, dep))
            dep = zero_link(accs[-1])
        gu = jnp.sum(jnp.concatenate(accs, axis=1), axis=0, keepdims=True)
        g, u = gu[:, :fc], gu[:, fc:]
        hnext = (g * jax.nn.sigmoid(g) * u).astype(_BF16).astype(_F32)
        lane = jax.lax.broadcasted_iota(jnp.int32, (1, fc), 1)
        hnext = jnp.where(lane < jnp.where(i > 0, f_dup, 0), 0.0, hnext)
        ys = []
        for c in range(n_cb):
            ys.append(chain_matvec(wd_v, jnp.maximum(i - 1, 0), c, hcol_v, y_v[:, cols(c)] + dep))
            dep = zero_link(ys[-1])
        yacc = jnp.concatenate([y + dep for y in ys], axis=1)
        y_v[...] = yacc
        yrow = jnp.sum(yacc, axis=0, keepdims=True) * gate_r

        ob = {}

        def q_job(t, c):
            xn = _unpack(xn_v[pl.ds(half0[t], hs), :])
            p = _phi(_dot_nt(_unpack(wqt_v[pl.ds(c * _CB // 2, _CB // 2), :]), xn))
            zc = zcol_v[cols(c), :]
            zc = jnp.concatenate([zc] * (_SUB // _G), axis=1)
            p3 = p.reshape(_CB // dh, dh, _SUB)
            den = jnp.sum(p3 * zc.reshape(_CB // dh, dh, _SUB), axis=1, keepdims=True) + _DEN_EPS
            o = (p3 * pl.reciprocal(den, approx=True)).reshape(_CB, _SUB).astype(_BF16)
            ob[t, c] = o.T

        n_h = fc // _G
        h_split = [range(0), range(0, n_h // 2), range(n_h // 2, n_h), range(0)]

        def out_job(t, c):
            if c == 0:
                ob[t] = jnp.concatenate([ob.pop((t, cb)) for cb in range(n_cb)], axis=1)
            rows = pl.ds(row0[t], _SUB)
            a = _dot(ob[t], _unpack(m_v[:, cols(c)]))
            res = x_v[rows, cols(c)].astype(_F32) + a + _unpack(xn_v[pl.ds(half0[t], hs), cols(c)]).astype(_F32)
            if t == 1:
                sel = jax.lax.broadcasted_iota(jnp.int32, (_SUB, _CB), 0) == (idx - row0[t])
                yc = yrow[:, c * _CB:(c + 1) * _CB]
                if len(h_split[c]):
                    for f in h_split[c]:
                        hcol_v[pl.ds(f * _G, _G), :] = _col_bcast(hnext[:, f * _G:(f + 1) * _G])
                    pin = zero_like(hcol_v[pl.ds(zero8, 1), :])
                    yc = yc + jnp.concatenate([pin] * (_CB // _G), axis=1)
                res = res + jnp.where(sel, yc, 0.0)
            out_v[rows, cols(c)] = res.astype(_BF16)
            if t == 1:
                pltpu.make_async_copy(out_v.at[rows, cols(c)], out_hbm.at[rows, cols(c)], sem_o).start()
            elif c == n_cb - 1:
                pltpu.make_async_copy(out_v.at[rows, :], out_hbm.at[rows, :], sem_o).start()

        for c in range(n_cb):
            q_job(0, c)
        for c in range(n_cb):
            q_job(1, c)
            out_job(0, c)
        for c in range(n_cb):
            out_job(1, c)
        return carry

    jax.lax.fori_loop(0, n_it, phase2, 0)
    wait("w_out", [pltpu.make_async_copy(out_v, out_hbm, sem_o)])


@jax.jit
def pallas_parallel_sum__linear_attn_block__moe_arch_mod__prompt_kernel(
    A_x: jax.Array,
    A_wqkv: jax.Array,
    A_wo: jax.Array,
    B_x: jax.Array,
    B_w_r: jax.Array,
    B_w_gate: jax.Array,
    B_w_up: jax.Array,
    B_w_down: jax.Array,
):
    del B_x
    B, S, D = A_x.shape
    assert B == 1
    F = B_w_gate.shape[1]
    n_fc = S // _SUB // 2 - 1
    fc = _ffn_chunks(F, n_fc)[0]
    any_spec = pl.BlockSpec(memory_space=pl.ANY)
    out = pl.pallas_call(
        functools.partial(_kernel, S=S, D=D, F=F),
        out_shape=jax.ShapeDtypeStruct((S, D), A_x.dtype),
        in_specs=[any_spec] * 7,
        out_specs=any_spec,
        scratch_shapes=[
            pltpu.VMEM((S, D), _BF16),
            pltpu.VMEM((D, D + _PAD), _BF16),
            pltpu.VMEM((D, D + _PAD), _BF16),
            pltpu.VMEM((D, D + _PAD), _BF16),
            pltpu.VMEM((D, D + _PAD), _BF16),
            pltpu.VMEM((D // _G, _G), _BF16),
            pltpu.VMEM((n_fc, D, 2 * fc), _BF16),
            pltpu.VMEM((n_fc, fc, D + _PAD), _BF16),
            pltpu.VMEM((_SUB // 2, D), _U32),
            pltpu.VMEM((_SUB // 2, D), _U32),
            pltpu.VMEM((S // 2, D), _U32),
            pltpu.VMEM((D // 2, D), _U32),
            pltpu.VMEM((D, D), _F32),
            pltpu.VMEM((8, D), _F32),
            pltpu.VMEM((8, 1), _F32),
            pltpu.VMEM((8, 1), jnp.int32),
            pltpu.VMEM((D, _G), _F32),
            pltpu.VMEM((D, _G), _F32),
            pltpu.VMEM((fc, _G), _F32),
            pltpu.VMEM((8, D), _F32),
            pltpu.VMEM((D // 2, D), _U32),
            pltpu.VMEM((S, D), _BF16),
            pltpu.SemaphoreType.DMA((9,)),
            pltpu.SemaphoreType.DMA,
            pltpu.SemaphoreType.REGULAR,
        ],
        compiler_params=pltpu.CompilerParams(
            vmem_limit_bytes=100 * 1024 * 1024,
            disable_bounds_checks=not _CHECKS,
            disable_semaphore_checks=not _CHECKS,
        ),
    )(A_x.reshape(S, D), A_wqkv, A_wo, B_w_r.reshape(D // _G, _G), B_w_gate, B_w_up, B_w_down)
    return out.reshape(B, S, D)
```

```python
import contextlib
import functools
import os

import jax
import jax.numpy as jnp
import jax.experimental.pallas as pl
import jax.experimental.pallas.tpu as pltpu

_H = 32
_LN_EPS = 1e-5
_PHI_EPS = 1e-6
_DEN_EPS = 1e-6
_SUB = 256
_CB = 256
_G = 128
_BLK = 16
_PAD = 128

_SCOPES = bool(os.environ.get("KSCOPES"))
_CHECKS = bool(os.environ.get("KCHECKS"))


def _scope(name):
    return jax.named_scope(name) if _SCOPES else contextlib.nullcontext()


_F32 = jnp.float32
_BF16 = jnp.bfloat16
_U32 = jnp.uint32


def _dot(a, b):
    return jnp.dot(a, b, preferred_element_type=_F32)


def _dot_tn(a, b):
    return jax.lax.dot_general(a, b, (((0,), (0,)), ((), ())), preferred_element_type=_F32)


def _dot_nt(a, b):
    return jax.lax.dot_general(a, b, (((1,), (1,)), ((), ())), preferred_element_type=_F32)


def _phi(t):
    return jnp.where(t > 0, t + 1.0, jnp.exp(t)) + _PHI_EPS


def _pack(v):
    return pltpu.bitcast(v, _U32)


def _unpack(v):
    return pltpu.bitcast(v, _BF16)


def _col_bcast(row):
    return jnp.broadcast_to(row, (_G, _G)).T


_A_IDX = (2, 3, 0, 1, 4, 5, 6)
_B_IDX = (2, 0, 6, 5, 1, 4, 3)


def _seven(a11, a12, a21, a22):
    return [a11, a22, a11 + a22, a21 + a22, a11 + a12, a21 - a11, a12 - a22]


def _strassen(prod, init=None):
    m1 = prod(0)
    m4 = prod(3)
    c11 = m1 + m4
    m2 = prod(1)
    c21 = m2 + m4
    c22 = m1 - m2
    m5 = prod(4)
    c11 = c11 - m5
    c11 = c11 + prod(6)
    m3 = prod(2)
    c12 = m3 + m5
    c22 = c22 + m3
    c22 = c22 + prod(5)
    out = (c11, c12, c21, c22)
    return out if init is None else tuple(a + b for a, b in zip(init, out))


def _ffn_chunks(F, n):
    nb = F // _G
    per = -(-nb // n)
    step = (nb - per) // (n - 1)
    assert step * (n - 1) == nb - per
    return per * _G, [j * step * _G for j in range(n)], (per - step) * _G


def _kernel(x_hbm, wqkv_hbm, wo_hbm, wr_hbm, wg_hbm, wu_hbm, wd_hbm, out_hbm,
            x_v, wq_v, wk_v, wv_v, wo_v, wr_v, gu_v, wd_v,
            sa_v, sb_v, xs_v, wks_v, wqt_v, wqs_v, gm_v, z_v, best_v, besti_v,
            zcol_v, xcol_v, hcol_v, y_v, ms_v, out_v,
            sem_i, sem_o, sem_b, *, S, D, F):
    n_sub = S // _SUB
    n_cb = D // _CB
    n_groups = D // _G
    dh = D // _H
    n_pair = n_sub // 2
    n_fc = n_pair - 1
    fc, f_start, f_dup = _ffn_chunks(F, n_fc)
    hs = _SUB // 2
    hd = D // 2
    n_sl = hd // _CB

    cols = lambda c: pl.ds(c * _CB, _CB)
    dcols = pl.ds(0, D)
    hcols = pl.ds(0, hd)
    gsl = lambda g: slice(g * _G, (g + 1) * _G)

    def x_cp(a, b, s):
        sl = pl.ds(int(a * _SUB), int((b - a) * _SUB))
        return pltpu.make_async_copy(x_hbm.at[sl, :], x_v.at[sl, :], sem_i.at[s])

    def k_cp(a, b, s):
        return pltpu.make_async_copy(wqkv_hbm.at[:, pl.ds(D + a * _CB, (b - a) * _CB)],
                                     wk_v.at[:, pl.ds(a * _CB, (b - a) * _CB)], sem_i.at[s])

    def gu_cps(j, s):
        src = pl.ds(f_start[j], fc)
        return [pltpu.make_async_copy(wg_hbm.at[:, src], gu_v.at[j, :, pl.ds(0, fc)], sem_i.at[s]),
                pltpu.make_async_copy(wu_hbm.at[:, src], gu_v.at[j, :, pl.ds(fc, fc)], sem_i.at[s])]

    def d_cp(j, s):
        return pltpu.make_async_copy(wd_hbm.at[pl.ds(f_start[j], fc), :], wd_v.at[j, :, dcols], sem_i.at[s])

    groups = dict(
        x0a=[x_cp(0, 0.5, 0)],
        k0=[k_cp(0, 1, 1)],
        x0b=[x_cp(0.5, 1, 2)],
        k1=[k_cp(1, 2, 3)],
        k2x1=[k_cp(2, n_cb, 4), x_cp(1, 2, 4)],
        x23=[x_cp(2, 4, 5), pltpu.make_async_copy(wr_hbm, wr_v, sem_i.at[5])],
        x45q=[x_cp(4, 6, 6),
              pltpu.make_async_copy(wqkv_hbm.at[:, pl.ds(0, D)], wq_v.at[:, dcols], sem_i.at[6])],
        x67=[x_cp(6, n_sub, 7)],
        vo=[pltpu.make_async_copy(wqkv_hbm.at[:, pl.ds(2 * D, D)], wv_v.at[:, dcols], sem_i.at[8]),
            pltpu.make_async_copy(wo_hbm, wo_v.at[:, dcols], sem_i.at[8])],
        f0=gu_cps(0, 9) + [d_cp(0, 9)],
        f1=sum([gu_cps(j, 10) + [d_cp(j, 10)] for j in range(1, n_fc)], []),
    )

    for grp in groups.values():
        for cp in grp:
            cp.start()
            pl.semaphore_signal(sem_b, 1)
            pl.semaphore_wait(sem_b, 1)

    def wait(name):
        with _scope("w_" + name):
            for cp in groups[name]:
                cp.wait()

    zero = pl.semaphore_read(sem_b)
    zero8 = pl.multiple_of(zero * 8, 8)
    zero_u = zero.astype(_U32)

    def zero_of_bits(u):
        return pltpu.bitcast(u & zero_u, _F32)

    def zero_like(v):
        return zero_of_bits(pltpu.bitcast(v, _U32))

    def zero_link(v):
        d = pltpu.bitcast(v, _U32)
        d = zero_of_bits(d[:, :_G] | d[:, _G:])
        return jnp.concatenate([d, d], axis=1)

    def rep(d, n):
        return jnp.concatenate([d] * n, axis=0)

    hcol_v[...] = jnp.zeros_like(hcol_v)
    y_v[...] = jnp.zeros_like(y_v)
    best_v[...] = jnp.full(best_v.shape, -jnp.inf, _F32)
    besti_v[...] = jnp.zeros_like(besti_v)

    def lane_partial(terms, dep):
        acc = terms[0] if dep is None else dep + terms[0]
        for t in terms[1:]:
            acc = acc + t
        return acc

    def ln_stats(x, dep, throttle, wr=None):
        s1 = lane_partial([x[:, gsl(g)] for g in range(n_groups)], dep)
        s2 = lane_partial([x[:, gsl(g)] * x[:, gsl(g)] for g in range(n_groups)],
                          zero_like(s1) if throttle else None)
        m = jnp.sum(s1, axis=-1, keepdims=True) * (1.0 / D)
        ex2 = jnp.sum(s2, axis=-1, keepdims=True) * (1.0 / D)
        rstd = jax.lax.rsqrt(jnp.maximum(ex2 - m * m, 0.0) + _LN_EPS)
        if wr is None:
            return m, rstd, None
        s3 = lane_partial([x[:, gsl(g)] * wr[0][:, gsl(g)] for g in range(n_groups)], zero_like(s2))
        r = (jnp.sum(s3, axis=-1, keepdims=True) - m * wr[1]) * rstd
        r = r.astype(_BF16).astype(_F32)
        rstd = jnp.where(r != r, r, rstd)
        return m, rstd, r

    def ln_plain(row0, n_rows, stage, rows, throttle):
        for j in range(n_rows // rows):
            r0 = row0 + j * rows
            s0 = (r0 % _SUB) // 2
            x = x_v[pl.ds(r0, rows), :].astype(_F32)
            dep = None
            if throttle and j > 0:
                dep = rep(zero_of_bits(stage[pl.ds(zero8, 8), pl.ds(0, _G)]), rows // 8)
            m, rstd, _ = ln_stats(x, dep, throttle)
            mb = jnp.broadcast_to(m, (rows, _G))
            for c in range(n_cb):
                xc = x_v[pl.ds(pl.multiple_of(r0 + zero * rows, rows), rows), cols(c)].astype(_F32)
                xn = _pack(((xc - jnp.concatenate([mb] * (_CB // _G), axis=1)) * rstd).astype(_BF16))
                stage[pl.ds(s0, rows // 2), cols(c)] = xn
                if throttle and c + 1 < n_cb:
                    mb = mb + rep(zero_of_bits(xn[:, :_G] | xn[:, _G:]), 2)

    sub_iota = jax.lax.broadcasted_iota(jnp.int32, (8, 1), 0)

    def ln_pair(pair, dst, dep):
        wr8 = wr_v[...].astype(_F32)
        wr = jnp.concatenate([wr8[g:g + 1, :] for g in range(n_groups)], axis=1)
        wr = (wr, jnp.sum(wr, axis=-1, keepdims=True))
        best, besti = best_v[...], besti_v[...]
        for j in range(_SUB // 16):
            r0 = [pl.multiple_of(pair * (2 * _SUB) + t * _SUB + j * 16, 16) for t in range(2)]
            x = jnp.concatenate([x_v[pl.ds(r, 16), :] for r in r0], axis=0).astype(_F32)
            if j > 0:
                dep = zero_of_bits(dst[0, pl.ds(zero8, 8), pl.ds(0, _G)])
            m, rstd, r = ln_stats(x, rep(dep, 4), True, wr)
            for t in range(4):
                rt = r[t * 8:(t + 1) * 8, :]
                row = sub_iota + (r0[t // 2] + (t % 2) * 8)
                upd = (rt > best) | ((rt == best) & (row < besti))
                best = jnp.where(upd, rt, best)
                besti = jnp.where(upd, row, besti)
            mb = jnp.broadcast_to(m, (32, _G))
            for g in range(hd // _G):
                blk = []
                for h in range(2):
                    csl = pl.ds(h * hd + g * _G, _G)
                    xc = jnp.concatenate([x_v[pl.ds(pl.multiple_of(r + zero * 16, 16), 16), csl] for r in r0], axis=0)
                    blk.append((xc.astype(_F32) - mb) * rstd)
                x11, x21, x12, x22 = blk[0][:16], blk[0][16:], blk[1][:16], blk[1][16:]
                nine = [_pack(v.astype(_BF16)) for v in _seven(x11, x12, x21, x22) + [x12, x21]]
                for b, v in enumerate(nine):
                    dst[b, pl.ds(j * 8, 8), pl.ds(g * _G, _G)] = v
                if g + 1 < hd // _G:
                    mb = mb + rep(zero_of_bits((nine[2] | nine[3]) | (nine[4] | nine[5])), 4)
        best_v[...] = best
        besti_v[...] = besti

    def seven_rows(load, dst, dst_row, n_units, dep):
        for j in range(n_units):
            for g in range(hd // _G):
                w = [load(a, b, j, g).astype(_F32) for a in range(2) for b in range(2)]
                w[0] = w[0] + rep(dep, 2)
                for b, v in enumerate(_seven(*w)):
                    dst[b, pl.ds(dst_row + j * 8, 8), pl.ds(g * _G, _G)] = _pack(v.astype(_BF16))
                dep = zero_of_bits(dst[0, pl.ds(dst_row + zero8, 8), pl.ds(0, _G)])
        return dep

    g_home = {(0, 0): 6, (0, 1): 2, (1, 0): 1, (1, 1): 5}

    def staged(stage, part):
        return _unpack(stage[...] if part is None else stage[pl.ds(part * hs // 2, hs // 2), :])

    def k_job(stage, c, first=False, part=None):
        p = _phi(_dot(staged(stage, part), wk_v[:, cols(c)]))
        zs = jnp.sum(p.reshape(p.shape[0] // 8, 8, _CB), axis=0)
        if first:
            z_v[:, cols(c)] = zs
        else:
            z_v[:, cols(c)] += zs
        return p.astype(_BF16)

    def g_job(pk, stage, c, first=False, part=None):
        upd = _dot_tn(pk, staged(stage, part))
        a, j = divmod(c, n_sl)
        for b in range(2):
            if first:
                gm_v[g_home[a, b], cols(j), :] = upd[:, b * hd:(b + 1) * hd]
            else:
                gm_v[g_home[a, b], cols(j), :] += upd[:, b * hd:(b + 1) * hd]

    def wk_load(j0):
        return lambda a, b, j, g: wk_v[pl.ds(a * hd + (j0 + j) * 16, 16), pl.ds(b * hd + g * _G, _G)]

    n_wu = hd // 16
    zero_v = jnp.zeros((8, _G), _F32)
    wait("x0a")
    ln_plain(0, _SUB // 2, sb_v, 16, False)
    wait("k0")
    p0a = k_job(sb_v, 0, True, part=0)
    wait("x0b")
    ln_plain(_SUB // 2, _SUB // 2, sb_v, 16, False)
    g_job(p0a, sb_v, 0, True, part=0)
    p0b = k_job(sb_v, 0, part=1)
    wait("k1")
    for m in (0, 3, 4):
        gm_v[m] = jnp.zeros(gm_v.shape[1:], _F32)
    p1 = k_job(sb_v, 1, True)
    g_job(p0b, sb_v, 0, part=1)
    g_job(p1, sb_v, 1, True)
    wait("k2x1")
    ln_plain(_SUB, _SUB, sa_v, 32, True)
    seven_rows(wk_load(0), wks_v, 0, n_wu // 2, zero_of_bits(sa_v[pl.ds(zero8, 8), pl.ds(0, _G)]))
    p2 = k_job(sb_v, 2, True)
    p3 = k_job(sb_v, 3, True)
    g_job(p2, sb_v, 2, True)
    g_job(p3, sb_v, 3, True)
    wait("x23")
    dep = seven_rows(wk_load(n_wu // 2), wks_v, n_wu // 2 * 8, n_wu // 2, zero_v)
    ln_pair(1, xs_v.at[0], dep)
    pk = [k_job(sa_v, 0), k_job(sa_v, 2)]
    g_job(pk[0], sa_v, 0)
    pk.append(k_job(sa_v, 1))
    g_job(pk[1], sa_v, 2)
    gm_v[5, cols(0), :] += gm_v[1, cols(0), :] - gm_v[2, cols(0), :]
    pk.append(k_job(sa_v, 3))
    g_job(pk[2], sa_v, 1)
    g_job(pk[3], sa_v, 3)
    gm_v[5, cols(1), :] += gm_v[1, cols(1), :] - gm_v[2, cols(1), :]
    wait("x45q")

    def phase1(i, carry):
        @pl.when(i == 1)
        def _():
            wait("x67")

        win = xs_v.at[pl.ds(i, 2)]
        cur = lambda b: _unpack(win[0, b, :, hcols])

        dep = zero_v
        for u in range(2):
            s = jnp.minimum(2 * i + u, hd // _G - 1)
            for b in range(2):
                f0 = pl.multiple_of(b * hd + s * _G, _G)
                for c in range(n_cb):
                    wqt_v[u, b, :, cols(c)] = _pack(wq_v[cols(c), pl.ds(f0, _G)].T)
            load = lambda a, b, j, g, u=u: _unpack(
                wqt_v[u, b, pl.ds(pl.multiple_of(j * 8 + zero8, 8), 8), pl.ds(a * hd + g * _G, _G)])
            dep = seven_rows(load, wqs_v, pl.multiple_of(s * (_G // 2), _G // 2), _G // 16, dep)
        ln_pair((i + 2) & (n_pair - 1), win.at[1], dep)

        def ks_job(j):
            c = map(_phi, _strassen(lambda m: _dot(cur(_A_IDX[m]), _unpack(wks_v[_B_IDX[m], :, cols(j)]))))
            p11, p12, p21, p22 = c
            z_v[:, cols(j)] += jnp.sum((p11 + p21).reshape(_SUB // 8, 8, _CB), axis=0)
            z_v[:, cols(n_sl + j)] += jnp.sum((p12 + p22).reshape(_SUB // 8, 8, _CB), axis=0)
            return [v.astype(_BF16) for v in _seven(p11, p21, p12, p22)]

        ps = [ks_job(j) for j in range(n_sl)]
        for j in range(n_sl):
            for m in range(7):
                gm_v[m, cols(j), :] += _dot_tn(ps[j][_A_IDX[m]], cur(_B_IDX[m]))
        return carry

    jax.lax.fori_loop(0, n_pair - 1, phase1, 0)
    wait("vo")

    best, besti = best_v[...], besti_v[...]
    rmax = jnp.max(best, axis=0, keepdims=True)
    idx = jnp.min(jnp.where(best == rmax, besti, S - 1))
    idx_pair = idx // (2 * _SUB)
    gate_r = jax.nn.sigmoid(rmax)

    in_b = (idx // _SUB) & 1
    slot = (idx_pair + n_pair - 1) & (n_pair - 1)
    prow = pl.ds(pl.multiple_of(((idx & (_SUB - 1)) >> 4) * 8, 8), 8)
    sel = jax.lax.broadcasted_iota(jnp.int32, (16, hd), 0) == (idx & 15)
    for h, (ba, bb) in enumerate(((0, 8), (7, 1))):
        xs = _unpack(xs_v[slot, jnp.where(in_b == 1, bb, ba), prow, hcols]).astype(_F32)
        xs = jnp.sum(jnp.where(sel, xs, 0.0), axis=0, keepdims=True)
        for g in range(hd // _G):
            xcol_v[pl.ds(h * hd + g * _G, _G), :] = _col_bcast(xs[:, gsl(g)])
    for g in range(n_groups):
        z = jnp.sum(z_v[:, pl.ds(g * _G, _G)], axis=0, keepdims=True)
        zcol_v[pl.ds(g * _G, _G), :] = _col_bcast(z)

    rr = jax.lax.broadcasted_iota(jnp.int32, (_G, _G), 0) // dh
    cc = jax.lax.broadcasted_iota(jnp.int32, (_G, _G), 1) // dh
    same_head = rr == cc
    n_hg = hd // _G
    kvb = {}

    def kv_job(g):
        gm = lambda m: gm_v[m, pl.ds((g % n_hg) * _G, _G), :]
        if g < n_hg:
            row = [gm(0) + gm(3) - gm(4) + gm(6), gm(2) + gm(4)]
        else:
            row = [gm(1) + gm(3), gm(0) - gm(1) + gm(2) + gm(5)]
        kv = _dot(jnp.concatenate(row, axis=1).astype(_BF16), wv_v[:, pl.ds(g * _G, _G)])
        kvb[g] = jnp.where(same_head, kv, 0.0).astype(_BF16)

    def m_job(g):
        top, bot = [_dot(kvb.pop(q), wo_v[pl.ds(q * _G, _G), dcols]) for q in (g, g + n_hg)]
        for b, v in enumerate(_seven(top[:, :hd], top[:, hd:], bot[:, :hd], bot[:, hd:])):
            ms_v[b, pl.ds(g * _G // 2, _G // 2), :] = _pack(v.astype(_BF16))

    for g in range(n_hg):
        kv_job(g)
        kv_job(g + n_hg)
        if g > 0:
            m_job(g - 1)
    m_job(n_hg - 1)
    wait("f0")

    def chain_matvec(w_ref, lead, cb, col_ref, acc0):
        n = col_ref.shape[0] // 8
        acc = [acc0[:, :_G], acc0[:, _G:]]
        link = None
        for k0 in range(0, n, _BLK):
            rows = pl.ds(k0 * 8, _BLK * 8)
            w = w_ref[lead, rows, cols(cb)].astype(_F32)
            colv = col_ref[rows, :]
            for h in range(2):
                prod = (w[:, h * _G:(h + 1) * _G] * colv).reshape(_BLK, 8, _G)
                first = acc[h] if link is None else acc[h] + link
                acc[h] = jnp.sum(jnp.concatenate([first[None], prod], axis=0), axis=0)
                link = zero_like(acc[h])
        return jnp.concatenate(acc, axis=1)

    def phase2(i, carry):
        @pl.when(i == 1)
        def _():
            wait("f1")

        slot = (idx_pair + i) & (n_pair - 1)
        pair = (slot + 1) & (n_pair - 1)
        row0 = [pl.multiple_of(pair * (2 * _SUB) + t * _SUB, _SUB) for t in range(2)]
        win = xs_v.at[slot]
        cur = lambda b: _unpack(win[b, :, hcols])

        dep = jnp.zeros((8, _CB), _F32)
        ys = []
        for c in range(n_cb):
            ys.append(chain_matvec(wd_v, jnp.maximum(i - 1, 0), c, hcol_v, y_v[:, cols(c)] + dep))
            dep = zero_link(ys[-1])
        yacc = jnp.concatenate(ys, axis=1)
        y_v[...] = yacc
        yrow = jnp.sum(yacc, axis=0, keepdims=True) * gate_r
        accs = []
        for f in range(2 * fc // _CB):
            accs.append(chain_matvec(gu_v, jnp.minimum(i, n_fc - 1), f, xcol_v, dep))
            dep = zero_link(accs[-1])
        gu = jnp.sum(jnp.concatenate([a + dep for a in accs], axis=1), axis=0, keepdims=True)
        g, u = gu[:, :fc], gu[:, fc:]
        hnext = (g * jax.nn.sigmoid(g) * u).astype(_BF16).astype(_F32)
        lane = jax.lax.broadcasted_iota(jnp.int32, (1, fc), 1)
        hnext = jnp.where(lane < jnp.where(i > 0, f_dup, 0), 0.0, hnext)

        def normalise(p, c):
            zc = jnp.concatenate([zcol_v[cols(c), :]] * (_SUB // _G), axis=1)
            p3 = p.reshape(_CB // dh, dh, _SUB)
            den = jnp.sum(p3 * zc.reshape(_CB // dh, dh, _SUB), axis=1, keepdims=True) + _DEN_EPS
            return (p3 * pl.reciprocal(den, approx=True)).reshape(_CB, _SUB)

        def qs_job(j):
            lhs = lambda m: _unpack(wqs_v[_B_IDX[m], pl.ds(j * _CB // 2, _CB // 2), :])
            p11, p12, p21, p22 = map(_phi, _strassen(lambda m: _dot_nt(lhs(m), cur(_A_IDX[m]))))
            o = [normalise(p11, j), normalise(p12, n_sl + j), normalise(p21, j), normalise(p22, n_sl + j)]
            return [v.astype(_BF16).T for v in _seven(*o)]

        n_h = fc // _G
        raw = {(0, 0): 0, (0, 1): 7, (1, 0): 8, (1, 1): 1}

        def finish(cs, j, h_parts):
            order = (2, 0, 1, 3)
            for n, q in enumerate(order):
                t, b = divmod(q, 2)
                c = b * n_sl + j
                rows = pl.ds(row0[t], _SUB)
                res = x_v[rows, cols(c)].astype(_F32) + cs[q] + _unpack(win[raw[t, b], :, cols(j)]).astype(_F32)
                yc = yrow[:, c * _CB:(c + 1) * _CB]
                if len(h_parts[n]):
                    for f in h_parts[n]:
                        hcol_v[pl.ds(f * _G, _G), :] = _col_bcast(hnext[:, gsl(f)])
                    pin = zero_like(hcol_v[pl.ds(zero8, 1), :])
                    yc = yc + jnp.concatenate([pin] * (_CB // _G), axis=1)
                sel = jax.lax.broadcasted_iota(jnp.int32, (_SUB, _CB), 0) == (idx - row0[t])
                out_v[rows, cols(c)] = (res + jnp.where(sel, yc, 0.0)).astype(_BF16)
                pltpu.make_async_copy(out_v.at[rows, cols(c)], out_hbm.at[rows, cols(c)], sem_o).start()

        os_ = [qs_job(j) for j in range(n_sl)]
        ms = lambda m, k, j: _unpack(ms_v[_B_IDX[m], pl.ds(k * _CB // 2, _CB // 2), cols(j)])
        cs = None
        for k in range(n_sl):
            cs = _strassen(lambda m: _dot(os_[k][_A_IDX[m]], ms(m, k, 0)), cs)
        finish(cs, 0, [range(0)] * 4)
        full = [jnp.concatenate([os_[k][b] for k in range(n_sl)], axis=1) for b in range(7)]
        for j in range(1, n_sl):
            cs = _strassen(lambda m: _dot(full[_A_IDX[m]], _unpack(ms_v[_B_IDX[m], :, cols(j)])))
            finish(cs, j, [range(0), range(0, n_h // 2), range(n_h // 2, n_h), range(0)])
        return carry

    jax.lax.fori_loop(0, n_pair, phase2, 0)
    with _scope("w_out"):
        pltpu.make_async_copy(out_v, out_hbm, sem_o).wait()


@jax.jit
def pallas_parallel_sum__linear_attn_block__moe_arch_mod__prompt_kernel(
    A_x: jax.Array,
    A_wqkv: jax.Array,
    A_wo: jax.Array,
    B_x: jax.Array,
    B_w_r: jax.Array,
    B_w_gate: jax.Array,
    B_w_up: jax.Array,
    B_w_down: jax.Array,
):
    del B_x
    B, S, D = A_x.shape
    assert B == 1
    F = B_w_gate.shape[1]
    n_pair = S // _SUB // 2
    n_fc = n_pair - 1
    fc = _ffn_chunks(F, n_fc)[0]
    hd = D // 2
    any_spec = pl.BlockSpec(memory_space=pl.ANY)
    out = pl.pallas_call(
        functools.partial(_kernel, S=S, D=D, F=F),
        out_shape=jax.ShapeDtypeStruct((S, D), A_x.dtype),
        in_specs=[any_spec] * 7,
        out_specs=any_spec,
        scratch_shapes=[
            pltpu.VMEM((S, D), _BF16),
            pltpu.VMEM((D, D + _PAD), _BF16),
            pltpu.VMEM((D, D + _PAD), _BF16),
            pltpu.VMEM((D, D + _PAD), _BF16),
            pltpu.VMEM((D, D + _PAD), _BF16),
            pltpu.VMEM((D // _G, _G), _BF16),
            pltpu.VMEM((n_fc, D, 2 * fc), _BF16),
            pltpu.VMEM((n_fc, fc, D + _PAD), _BF16),
            pltpu.VMEM((_SUB // 2, D), _U32),
            pltpu.VMEM((_SUB // 2, D), _U32),
            pltpu.VMEM((n_pair, 9, _SUB // 2, hd + _PAD), _U32),
            pltpu.VMEM((7, hd // 2, hd), _U32),
            pltpu.VMEM((2, 2, _G // 2, D), _U32),
            pltpu.VMEM((7, hd // 2, hd), _U32),
            pltpu.VMEM((7, hd, hd), _F32),
            pltpu.VMEM((8, D), _F32),
            pltpu.VMEM((8, 1), _F32),
            pltpu.VMEM((8, 1), jnp.int32),
            pltpu.VMEM((D, _G), _F32),
            pltpu.VMEM((D, _G), _F32),
            pltpu.VMEM((fc, _G), _F32),
            pltpu.VMEM((8, D), _F32),
            pltpu.VMEM((7, hd // 2, hd), _U32),
            pltpu.VMEM((S, D), _BF16),
            pltpu.SemaphoreType.DMA((11,)),
            pltpu.SemaphoreType.DMA,
            pltpu.SemaphoreType.REGULAR,
        ],
        compiler_params=pltpu.CompilerParams(
            vmem_limit_bytes=110 * 1024 * 1024,
            disable_bounds_checks=not _CHECKS,
            disable_semaphore_checks=not _CHECKS,
        ),
    )(A_x.reshape(S, D), A_wqkv, A_wo, B_w_r.reshape(D // _G, _G), B_w_gate, B_w_up, B_w_down)
    return out.reshape(B, S, D)
```

```python
import contextlib
import functools
import os

import jax
import jax.numpy as jnp
import jax.experimental.pallas as pl
import jax.experimental.pallas.tpu as pltpu

_H = 32
_LN_EPS = 1e-5
_PHI_EPS = 1e-6
_DEN_EPS = 1e-6
_SUB = 256
_CB = 256
_G = 128
_BLK = 16
_PAD = 128

_PINM = tuple(int(v) for v in os.environ.get('PINM', '4,4').split(','))
_SCOPES = bool(os.environ.get("KSCOPES"))
_CHECKS = bool(os.environ.get("KCHECKS"))


def _scope(name):
    return jax.named_scope(name) if _SCOPES else contextlib.nullcontext()


_F32 = jnp.float32
_BF16 = jnp.bfloat16
_U32 = jnp.uint32


def _dot(a, b):
    return jnp.dot(a, b, preferred_element_type=_F32)


def _dot_tn(a, b):
    return jax.lax.dot_general(a, b, (((0,), (0,)), ((), ())), preferred_element_type=_F32)


def _dot_nt(a, b):
    return jax.lax.dot_general(a, b, (((1,), (1,)), ((), ())), preferred_element_type=_F32)


def _phi(t):
    return jnp.where(t > 0, t + 1.0, jnp.exp(t)) + _PHI_EPS


def _pack(v):
    return pltpu.bitcast(v, _U32)


def _unpack(v):
    return pltpu.bitcast(v, _BF16)


def _col_bcast(row):
    return jnp.broadcast_to(row, (_G, _G)).T


_A_IDX = (2, 3, 0, 1, 4, 5, 6)
_B_IDX = (2, 0, 6, 5, 1, 4, 3)


def _seven(a11, a12, a21, a22):
    return [a11, a22, a11 + a22, a21 + a22, a11 + a12, a21 - a11, a12 - a22]


_SEVEN = (
    lambda a: a[0, 0],
    lambda a: a[1, 1],
    lambda a: a[0, 0] + a[1, 1],
    lambda a: a[1, 0] + a[1, 1],
    lambda a: a[0, 0] + a[0, 1],
    lambda a: a[1, 0] - a[0, 0],
    lambda a: a[0, 1] - a[1, 1],
)
_STAGES = ((((0, 0),), (0,)), (((1, 1),), (1, 2)), (((0, 1),), (4, 6)), (((1, 0),), (3, 5)))


def _strassen(prod):
    m1 = prod(0)
    m4 = prod(3)
    c11 = m1 + m4
    m2 = prod(1)
    c21 = m2 + m4
    c22 = m1 - m2
    m5 = prod(4)
    c11 = c11 - m5
    c11 = c11 + prod(6)
    m3 = prod(2)
    c12 = m3 + m5
    c22 = c22 + m3
    c22 = c22 + prod(5)
    return c11, c12, c21, c22


def _strassen_late22(prod):
    m6 = prod(5)
    m3 = prod(2)
    c22 = m6 + m3
    m5 = prod(4)
    c12 = m3 + m5
    m1 = prod(0)
    c11 = m1 - m5
    c22 = c22 + m1
    m2 = prod(1)
    c22 = c22 - m2
    m4 = prod(3)
    c21 = m2 + m4
    c11 = c11 + m4
    c11 = c11 + prod(6)
    return c11, c12, c21, c22


def _ffn_chunks(F, n):
    nb = F // _G
    per = -(-nb // n)
    step = (nb - per) // (n - 1)
    assert step * (n - 1) == nb - per
    return per * _G, [j * step * _G for j in range(n)], (per - step) * _G


def _kernel(x_hbm, wqkv_hbm, wo_hbm, wr_hbm, wg_hbm, wu_hbm, wd_hbm, out_hbm,
            x_v, wq_v, wk_v, wv_v, wo_v, wr_v, gu_v, wd_v,
            sa_v, sb_v, xs_v, res_v, wks_v, wqt_v, wqs_v, gm_v, z_v, best_v, besti_v,
            zcol_v, xcol_v, hcol_v, y_v, tr_v, ms_v, out_v,
            sem_i, sem_o, sem_b, *, S, D, F):
    n_sub = S // _SUB
    n_cb = D // _CB
    n_groups = D // _G
    dh = D // _H
    n_pair = n_sub // 2
    n_fc = n_pair - 1
    fc, f_start, f_dup = _ffn_chunks(F, n_fc)
    hs = _SUB // 2
    hd = D // 2
    n_sl = hd // _CB

    cols = lambda c: pl.ds(c * _CB, _CB)
    dcols = pl.ds(0, D)
    hcols = pl.ds(0, hd)
    gsl = lambda g: slice(g * _G, (g + 1) * _G)

    def x_cp(a, b, s):
        sl = pl.ds(int(a * _SUB), int((b - a) * _SUB))
        return pltpu.make_async_copy(x_hbm.at[sl, :], x_v.at[sl, :], sem_i.at[s])

    def k_cp(a, b, s):
        return pltpu.make_async_copy(wqkv_hbm.at[:, pl.ds(D + a * _CB, (b - a) * _CB)],
                                     wk_v.at[:, pl.ds(a * _CB, (b - a) * _CB)], sem_i.at[s])

    def gu_cps(j, s):
        src = pl.ds(f_start[j], fc)
        return [pltpu.make_async_copy(wg_hbm.at[:, src], gu_v.at[j, :, pl.ds(0, fc)], sem_i.at[s]),
                pltpu.make_async_copy(wu_hbm.at[:, src], gu_v.at[j, :, pl.ds(fc, fc)], sem_i.at[s])]

    def d_cp(j, s):
        return pltpu.make_async_copy(wd_hbm.at[pl.ds(f_start[j], fc), :], wd_v.at[j, :, dcols], sem_i.at[s])

    groups = dict(
        x0a=[x_cp(0, 0.5, 0)],
        k0=[k_cp(0, 1, 1)],
        x0b=[x_cp(0.5, 1, 2)],
        k1=[k_cp(1, 2, 3)],
        k2x1=[k_cp(2, n_cb, 4), x_cp(1, 2, 4)],
        x23=[x_cp(2, 4, 5), pltpu.make_async_copy(wr_hbm, wr_v, sem_i.at[5])],
        x45q=[x_cp(4, 6, 6),
              pltpu.make_async_copy(wqkv_hbm.at[:, pl.ds(0, D)], wq_v.at[:, dcols], sem_i.at[6])],
        x67=[x_cp(6, n_sub, 7)],
        vo=[pltpu.make_async_copy(wqkv_hbm.at[:, pl.ds(2 * D, D)], wv_v.at[:, dcols], sem_i.at[8]),
            pltpu.make_async_copy(wo_hbm, wo_v.at[:, dcols], sem_i.at[8])],
        f0=gu_cps(0, 9) + [d_cp(0, 9)],
        f1=sum([gu_cps(j, 10) + [d_cp(j, 10)] for j in range(1, n_fc)], []),
    )

    for grp in groups.values():
        for cp in grp:
            cp.start()
            pl.semaphore_signal(sem_b, 1)
            pl.semaphore_wait(sem_b, 1)

    def wait(name):
        with _scope("w_" + name):
            for cp in groups[name]:
                cp.wait()

    zero = pl.semaphore_read(sem_b)
    zero8 = pl.multiple_of(zero * 8, 8)
    zero_u = zero.astype(_U32)

    def zero_of_bits(u):
        return pltpu.bitcast(u & zero_u, _F32)

    def zero_like(v):
        return zero_of_bits(pltpu.bitcast(v, _U32))

    def zero_link(v):
        d = pltpu.bitcast(v, _U32)
        d = zero_of_bits(d[:, :_G] | d[:, _G:])
        return jnp.concatenate([d, d], axis=1)

    def rep(d, n):
        return jnp.concatenate([d] * n, axis=0)

    hcol_v[...] = jnp.zeros_like(hcol_v)
    y_v[...] = jnp.zeros_like(y_v)
    best_v[...] = jnp.full(best_v.shape, -jnp.inf, _F32)
    besti_v[...] = jnp.zeros_like(besti_v)

    def lane_partial(terms, dep):
        acc = terms[0] if dep is None else dep + terms[0]
        for t in terms[1:]:
            acc = acc + t
        return acc

    def ln_stats(x, dep, throttle, wr=None):
        s1 = lane_partial([x[:, gsl(g)] for g in range(n_groups)], dep)
        s2 = lane_partial([x[:, gsl(g)] * x[:, gsl(g)] for g in range(n_groups)],
                          zero_like(s1) if throttle else None)
        m = jnp.sum(s1, axis=-1, keepdims=True) * (1.0 / D)
        ex2 = jnp.sum(s2, axis=-1, keepdims=True) * (1.0 / D)
        rstd = jax.lax.rsqrt(jnp.maximum(ex2 - m * m, 0.0) + _LN_EPS)
        if wr is None:
            return m, rstd
        s3 = lane_partial([x[:, gsl(g)] * wr[0][:, gsl(g)] for g in range(n_groups)], zero_like(s2))
        r = (jnp.sum(s3, axis=-1, keepdims=True) - m * wr[1]) * rstd
        r = r.astype(_BF16).astype(_F32)
        rstd = jnp.where(r != r, r, rstd)
        return m, rstd, r, zero_like(s3)

    def ln_plain(row0, n_rows, stage, rows, throttle):
        for j in range(n_rows // rows):
            r0 = row0 + j * rows
            s0 = (r0 % _SUB) // 2
            x = x_v[pl.ds(r0, rows), :].astype(_F32)
            dep = None
            if throttle and j > 0:
                dep = rep(zero_of_bits(stage[pl.ds(zero8, 8), pl.ds(0, _G)]), rows // 8)
            m, rstd = ln_stats(x, dep, throttle)
            mb = jnp.broadcast_to(m, (rows, _G))
            for c in range(n_cb):
                xc = x_v[pl.ds(pl.multiple_of(r0 + zero * rows, rows), rows), cols(c)].astype(_F32)
                xn = _pack(((xc - jnp.concatenate([mb] * (_CB // _G), axis=1)) * rstd).astype(_BF16))
                stage[pl.ds(s0, rows // 2), cols(c)] = xn
                if throttle and c + 1 < n_cb:
                    mb = mb + rep(zero_of_bits(stage[pl.ds(zero8, 8), pl.ds(0, _G)]), rows // 8)

    sub_iota = jax.lax.broadcasted_iota(jnp.int32, (8, 1), 0)

    def ln_pair(pair, dst, dep):
        wr8 = wr_v[...].astype(_F32)
        wr = jnp.concatenate([wr8[g:g + 1, :] for g in range(n_groups)], axis=1)
        wr = (wr, jnp.sum(wr, axis=-1, keepdims=True))
        best, besti = best_v[...], besti_v[...]
        n_u = _SUB // 16
        r0 = [[pl.multiple_of(pair * (2 * _SUB) + t * _SUB + j * 16, 16) for t in range(2)] for j in range(n_u)]
        st = {}
        for j in range(-1, n_u):
            if j + 1 < n_u:
                d = dep
                for t in range(2):
                    x = x_v[pl.ds(r0[j + 1][t], 16), :].astype(_F32)
                    ms, rs = [], []
                    for q in range(2):
                        m, rstd, r, d = ln_stats(x[q * 8:(q + 1) * 8], d, True, wr)
                        ms.append(jnp.broadcast_to(m, (8, _G)))
                        rs.append(jnp.broadcast_to(rstd, (8, _G)))
                        row = sub_iota + (r0[j + 1][t] + q * 8)
                        upd = (r > best) | ((r == best) & (row < besti))
                        best = jnp.where(upd, r, best)
                        besti = jnp.where(upd, row, besti)
                    st[j + 1, t] = (jnp.concatenate(ms, axis=0), jnp.concatenate(rs, axis=0))
            if j < 0:
                continue
            for g in range(hd // _G):
                xn = {}
                for blocks, outs in _STAGES:
                    for t, h in blocks:
                        rows = pl.ds(pl.multiple_of(r0[j][t] + zero * 16, 16), 16)
                        csl = pl.ds(h * hd + g * _G, _G)
                        xc = x_v[rows, csl].astype(_F32)
                        xn[t, h] = (xc - (st[j, t][0] + rep(dep, 2))) * st[j, t][1]
                        res_v[pl.ds(pl.multiple_of(r0[j][t] // 2, 8), 8), csl] = _pack((xc + xn[t, h]).astype(_BF16))
                    for b in outs:
                        dst.at[b][pl.ds(j * 8, 8), pl.ds(g * _G, _G)] = _pack(_SEVEN[b](xn).astype(_BF16))
                    dep = zero_of_bits(dst[0, pl.ds(zero8, 8), pl.ds(0, _G)])
        best_v[...] = best
        besti_v[...] = besti

    def seven_rows(load, dst, dst_row, n_units, dep):
        for j in range(n_units):
            for g in range(hd // _G):
                w = {(a, b): load(a, b, j, g).astype(_F32) for a in range(2) for b in range(2)}
                for gate, outs in (((0, 0), (0, 1, 2, 4)), ((1, 0), (3, 5, 6))):
                    w[gate] = w[gate] + rep(dep, 2)
                    for b in outs:
                        dst.at[b][pl.ds(dst_row + j * 8, 8), pl.ds(g * _G, _G)] = _pack(_SEVEN[b](w).astype(_BF16))
                    dep = zero_of_bits(dst[0, pl.ds(dst_row + zero8, 8), pl.ds(0, _G)])
        return dep

    g_home = {(0, 0): 6, (0, 1): 2, (1, 0): 1, (1, 1): 5}

    def staged(stage, part):
        return _unpack(stage[...] if part is None else stage[pl.ds(part * hs // 2, hs // 2), :])

    def k_job(stage, c, first=False, part=None):
        p = _phi(_dot(staged(stage, part), wk_v[:, cols(c)]))
        zs = jnp.sum(p.reshape(p.shape[0] // 8, 8, _CB), axis=0)
        if first:
            z_v[:, cols(c)] = zs
        else:
            z_v[:, cols(c)] += zs
        return p.astype(_BF16)

    def g_job(pk, stage, c, first=False, part=None):
        upd = _dot_tn(pk, staged(stage, part))
        a, j = divmod(c, n_sl)
        for b in range(2):
            if first:
                gm_v[g_home[a, b], cols(j), :] = upd[:, b * hd:(b + 1) * hd]
            else:
                gm_v[g_home[a, b], cols(j), :] += upd[:, b * hd:(b + 1) * hd]

    def wk_load(j0):
        return lambda a, b, j, g: wk_v[pl.ds(a * hd + (j0 + j) * 16, 16), pl.ds(b * hd + g * _G, _G)]

    n_wu = hd // 16
    zero_v = jnp.zeros((8, _G), _F32)
    wait("x0a")
    ln_plain(0, _SUB // 2, sb_v, 16, False)
    wait("k0")
    p0a = k_job(sb_v, 0, True, part=0)
    wait("x0b")
    ln_plain(_SUB // 2, _SUB // 2, sb_v, 16, False)
    g_job(p0a, sb_v, 0, True, part=0)
    p0b = k_job(sb_v, 0, part=1)
    wait("k1")
    for m in (0, 3, 4):
        gm_v[m] = jnp.zeros(gm_v.shape[1:], _F32)
    p1 = k_job(sb_v, 1, True)
    g_job(p0b, sb_v, 0, part=1)
    g_job(p1, sb_v, 1, True)
    wait("k2x1")
    ln_plain(_SUB, _SUB, sa_v, 32, True)
    n_wa = n_wu * 5 // 8
    seven_rows(wk_load(0), wks_v, 0, n_wa, zero_v)
    p2 = k_job(sb_v, 2, True)
    p3 = k_job(sb_v, 3, True)
    g_job(p2, sb_v, 2, True)
    g_job(p3, sb_v, 3, True)
    wait("x23")
    seven_rows(wk_load(n_wa), wks_v, n_wa * 8, n_wu - n_wa, zero_v)
    ln_pair(1, xs_v.at[0], zero_v)
    pk = [k_job(sa_v, 0), k_job(sa_v, 2)]
    g_job(pk[0], sa_v, 0)
    pk.append(k_job(sa_v, 1))
    g_job(pk[1], sa_v, 2)
    gm_v[5, cols(0), :] += gm_v[1, cols(0), :] - gm_v[2, cols(0), :]
    pk.append(k_job(sa_v, 3))
    g_job(pk[2], sa_v, 1)
    g_job(pk[3], sa_v, 3)
    gm_v[5, cols(1), :] += gm_v[1, cols(1), :] - gm_v[2, cols(1), :]
    wait("x45q")

    def store_tr(blocks, j):
        for b, v in enumerate(_seven(*blocks)):
            tr_v.at[b][:, cols(j)] = _pack(v.astype(_BF16).T)
        return zero_of_bits(tr_v[0, pl.ds(zero8, 8), cols(0)])

    def phase1(i, carry):
        @pl.when(i == 1)
        def _():
            wait("x67")

        win = xs_v.at[pl.ds(i, 2)]
        cur = lambda b: _unpack(win[0, b, :, hcols])

        for u in range(2):
            s = jnp.minimum(2 * i + u, hd // _G - 1)
            for b in range(2):
                f0 = pl.multiple_of(b * hd + s * _G, _G)
                for c in range(n_cb):
                    wqt_v[u, b, :, cols(c)] = _pack(wq_v[cols(c), pl.ds(f0, _G)].T)
        wq_pin = zero_of_bits(wqt_v[0, 0, pl.ds(zero8, 1), cols(0)])
        dep = zero_v
        for u in range(2):
            s = jnp.minimum(2 * i + u, hd // _G - 1)
            load = lambda a, b, j, g, u=u: _unpack(
                wqt_v[u, b, pl.ds(pl.multiple_of(j * 8 + zero8, 8), 8), pl.ds(a * hd + g * _G, _G)])
            dep = seven_rows(load, wqs_v, pl.multiple_of(s * (_G // 2), _G // 2), _G // 16, dep)
        def ks_job(j, pin):
            def prod(m):
                p = _dot(cur(_A_IDX[m]), _unpack(wks_v[_B_IDX[m], :, cols(j)]))
                return p + pin if m == _PINM[0] else p

            p11, p12, p21, p22 = map(_phi, _strassen(prod))
            z_v[:, cols(j)] += jnp.sum((p11 + p21).reshape(_SUB // 8, 8, _CB), axis=0)
            z_v[:, cols(n_sl + j)] += jnp.sum((p12 + p22).reshape(_SUB // 8, 8, _CB), axis=0)
            return store_tr((p11, p21, p12, p22), j)

        pin = wq_pin
        for j in range(n_sl):
            pin = ks_job(j, pin[0:1, :])
        for j in range(n_sl):
            for m in range(7):
                gm_v[m, cols(j), :] += _dot(_unpack(tr_v[_A_IDX[m], :, cols(j)]), cur(_B_IDX[m]))
        ln_pair((i + 2) & (n_pair - 1), win.at[1], dep + pin[:, :_G])
        return carry

    jax.lax.fori_loop(0, n_pair - 1, phase1, 0)
    wait("vo")

    best, besti = best_v[...], besti_v[...]
    rmax = jnp.max(best, axis=0, keepdims=True)
    idx = jnp.min(jnp.where(best == rmax, besti, S - 1))
    idx_pair = idx // (2 * _SUB)
    gate_r = jax.nn.sigmoid(rmax)

    xs = x_v[pl.ds(pl.multiple_of((idx >> 4) * 16, 16), 16), :].astype(_F32)
    m, rstd = ln_stats(xs, None, False)
    xs = ((xs - m) * rstd).astype(_BF16).astype(_F32)
    sel = jax.lax.broadcasted_iota(jnp.int32, (16, D), 0) == (idx & 15)
    xs = jnp.sum(jnp.where(sel, xs, 0.0), axis=0, keepdims=True)
    for g in range(n_groups):
        xcol_v[pl.ds(g * _G, _G), :] = _col_bcast(xs[:, gsl(g)])
    res_row = pl.ds(pl.multiple_of((idx >> 4) * 8, 8), 8)
    for g in range(n_groups):
        z = jnp.sum(z_v[:, pl.ds(g * _G, _G)], axis=0, keepdims=True)
        zcol_v[pl.ds(g * _G, _G), :] = _col_bcast(z)

    rr = jax.lax.broadcasted_iota(jnp.int32, (_G, _G), 0) // dh
    cc = jax.lax.broadcasted_iota(jnp.int32, (_G, _G), 1) // dh
    same_head = rr == cc
    n_hg = hd // _G
    kvb = {}

    def kv_job(g):
        gm = lambda m: gm_v[m, pl.ds((g % n_hg) * _G, _G), :]
        if g < n_hg:
            row = [gm(0) + gm(3) - gm(4) + gm(6), gm(2) + gm(4)]
        else:
            row = [gm(1) + gm(3), gm(0) - gm(1) + gm(2) + gm(5)]
        kv = _dot(jnp.concatenate(row, axis=1).astype(_BF16), wv_v[:, pl.ds(g * _G, _G)])
        kvb[g] = jnp.where(same_head, kv, 0.0).astype(_BF16)

    def m_job(g):
        top, bot = [_dot(kvb.pop(q), wo_v[pl.ds(q * _G, _G), dcols]) for q in (g, g + n_hg)]
        for b, v in enumerate(_seven(top[:, :hd], top[:, hd:], bot[:, :hd], bot[:, hd:])):
            ms_v.at[b][pl.ds(g * _G // 2, _G // 2), :] = _pack(v.astype(_BF16))

    for g in range(n_hg):
        kv_job(g)
        kv_job(g + n_hg)
        if g > 0:
            m_job(g - 1)
    m_job(n_hg - 1)
    wait("f0")

    def chain_matvec(w_ref, lead, cb, col_ref, acc0):
        n = col_ref.shape[0] // 8
        acc = [acc0[:, :_G], acc0[:, _G:]]
        link = None
        for k0 in range(0, n, _BLK):
            rows = pl.ds(k0 * 8, _BLK * 8)
            w = w_ref[lead, rows, cols(cb)].astype(_F32)
            colv = col_ref[rows, :]
            for h in range(2):
                prod = (w[:, h * _G:(h + 1) * _G] * colv).reshape(_BLK, 8, _G)
                first = acc[h] if link is None else acc[h] + link
                acc[h] = jnp.sum(jnp.concatenate([first[None], prod], axis=0), axis=0)
                link = zero_like(acc[h])
        return jnp.concatenate(acc, axis=1)

    def phase2(i, carry):
        @pl.when(i == 1)
        def _():
            wait("f1")

        slot = (idx_pair + i) & (n_pair - 1)
        pair = (slot + 1) & (n_pair - 1)
        row0 = [pl.multiple_of(pair * (2 * _SUB) + t * _SUB, _SUB) for t in range(2)]
        win = xs_v.at[slot]
        cur = lambda b: _unpack(win[b, :, hcols])

        dep = jnp.zeros((8, _CB), _F32)
        ys = []
        for c in range(n_cb):
            ys.append(chain_matvec(wd_v, jnp.maximum(i - 1, 0), c, hcol_v, y_v[:, cols(c)] + dep))
            dep = zero_link(ys[-1])
        yacc = jnp.concatenate(ys, axis=1)
        y_v[...] = yacc
        yrow = jnp.sum(yacc, axis=0, keepdims=True) * gate_r
        hit = jax.lax.broadcasted_iota(jnp.int32, (16, D), 0) == jnp.where(i == n_pair - 1, idx & 15, -1)
        upd = _unpack(res_v[res_row, :]).astype(_F32) + jnp.where(hit, yrow, 0.0)
        res_v[res_row, :] = _pack(upd.astype(_BF16))
        accs = []
        for f in range(2 * fc // _CB):
            accs.append(chain_matvec(gu_v, jnp.minimum(i, n_fc - 1), f, xcol_v, dep))
            dep = zero_link(accs[-1])
        gu = jnp.sum(jnp.concatenate([a + dep for a in accs], axis=1), axis=0, keepdims=True)
        g, u = gu[:, :fc], gu[:, fc:]
        hnext = (g * jax.nn.sigmoid(g) * u).astype(_BF16).astype(_F32)
        lane = jax.lax.broadcasted_iota(jnp.int32, (1, fc), 1)
        hnext = jnp.where(lane < jnp.where(i > 0, f_dup, 0), 0.0, hnext)

        def normalise(p, c):
            zc = jnp.concatenate([zcol_v[cols(c), :]] * (_SUB // _G), axis=1)
            p3 = p.reshape(_CB // dh, dh, _SUB)
            den = jnp.sum(p3 * zc.reshape(_CB // dh, dh, _SUB), axis=1, keepdims=True) + _DEN_EPS
            return (p3 * pl.reciprocal(den, approx=True)).reshape(_CB, _SUB)

        def qs_job(j, pin):
            def prod(m):
                p = _dot_nt(_unpack(wqs_v[_B_IDX[m], pl.ds(j * _CB // 2, _CB // 2), :]), cur(_A_IDX[m]))
                return p + pin if pin is not None and m == _PINM[1] else p

            p11, p12, p21, p22 = map(_phi, _strassen(prod))
            o = [normalise(p11, j), normalise(p12, n_sl + j), normalise(p21, j), normalise(p22, n_sl + j)]
            return store_tr(o, j)[0:1, :]

        n_h = fc // _G

        def finish(cs, j, h_parts):
            order = (1, 3, 2, 0)
            for n, q in enumerate(order):
                t, b = divmod(q, 2)
                c = b * n_sl + j
                rows = pl.ds(row0[t], _SUB)
                res = cs[q] + _unpack(res_v[pl.ds(pl.multiple_of(row0[t] // 2, hs), hs), cols(c)]).astype(_F32)
                if len(h_parts[n]):
                    for f in h_parts[n]:
                        hcol_v[pl.ds(f * _G, _G), :] = _col_bcast(hnext[:, gsl(f)])
                    pin = zero_like(hcol_v[pl.ds(zero8, 1), :])
                    res = res + jnp.concatenate([pin] * (_CB // _G), axis=1)
                out_v[rows, cols(c)] = res.astype(_BF16)
                pltpu.make_async_copy(out_v.at[rows, cols(c)], out_hbm.at[rows, cols(c)], sem_o).start()

        pin = None
        for j in range(n_sl):
            pin = qs_job(j, pin)
        for j in range(n_sl):
            cs = _strassen_late22(lambda m: _dot(_unpack(tr_v[_A_IDX[m]]), _unpack(ms_v[_B_IDX[m], :, cols(j)])))
            last = j == n_sl - 1
            finish(cs, j, [range(0), range(0, n_h // 2), range(n_h // 2, n_h), range(0)] if last else [range(0)] * 4)
        return carry

    jax.lax.fori_loop(0, n_pair, phase2, 0)
    with _scope("w_out"):
        pltpu.make_async_copy(out_v, out_hbm, sem_o).wait()


@jax.jit
def pallas_parallel_sum__linear_attn_block__moe_arch_mod__prompt_kernel(
    A_x: jax.Array,
    A_wqkv: jax.Array,
    A_wo: jax.Array,
    B_x: jax.Array,
    B_w_r: jax.Array,
    B_w_gate: jax.Array,
    B_w_up: jax.Array,
    B_w_down: jax.Array,
):
    del B_x
    B, S, D = A_x.shape
    assert B == 1
    F = B_w_gate.shape[1]
    n_pair = S // _SUB // 2
    n_fc = n_pair - 1
    fc = _ffn_chunks(F, n_fc)[0]
    hd = D // 2
    any_spec = pl.BlockSpec(memory_space=pl.ANY)
    out = pl.pallas_call(
        functools.partial(_kernel, S=S, D=D, F=F),
        out_shape=jax.ShapeDtypeStruct((S, D), A_x.dtype),
        in_specs=[any_spec] * 7,
        out_specs=any_spec,
        scratch_shapes=[
            pltpu.VMEM((S, D), _BF16),
            pltpu.VMEM((D, D + _PAD), _BF16),
            pltpu.VMEM((D, D + _PAD), _BF16),
            pltpu.VMEM((D, D + _PAD), _BF16),
            pltpu.VMEM((D, D + _PAD), _BF16),
            pltpu.VMEM((D // _G, _G), _BF16),
            pltpu.VMEM((n_fc, D, 2 * fc), _BF16),
            pltpu.VMEM((n_fc, fc, D + _PAD), _BF16),
            pltpu.VMEM((_SUB // 2, D), _U32),
            pltpu.VMEM((_SUB // 2, D), _U32),
            pltpu.VMEM((n_pair, 7, _SUB // 2, hd + _PAD), _U32),
            pltpu.VMEM((S // 2, D), _U32),
            pltpu.VMEM((7, hd // 2, hd), _U32),
            pltpu.VMEM((2, 2, _G // 2, D), _U32),
            pltpu.VMEM((7, hd // 2, hd), _U32),
            pltpu.VMEM((7, hd, hd), _F32),
            pltpu.VMEM((8, D), _F32),
            pltpu.VMEM((8, 1), _F32),
            pltpu.VMEM((8, 1), jnp.int32),
            pltpu.VMEM((D, _G), _F32),
            pltpu.VMEM((D, _G), _F32),
            pltpu.VMEM((fc, _G), _F32),
            pltpu.VMEM((8, D), _F32),
            pltpu.VMEM((7, _SUB // 2, hd), _U32),
            pltpu.VMEM((7, hd // 2, hd), _U32),
            pltpu.VMEM((S, D), _BF16),
            pltpu.SemaphoreType.DMA((11,)),
            pltpu.SemaphoreType.DMA,
            pltpu.SemaphoreType.REGULAR,
        ],
        compiler_params=pltpu.CompilerParams(
            vmem_limit_bytes=110 * 1024 * 1024,
            disable_bounds_checks=not _CHECKS,
            disable_semaphore_checks=not _CHECKS,
        ),
    )(A_x.reshape(S, D), A_wqkv, A_wo, B_w_r.reshape(D // _G, _G), B_w_gate, B_w_up, B_w_down)
    return out.reshape(B, S, D)
```

```python
import contextlib
import functools
import os

import jax
import jax.numpy as jnp
import jax.experimental.pallas as pl
import jax.experimental.pallas.tpu as pltpu

_H = 32
_LN_EPS = 1e-5
_PHI_EPS = 1e-6
_DEN_EPS = 1e-6
_SUB = 256
_CB = 256
_G = 128
_BLK = 16
_PAD = 128

_PINM = tuple(int(v) for v in os.environ.get('PINM', '4,4').split(','))
_SEG = tuple(int(v) for v in os.environ.get('SEG', '3,6,5,6').split(','))
_SCOPES = bool(os.environ.get("KSCOPES"))
_CHECKS = bool(os.environ.get("KCHECKS"))


def _scope(name):
    return jax.named_scope(name) if _SCOPES else contextlib.nullcontext()


_F32 = jnp.float32
_BF16 = jnp.bfloat16
_U32 = jnp.uint32


def _dot(a, b):
    return jnp.dot(a, b, preferred_element_type=_F32)


def _dot_tn(a, b):
    return jax.lax.dot_general(a, b, (((0,), (0,)), ((), ())), preferred_element_type=_F32)


def _dot_nt(a, b):
    return jax.lax.dot_general(a, b, (((1,), (1,)), ((), ())), preferred_element_type=_F32)


def _phi(t):
    return jnp.where(t > 0, t + 1.0, jnp.exp(t)) + _PHI_EPS


def _pack(v):
    return pltpu.bitcast(v, _U32)


def _unpack(v):
    return pltpu.bitcast(v, _BF16)


def _col_bcast(row):
    return jnp.broadcast_to(row, (_G, _G)).T


_A_IDX = (2, 3, 0, 1, 4, 5, 6)
_B_IDX = (2, 0, 6, 5, 1, 4, 3)


def _seven(a11, a12, a21, a22):
    return [a11, a22, a11 + a22, a21 + a22, a11 + a12, a21 - a11, a12 - a22]


_SEVEN = (
    lambda a: a[0, 0],
    lambda a: a[1, 1],
    lambda a: a[0, 0] + a[1, 1],
    lambda a: a[1, 0] + a[1, 1],
    lambda a: a[0, 0] + a[0, 1],
    lambda a: a[1, 0] - a[0, 0],
    lambda a: a[0, 1] - a[1, 1],
)
_STAGES = ((((0, 0),), (0,)), (((1, 1),), (1, 2)), (((0, 1),), (4, 6)), (((1, 0),), (3, 5)))


def _strassen(prod):
    m1 = prod(0)
    m4 = prod(3)
    c11 = m1 + m4
    m2 = prod(1)
    c21 = m2 + m4
    c22 = m1 - m2
    m5 = prod(4)
    c11 = c11 - m5
    c11 = c11 + prod(6)
    m3 = prod(2)
    c12 = m3 + m5
    c22 = c22 + m3
    c22 = c22 + prod(5)
    return c11, c12, c21, c22


def _strassen_late22(prod):
    m6 = prod(5)
    m3 = prod(2)
    c22 = m6 + m3
    m5 = prod(4)
    c12 = m3 + m5
    m1 = prod(0)
    c11 = m1 - m5
    c22 = c22 + m1
    m2 = prod(1)
    c22 = c22 - m2
    m4 = prod(3)
    c21 = m2 + m4
    c11 = c11 + m4
    c11 = c11 + prod(6)
    return c11, c12, c21, c22


def _ffn_chunks(F, n):
    nb = F // _G
    per = -(-nb // n)
    step = (nb - per) // (n - 1)
    assert step * (n - 1) == nb - per
    return per * _G, [j * step * _G for j in range(n)], (per - step) * _G


def _kernel(x_hbm, wqkv_hbm, wo_hbm, wr_hbm, wg_hbm, wu_hbm, wd_hbm, out_hbm,
            x_v, wq_v, wk_v, wv_v, wo_v, wr_v, gu_v, wd_v,
            sa_v, sb_v, xs_v, res_v, wks_v, wqt_v, wqs_v, gm_v, z_v, best_v, besti_v,
            zcol_v, xcol_v, hcol_v, y_v, tr_v, ms_v, out_v,
            sem_i, sem_o, sem_b, *, S, D, F):
    n_sub = S // _SUB
    n_cb = D // _CB
    n_groups = D // _G
    dh = D // _H
    n_pair = n_sub // 2
    n_fc = n_pair - 1
    fc, f_start, f_dup = _ffn_chunks(F, n_fc)
    hs = _SUB // 2
    hd = D // 2
    n_sl = hd // _CB

    cols = lambda c: pl.ds(c * _CB, _CB)
    dcols = pl.ds(0, D)
    hcols = pl.ds(0, hd)
    gsl = lambda g: slice(g * _G, (g + 1) * _G)

    def x_cp(a, b, s):
        sl = pl.ds(int(a * _SUB), int((b - a) * _SUB))
        return pltpu.make_async_copy(x_hbm.at[sl, :], x_v.at[sl, :], sem_i.at[s])

    def k_cp(a, b, s):
        return pltpu.make_async_copy(wqkv_hbm.at[:, pl.ds(D + a * _CB, (b - a) * _CB)],
                                     wk_v.at[:, pl.ds(a * _CB, (b - a) * _CB)], sem_i.at[s])

    def gu_cps(j, s):
        src = pl.ds(f_start[j], fc)
        return [pltpu.make_async_copy(wg_hbm.at[:, src], gu_v.at[j, :, pl.ds(0, fc)], sem_i.at[s]),
                pltpu.make_async_copy(wu_hbm.at[:, src], gu_v.at[j, :, pl.ds(fc, fc)], sem_i.at[s])]

    def d_cp(j, s):
        return pltpu.make_async_copy(wd_hbm.at[pl.ds(f_start[j], fc), :], wd_v.at[j, :, dcols], sem_i.at[s])

    groups = dict(
        x0a=[x_cp(0, 0.5, 0)],
        k0=[k_cp(0, 1, 1)],
        x0b=[x_cp(0.5, 1, 2)],
        k1=[k_cp(1, 2, 3)],
        k2x1=[k_cp(2, n_cb, 4), x_cp(1, 2, 4)],
        x23=[x_cp(2, 4, 5), pltpu.make_async_copy(wr_hbm, wr_v, sem_i.at[5])],
        x45q=[x_cp(4, 6, 6),
              pltpu.make_async_copy(wqkv_hbm.at[:, pl.ds(0, D)], wq_v.at[:, dcols], sem_i.at[6])],
        x67=[x_cp(6, n_sub, 7)],
        vo=[pltpu.make_async_copy(wqkv_hbm.at[:, pl.ds(2 * D, D)], wv_v.at[:, dcols], sem_i.at[8]),
            pltpu.make_async_copy(wo_hbm, wo_v.at[:, dcols], sem_i.at[8])],
        f0=gu_cps(0, 9) + [d_cp(0, 9)],
        f1=sum([gu_cps(j, 10) + [d_cp(j, 10)] for j in range(1, n_fc)], []),
    )

    for grp in groups.values():
        for cp in grp:
            cp.start()
            pl.semaphore_signal(sem_b, 1)
            pl.semaphore_wait(sem_b, 1)

    def wait(name):
        with _scope("w_" + name):
            for cp in groups[name]:
                cp.wait()

    zero = pl.semaphore_read(sem_b)
    zero8 = pl.multiple_of(zero * 8, 8)
    zero_u = zero.astype(_U32)

    def zero_of_bits(u):
        return pltpu.bitcast(u & zero_u, _F32)

    def zero_like(v):
        return zero_of_bits(pltpu.bitcast(v, _U32))

    def zero_link(v):
        d = pltpu.bitcast(v, _U32)
        d = zero_of_bits(d[:, :_G] | d[:, _G:])
        return jnp.concatenate([d, d], axis=1)

    def rep(d, n):
        return jnp.concatenate([d] * n, axis=0)

    hcol_v[...] = jnp.zeros_like(hcol_v)
    y_v[...] = jnp.zeros_like(y_v)
    best_v[...] = jnp.full(best_v.shape, -jnp.inf, _F32)
    besti_v[...] = jnp.zeros_like(besti_v)

    def lane_partial(terms, dep):
        acc = terms[0] if dep is None else dep + terms[0]
        for t in terms[1:]:
            acc = acc + t
        return acc

    def ln_stats(x, dep, throttle, wr=None):
        s1 = lane_partial([x[:, gsl(g)] for g in range(n_groups)], dep)
        s2 = lane_partial([x[:, gsl(g)] * x[:, gsl(g)] for g in range(n_groups)],
                          zero_like(s1) if throttle else None)
        m = jnp.sum(s1, axis=-1, keepdims=True) * (1.0 / D)
        ex2 = jnp.sum(s2, axis=-1, keepdims=True) * (1.0 / D)
        rstd = jax.lax.rsqrt(jnp.maximum(ex2 - m * m, 0.0) + _LN_EPS)
        if wr is None:
            return m, rstd
        s3 = lane_partial([x[:, gsl(g)] * wr[0][:, gsl(g)] for g in range(n_groups)], zero_like(s2))
        r = (jnp.sum(s3, axis=-1, keepdims=True) - m * wr[1]) * rstd
        r = r.astype(_BF16).astype(_F32)
        rstd = jnp.where(r != r, r, rstd)
        return m, rstd, r, zero_like(s3)

    def ln_plain(row0, n_rows, stage, rows, throttle):
        for j in range(n_rows // rows):
            r0 = row0 + j * rows
            s0 = (r0 % _SUB) // 2
            x = x_v[pl.ds(r0, rows), :].astype(_F32)
            dep = None
            if throttle and j > 0:
                dep = rep(zero_of_bits(stage[pl.ds(zero8, 8), pl.ds(0, _G)]), rows // 8)
            m, rstd = ln_stats(x, dep, throttle)
            mb = jnp.broadcast_to(m, (rows, _G))
            for c in range(n_cb):
                xc = x_v[pl.ds(pl.multiple_of(r0 + zero * rows, rows), rows), cols(c)].astype(_F32)
                xn = _pack(((xc - jnp.concatenate([mb] * (_CB // _G), axis=1)) * rstd).astype(_BF16))
                stage[pl.ds(s0, rows // 2), cols(c)] = xn
                if throttle and c + 1 < n_cb:
                    mb = mb + rep(zero_of_bits(stage[pl.ds(zero8, 8), pl.ds(0, _G)]), rows // 8)

    sub_iota = jax.lax.broadcasted_iota(jnp.int32, (8, 1), 0)

    def ln_pair(pair, dst, dep):
        wr8 = wr_v[...].astype(_F32)
        wr = jnp.concatenate([wr8[g:g + 1, :] for g in range(n_groups)], axis=1)
        wr = (wr, jnp.sum(wr, axis=-1, keepdims=True))
        best, besti = best_v[...], besti_v[...]
        n_u = _SUB // 16
        base = pair * (2 * _SUB)
        x1 = x_v.at[pl.ds(pl.multiple_of(base, 2 * _SUB), 2 * _SUB)]
        x2 = x_v.at[pl.ds(pl.multiple_of(base + zero * 16, 16), 2 * _SUB)]
        res = res_v.at[pl.ds(pl.multiple_of(pair * _SUB, _SUB), _SUB)]
        row_iota = sub_iota + base
        r0 = [[t * _SUB + j * 16 for t in range(2)] for j in range(n_u)]
        st = {}
        for j in range(-1, n_u):
            if j + 1 < n_u:
                d = dep
                for t in range(2):
                    x = x1[pl.ds(r0[j + 1][t], 16), :].astype(_F32)
                    ms, rs = [], []
                    for q in range(2):
                        m, rstd, r, d = ln_stats(x[q * 8:(q + 1) * 8], d, True, wr)
                        ms.append(jnp.broadcast_to(m, (8, _G)))
                        rs.append(jnp.broadcast_to(rstd, (8, _G)))
                        row = row_iota + (r0[j + 1][t] + q * 8)
                        upd = (r > best) | ((r == best) & (row < besti))
                        best = jnp.where(upd, r, best)
                        besti = jnp.where(upd, row, besti)
                    st[j + 1, t] = (jnp.concatenate(ms, axis=0), jnp.concatenate(rs, axis=0))
            if j < 0:
                continue
            for g in range(hd // _G):
                xn = {}
                for blocks, outs in _STAGES:
                    for t, h in blocks:
                        csl = pl.ds(h * hd + g * _G, _G)
                        xc = x2[pl.ds(r0[j][t], 16), csl].astype(_F32)
                        xn[t, h] = (xc - (st[j, t][0] + rep(dep, 2))) * st[j, t][1]
                        res[pl.ds(r0[j][t] // 2, 8), csl] = _pack((xc + xn[t, h]).astype(_BF16))
                    for b in outs:
                        dst.at[b][pl.ds(j * 8, 8), pl.ds(g * _G, _G)] = _pack(_SEVEN[b](xn).astype(_BF16))
                    dep = zero_of_bits(dst[0, pl.ds(zero8, 8), pl.ds(0, _G)])
        best_v[...] = best
        besti_v[...] = besti

    def seven_rows(load, dst, dst_row, n_units, dep):
        for j in range(n_units):
            for g in range(hd // _G):
                w = {(a, b): load(a, b, j, g).astype(_F32) for a in range(2) for b in range(2)}
                for gate, outs in (((0, 0), (0, 1, 2, 4)), ((1, 0), (3, 5, 6))):
                    w[gate] = w[gate] + rep(dep, 2)
                    for b in outs:
                        dst.at[b][pl.ds(dst_row + j * 8, 8), pl.ds(g * _G, _G)] = _pack(_SEVEN[b](w).astype(_BF16))
                    dep = zero_of_bits(dst[0, pl.ds(dst_row + zero8, 8), pl.ds(0, _G)])
        return dep

    g_home = {(0, 0): 6, (0, 1): 2, (1, 0): 1, (1, 1): 5}

    def staged(stage, part):
        return _unpack(stage[...] if part is None else stage[pl.ds(part * hs // 2, hs // 2), :])

    def k_job(stage, c, first=False, part=None):
        p = _phi(_dot(staged(stage, part), wk_v[:, cols(c)]))
        zs = jnp.sum(p.reshape(p.shape[0] // 8, 8, _CB), axis=0)
        if first:
            z_v[:, cols(c)] = zs
        else:
            z_v[:, cols(c)] += zs
        return p.astype(_BF16)

    def g_job(pk, stage, c, first=False, part=None):
        upd = _dot_tn(pk, staged(stage, part))
        a, j = divmod(c, n_sl)
        for b in range(2):
            if first:
                gm_v[g_home[a, b], cols(j), :] = upd[:, b * hd:(b + 1) * hd]
            else:
                gm_v[g_home[a, b], cols(j), :] += upd[:, b * hd:(b + 1) * hd]

    def wk_load(j0):
        return lambda a, b, j, g: wk_v[pl.ds(a * hd + (j0 + j) * 16, 16), pl.ds(b * hd + g * _G, _G)]

    n_wu = hd // 16
    zero_v = jnp.zeros((8, _G), _F32)
    wait("x0a")
    ln_plain(0, _SUB // 2, sb_v, 16, False)
    wait("k0")
    p0a = k_job(sb_v, 0, True, part=0)
    wait("x0b")
    ln_plain(_SUB // 2, _SUB // 2, sb_v, 16, False)
    g_job(p0a, sb_v, 0, True, part=0)
    p0b = k_job(sb_v, 0, part=1)
    wait("k1")
    for m in (0, 3, 4):
        gm_v[m] = jnp.zeros(gm_v.shape[1:], _F32)
    p1 = k_job(sb_v, 1, True)
    g_job(p0b, sb_v, 0, part=1)
    g_job(p1, sb_v, 1, True)
    wait("k2x1")
    ln_plain(_SUB, _SUB, sa_v, 32, True)
    n_wa = n_wu * 5 // 8
    seven_rows(wk_load(0), wks_v, 0, n_wa, zero_v)
    p2 = k_job(sb_v, 2, True)
    p3 = k_job(sb_v, 3, True)
    g_job(p2, sb_v, 2, True)
    g_job(p3, sb_v, 3, True)
    wait("x23")
    seven_rows(wk_load(n_wa), wks_v, n_wa * 8, n_wu - n_wa, zero_v)
    ln_pair(1, xs_v.at[0], zero_v)
    pk = [k_job(sa_v, 0), k_job(sa_v, 2)]
    g_job(pk[0], sa_v, 0)
    pk.append(k_job(sa_v, 1))
    g_job(pk[1], sa_v, 2)
    gm_v[5, cols(0), :] += gm_v[1, cols(0), :] - gm_v[2, cols(0), :]
    pk.append(k_job(sa_v, 3))
    g_job(pk[2], sa_v, 1)
    g_job(pk[3], sa_v, 3)
    gm_v[5, cols(1), :] += gm_v[1, cols(1), :] - gm_v[2, cols(1), :]
    wait("x45q")

    def store_tr(blocks, j):
        for b, v in enumerate(_seven(*blocks)):
            tr_v.at[b][:, cols(j)] = _pack(v.astype(_BF16).T)
        return zero_of_bits(tr_v[0, pl.ds(zero8, 8), cols(0)])

    def phase1(i, carry):
        @pl.when(i == 1)
        def _():
            wait("x67")

        win = xs_v.at[pl.ds(i, 2)]
        cur = lambda b: _unpack(win[0, b, :, hcols])

        for u in range(2):
            s = jnp.minimum(2 * i + u, hd // _G - 1)
            for b in range(2):
                f0 = pl.multiple_of(b * hd + s * _G, _G)
                for c in range(n_cb):
                    wqt_v[u, b, :, cols(c)] = _pack(wq_v[cols(c), pl.ds(f0, _G)].T)
        wq_pin = zero_of_bits(wqt_v[0, 0, pl.ds(zero8, 1), cols(0)])
        dep = zero_v
        for u in range(2):
            s = jnp.minimum(2 * i + u, hd // _G - 1)
            load = lambda a, b, j, g, u=u: _unpack(
                wqt_v[u, b, pl.ds(pl.multiple_of(j * 8 + zero8, 8), 8), pl.ds(a * hd + g * _G, _G)])
            dep = seven_rows(load, wqs_v, pl.multiple_of(s * (_G // 2), _G // 2), _G // 16, dep)
        def ks_job(j, pin):
            def prod(m):
                p = _dot(cur(_A_IDX[m]), _unpack(wks_v[_B_IDX[m], :, cols(j)]))
                return p + pin if m == _PINM[0] else p

            p11, p12, p21, p22 = map(_phi, _strassen(prod))
            z_v[:, cols(j)] += jnp.sum((p11 + p21).reshape(_SUB // 8, 8, _CB), axis=0)
            z_v[:, cols(n_sl + j)] += jnp.sum((p12 + p22).reshape(_SUB // 8, 8, _CB), axis=0)
            return store_tr((p11, p21, p12, p22), j)

        pin = wq_pin
        for j in range(n_sl):
            pin = ks_job(j, pin[0:1, :])
        for j in range(n_sl):
            for m in range(7):
                gm_v[m, cols(j), :] += _dot(_unpack(tr_v[_A_IDX[m], :, cols(j)]), cur(_B_IDX[m]))
        ln_pair((i + 2) & (n_pair - 1), win.at[1], dep + pin[:, :_G])
        return carry

    jax.lax.fori_loop(0, n_pair - 1, phase1, 0)
    wait("vo")

    best, besti = best_v[...], besti_v[...]
    rmax = jnp.max(best, axis=0, keepdims=True)
    idx = jnp.min(jnp.where(best == rmax, besti, S - 1))
    idx_pair = idx // (2 * _SUB)
    gate_r = jax.nn.sigmoid(rmax)

    xs = x_v[pl.ds(pl.multiple_of((idx >> 4) * 16, 16), 16), :].astype(_F32)
    m, rstd = ln_stats(xs, None, False)
    xs = ((xs - m) * rstd).astype(_BF16).astype(_F32)
    sel = jax.lax.broadcasted_iota(jnp.int32, (16, D), 0) == (idx & 15)
    xs = jnp.sum(jnp.where(sel, xs, 0.0), axis=0, keepdims=True)
    for g in range(n_groups):
        xcol_v[pl.ds(g * _G, _G), :] = _col_bcast(xs[:, gsl(g)])
    res_row = pl.ds(pl.multiple_of((idx >> 4) * 8, 8), 8)
    for g in range(n_groups):
        z = jnp.sum(z_v[:, pl.ds(g * _G, _G)], axis=0, keepdims=True)
        zcol_v[pl.ds(g * _G, _G), :] = _col_bcast(z)

    rr = jax.lax.broadcasted_iota(jnp.int32, (_G, _G), 0) // dh
    cc = jax.lax.broadcasted_iota(jnp.int32, (_G, _G), 1) // dh
    same_head = rr == cc
    n_hg = hd // _G
    kvb = {}

    def kv_job(g):
        gm = lambda m: gm_v[m, pl.ds((g % n_hg) * _G, _G), :]
        if g < n_hg:
            row = [gm(0) + gm(3) - gm(4) + gm(6), gm(2) + gm(4)]
        else:
            row = [gm(1) + gm(3), gm(0) - gm(1) + gm(2) + gm(5)]
        kv = _dot(jnp.concatenate(row, axis=1).astype(_BF16), wv_v[:, pl.ds(g * _G, _G)])
        kvb[g] = jnp.where(same_head, kv, 0.0).astype(_BF16)

    def m_job(g):
        top, bot = [_dot(kvb.pop(q), wo_v[pl.ds(q * _G, _G), dcols]) for q in (g, g + n_hg)]
        for b, v in enumerate(_seven(top[:, :hd], top[:, hd:], bot[:, :hd], bot[:, hd:])):
            ms_v.at[b][pl.ds(g * _G // 2, _G // 2), :] = _pack(v.astype(_BF16))

    for g in range(n_hg):
        kv_job(g)
        kv_job(g + n_hg)
        if g > 0:
            m_job(g - 1)
    m_job(n_hg - 1)
    wait("f0")

    def chain_matvec(w_ref, lead, cb, col_ref, acc0):
        n = col_ref.shape[0] // 8
        acc = [acc0[:, :_G], acc0[:, _G:]]
        link = None
        for k0 in range(0, n, _BLK):
            rows = pl.ds(k0 * 8, _BLK * 8)
            w = w_ref[lead, rows, cols(cb)].astype(_F32)
            colv = col_ref[rows, :]
            for h in range(2):
                prod = (w[:, h * _G:(h + 1) * _G] * colv).reshape(_BLK, 8, _G)
                first = acc[h] if link is None else acc[h] + link
                acc[h] = jnp.sum(jnp.concatenate([first[None], prod], axis=0), axis=0)
                link = zero_like(acc[h])
        return jnp.concatenate(acc, axis=1)

    def phase2(i, carry):
        @pl.when(i == 1)
        def _():
            wait("f1")

        slot = (idx_pair + i) & (n_pair - 1)
        pair = (slot + 1) & (n_pair - 1)
        prows = pl.ds(pl.multiple_of(pair * (2 * _SUB), 2 * _SUB), 2 * _SUB)
        out_w, hbm_w = out_v.at[prows], out_hbm.at[prows]
        res_w = res_v.at[pl.ds(pl.multiple_of(pair * _SUB, _SUB), _SUB)]
        win = xs_v.at[slot]
        cur = lambda b: _unpack(win[b, :, hcols])

        ys, accs, pins = [], [], {}
        n_gu = 2 * fc // _CB

        def ffn_part(first, last, dep):
            for n in range(first, last):
                if n < n_cb:
                    ys.append(chain_matvec(wd_v, jnp.maximum(i - 1, 0), n, hcol_v, y_v[:, cols(n)] + dep))
                    dep = zero_link(ys[-1])
                else:
                    accs.append(chain_matvec(gu_v, jnp.minimum(i, n_fc - 1), n - n_cb, xcol_v, dep))
                    dep = zero_link(accs[-1])
            return dep

        def normalise(p, c):
            zc = jnp.concatenate([zcol_v[cols(c), :]] * (_SUB // _G), axis=1)
            p3 = p.reshape(_CB // dh, dh, _SUB)
            den = jnp.sum(p3 * zc.reshape(_CB // dh, dh, _SUB), axis=1, keepdims=True) + _DEN_EPS
            return (p3 * pl.reciprocal(den, approx=True)).reshape(_CB, _SUB)

        def qs_job(j, pin):
            def prod(m):
                p = _dot_nt(_unpack(wqs_v[_B_IDX[m], pl.ds(j * _CB // 2, _CB // 2), :]), cur(_A_IDX[m]))
                if (j, m) in pins:
                    p = p + pins[j, m]
                return p + pin if pin is not None and m == _PINM[1] else p

            p11, p12, p21, p22 = map(_phi, _strassen(prod))
            o = [normalise(p11, j), normalise(p12, n_sl + j), normalise(p21, j), normalise(p22, n_sl + j)]
            return store_tr(o, j)

        n_h = fc // _G

        def finish(cs, j, h_parts):
            order = (1, 3, 2, 0)
            for n, q in enumerate(order):
                t, b = divmod(q, 2)
                c = b * n_sl + j
                rows = pl.ds(t * _SUB, _SUB)
                res = cs[q] + _unpack(res_w[pl.ds(t * hs, hs), cols(c)]).astype(_F32)
                if len(h_parts[n]):
                    for f in h_parts[n]:
                        hcol_v[pl.ds(f * _G, _G), :] = _col_bcast(hnext[:, gsl(f)])
                    pin = zero_like(hcol_v[pl.ds(zero8, 1), :])
                    res = res + jnp.concatenate([pin] * (_CB // _G), axis=1)
                out_w[rows, cols(c)] = res.astype(_BF16)
                pltpu.make_async_copy(out_w.at[rows, cols(c)], hbm_w.at[rows, cols(c)], sem_o).start()

        dep = ffn_part(0, _SEG[0], jnp.zeros((8, _CB), _F32))
        pins[0, _SEG[1]] = dep[0:1, :]
        rel = qs_job(0, None)
        dep = ffn_part(_SEG[0], _SEG[2], dep + rel)
        pins[1, _SEG[3]] = dep[0:1, :]
        qs_job(1, rel[0:1, :])
        dep = ffn_part(_SEG[2], n_cb + n_gu, jnp.zeros((8, _CB), _F32))

        yacc = jnp.concatenate(ys, axis=1)
        y_v[...] = yacc
        yrow = jnp.sum(yacc, axis=0, keepdims=True) * gate_r
        hit = jax.lax.broadcasted_iota(jnp.int32, (16, D), 0) == jnp.where(i == n_pair - 1, idx & 15, -1)
        upd = _unpack(res_v[res_row, :]).astype(_F32) + jnp.where(hit, yrow, 0.0)
        res_v[res_row, :] = _pack(upd.astype(_BF16))
        gu = jnp.sum(jnp.concatenate([a + dep for a in accs], axis=1), axis=0, keepdims=True)
        g, u = gu[:, :fc], gu[:, fc:]
        hnext = (g * jax.nn.sigmoid(g) * u).astype(_BF16).astype(_F32)
        lane = jax.lax.broadcasted_iota(jnp.int32, (1, fc), 1)
        hnext = jnp.where(lane < jnp.where(i > 0, f_dup, 0), 0.0, hnext)

        for j in range(n_sl):
            cs = _strassen_late22(lambda m: _dot(_unpack(tr_v[_A_IDX[m]]), _unpack(ms_v[_B_IDX[m], :, cols(j)])))
            last = j == n_sl - 1
            finish(cs, j, [range(0), range(0, n_h // 2), range(n_h // 2, n_h), range(0)] if last else [range(0)] * 4)
        return carry

    jax.lax.fori_loop(0, n_pair, phase2, 0)
    with _scope("w_out"):
        pltpu.make_async_copy(out_v, out_hbm, sem_o).wait()


@jax.jit
def pallas_parallel_sum__linear_attn_block__moe_arch_mod__prompt_kernel(
    A_x: jax.Array,
    A_wqkv: jax.Array,
    A_wo: jax.Array,
    B_x: jax.Array,
    B_w_r: jax.Array,
    B_w_gate: jax.Array,
    B_w_up: jax.Array,
    B_w_down: jax.Array,
):
    del B_x
    B, S, D = A_x.shape
    assert B == 1
    F = B_w_gate.shape[1]
    n_pair = S // _SUB // 2
    n_fc = n_pair - 1
    fc = _ffn_chunks(F, n_fc)[0]
    hd = D // 2
    any_spec = pl.BlockSpec(memory_space=pl.ANY)
    out = pl.pallas_call(
        functools.partial(_kernel, S=S, D=D, F=F),
        out_shape=jax.ShapeDtypeStruct((S, D), A_x.dtype),
        in_specs=[any_spec] * 7,
        out_specs=any_spec,
        scratch_shapes=[
            pltpu.VMEM((S, D), _BF16),
            pltpu.VMEM((D, D + _PAD), _BF16),
            pltpu.VMEM((D, D + _PAD), _BF16),
            pltpu.VMEM((D, D + _PAD), _BF16),
            pltpu.VMEM((D, D + _PAD), _BF16),
            pltpu.VMEM((D // _G, _G), _BF16),
            pltpu.VMEM((n_fc, D, 2 * fc), _BF16),
            pltpu.VMEM((n_fc, fc, D + _PAD), _BF16),
            pltpu.VMEM((_SUB // 2, D), _U32),
            pltpu.VMEM((_SUB // 2, D), _U32),
            pltpu.VMEM((n_pair, 7, _SUB // 2, hd + _PAD), _U32),
            pltpu.VMEM((S // 2, D), _U32),
            pltpu.VMEM((7, hd // 2, hd), _U32),
            pltpu.VMEM((2, 2, _G // 2, D), _U32),
            pltpu.VMEM((7, hd // 2, hd), _U32),
            pltpu.VMEM((7, hd, hd), _F32),
            pltpu.VMEM((8, D), _F32),
            pltpu.VMEM((8, 1), _F32),
            pltpu.VMEM((8, 1), jnp.int32),
            pltpu.VMEM((D, _G), _F32),
            pltpu.VMEM((D, _G), _F32),
            pltpu.VMEM((fc, _G), _F32),
            pltpu.VMEM((8, D), _F32),
            pltpu.VMEM((7, _SUB // 2, hd), _U32),
            pltpu.VMEM((7, hd // 2, hd), _U32),
            pltpu.VMEM((S, D), _BF16),
            pltpu.SemaphoreType.DMA((11,)),
            pltpu.SemaphoreType.DMA,
            pltpu.SemaphoreType.REGULAR,
        ],
        compiler_params=pltpu.CompilerParams(
            vmem_limit_bytes=110 * 1024 * 1024,
            disable_bounds_checks=not _CHECKS,
            disable_semaphore_checks=not _CHECKS,
        ),
    )(A_x.reshape(S, D), A_wqkv, A_wo, B_w_r.reshape(D // _G, _G), B_w_gate, B_w_up, B_w_down)
    return out.reshape(B, S, D)
```

```python
import functools

import jax
import jax.numpy as jnp
import jax.experimental.pallas as pl
import jax.experimental.pallas.tpu as pltpu

_H = 32
_LN_EPS = 1e-5
_PHI_EPS = 1e-6
_DEN_EPS = 1e-6
_SUB = 256
_CB = 256
_G = 128
_BLK = 16
_PAD = 128

_RUNTIME_CHECKS = False

_F32 = jnp.float32
_BF16 = jnp.bfloat16
_U32 = jnp.uint32


def _dot(a, b):
    return jnp.dot(a, b, preferred_element_type=_F32)


def _dot_tn(a, b):
    return jax.lax.dot_general(a, b, (((0,), (0,)), ((), ())), preferred_element_type=_F32)


def _dot_nt(a, b):
    return jax.lax.dot_general(a, b, (((1,), (1,)), ((), ())), preferred_element_type=_F32)


def _phi(t):
    return jnp.where(t > 0, t + 1.0, jnp.exp(t)) + _PHI_EPS


def _pack(v):
    return pltpu.bitcast(v, _U32)


def _unpack(v):
    return pltpu.bitcast(v, _BF16)


def _col_bcast(row):
    return jnp.broadcast_to(row, (_G, _G)).T


_A_IDX = (2, 3, 0, 1, 4, 5, 6)
_B_IDX = (2, 0, 6, 5, 1, 4, 3)


def _seven(a11, a12, a21, a22):
    return [a11, a22, a11 + a22, a21 + a22, a11 + a12, a21 - a11, a12 - a22]


_SEVEN = (
    lambda a: a[0, 0],
    lambda a: a[1, 1],
    lambda a: a[0, 0] + a[1, 1],
    lambda a: a[1, 0] + a[1, 1],
    lambda a: a[0, 0] + a[0, 1],
    lambda a: a[1, 0] - a[0, 0],
    lambda a: a[0, 1] - a[1, 1],
)
_STAGES3 = ((((0, 0), (1, 1)), (0, 1, 2)), (((0, 1),), (4, 6)), (((1, 0),), (3, 5)))
_STAGES = ((((0, 0),), (0,)), (((1, 1),), (1, 2)), (((0, 1),), (4, 6)), (((1, 0),), (3, 5)))


def _strassen(prod):
    m1 = prod(0)
    m4 = prod(3)
    c11 = m1 + m4
    m2 = prod(1)
    c21 = m2 + m4
    c22 = m1 - m2
    m5 = prod(4)
    c11 = c11 - m5
    c11 = c11 + prod(6)
    m3 = prod(2)
    c12 = m3 + m5
    c22 = c22 + m3
    c22 = c22 + prod(5)
    return c11, c12, c21, c22


def _strassen_late22(prod):
    m6 = prod(5)
    m3 = prod(2)
    c22 = m6 + m3
    m5 = prod(4)
    c12 = m3 + m5
    m1 = prod(0)
    c11 = m1 - m5
    c22 = c22 + m1
    m2 = prod(1)
    c22 = c22 - m2
    m4 = prod(3)
    c21 = m2 + m4
    c11 = c11 + m4
    c11 = c11 + prod(6)
    return c11, c12, c21, c22


def _ffn_chunks(F, n):
    nb = F // _G
    per = -(-nb // n)
    step = (nb - per) // (n - 1)
    assert step * (n - 1) == nb - per
    return per * _G, [j * step * _G for j in range(n)], (per - step) * _G


def _kernel(x_hbm, wqkv_hbm, wo_hbm, wr_hbm, wg_hbm, wu_hbm, wd_hbm, out_hbm,
            x_v, wq_v, wk_v, wv_v, wo_v, wr_v, gu_v, wd_v,
            xh_v, sb_v, xs_v, res_v, wks_v, wqt_v, wqs_v, gm_v, z_v, best_v,
            zcol_v, xcol_v, h_v, hcol_v, y_v, tr_v, ms_v, out_v,
            sem_i, sem_o, sem_b, *, S, D, F):
    n_sub = S // _SUB
    n_cb = D // _CB
    n_groups = D // _G
    dh = D // _H
    n_pair = n_sub // 2
    n_fc = n_pair - 1
    fc, f_start, f_dup = _ffn_chunks(F, n_fc)
    hs = _SUB // 2
    hd = D // 2
    n_sl = hd // _CB

    cols = lambda c: pl.ds(c * _CB, _CB)
    dcols = pl.ds(0, D)
    hcols = pl.ds(0, hd)
    gsl = lambda g: slice(g * _G, (g + 1) * _G)

    def x_cp(a, b, s):
        sl = pl.ds(int(a * _SUB), int((b - a) * _SUB))
        return pltpu.make_async_copy(x_hbm.at[sl, :], x_v.at[sl, :], sem_i.at[s])

    def k_cp(a, b, s):
        return pltpu.make_async_copy(wqkv_hbm.at[:, pl.ds(D + a * _CB, (b - a) * _CB)],
                                     wk_v.at[:, pl.ds(a * _CB, (b - a) * _CB)], sem_i.at[s])

    def gu_cps(j, s):
        src = pl.ds(f_start[j], fc)
        return [pltpu.make_async_copy(wg_hbm.at[:, src], gu_v.at[j, :, pl.ds(0, fc)], sem_i.at[s]),
                pltpu.make_async_copy(wu_hbm.at[:, src], gu_v.at[j, :, pl.ds(fc, fc)], sem_i.at[s])]

    def d_cp(j, s):
        return pltpu.make_async_copy(wd_hbm.at[pl.ds(f_start[j], fc), :], wd_v.at[j, :, dcols], sem_i.at[s])

    groups = dict(
        x0a=[x_cp(0, 0.5, 0)],
        k0=[k_cp(0, 1, 1)],
        x0b=[x_cp(0.5, 1, 2)],
        k1=[k_cp(2, 3, 3)],
        k2x1=[k_cp(1, 2, 4), k_cp(3, 4, 4), x_cp(1, 2, 4)],
        x23=[x_cp(2, 4, 5), pltpu.make_async_copy(wr_hbm, wr_v, sem_i.at[5])],
        x45q=[x_cp(4, 6, 6),
              pltpu.make_async_copy(wqkv_hbm.at[:, pl.ds(0, D)], wq_v.at[:, dcols], sem_i.at[6])],
        x67=[x_cp(6, n_sub, 7)],
        vo=[pltpu.make_async_copy(wqkv_hbm.at[:, pl.ds(2 * D, D)], wv_v.at[:, dcols], sem_i.at[8]),
            pltpu.make_async_copy(wo_hbm, wo_v.at[:, dcols], sem_i.at[8])],
        f0=gu_cps(0, 9) + [d_cp(0, 9)],
        f1=sum([gu_cps(j, 10) + [d_cp(j, 10)] for j in range(1, n_fc)], []),
    )

    for grp in groups.values():
        for cp in grp:
            cp.start()
            pl.semaphore_signal(sem_b, 1)
            pl.semaphore_wait(sem_b, 1)

    def wait(name):
        for cp in groups[name]:
            cp.wait()

    zero = pl.semaphore_read(sem_b)
    zero8 = pl.multiple_of(zero * 8, 8)
    zero_u = zero.astype(_U32)

    def zero_of_bits(u):
        return pltpu.bitcast(u & zero_u, _F32)

    def zero_like(v):
        return zero_of_bits(pltpu.bitcast(v, _U32))

    def zero_link(v):
        d = pltpu.bitcast(v, _U32)
        d = zero_of_bits(d[:, :_G] | d[:, _G:])
        return jnp.concatenate([d, d], axis=1)

    def rep(d, n):
        return jnp.concatenate([d] * n, axis=0)

    h_v[...] = jnp.zeros_like(h_v)
    y_v[...] = jnp.zeros_like(y_v)
    best_v[...] = jnp.full(best_v.shape, -jnp.inf, _F32)

    def lane_partial(terms, dep):
        acc = terms[0] if dep is None else dep + terms[0]
        for t in terms[1:]:
            acc = acc + t
        return acc

    def ln_stats(x, dep, throttle, wr=None):
        s1 = lane_partial([x[:, gsl(g)] for g in range(n_groups)], dep)
        s2 = lane_partial([x[:, gsl(g)] * x[:, gsl(g)] for g in range(n_groups)],
                          zero_like(s1) if throttle else None)
        m = jnp.sum(s1, axis=-1, keepdims=True) * (1.0 / D)
        ex2 = jnp.sum(s2, axis=-1, keepdims=True) * (1.0 / D)
        rstd = jnp.exp2(-0.5 * jnp.log2(jnp.maximum(ex2 - m * m, 0.0) + _LN_EPS))
        if wr is None:
            return m, rstd, None, zero_like(s2)
        s3 = lane_partial([x[:, gsl(g)] * wr[0][:, gsl(g)] for g in range(n_groups)], zero_like(s2))
        r = (jnp.sum(s3, axis=-1, keepdims=True) - m * wr[1]) * rstd
        r = r.astype(_BF16).astype(_F32)
        return m, rstd + zero_like(r), r, zero_like(s3)

    def ln_plain(row0, n_rows, stage, rows, throttle):
        for j in range(n_rows // rows):
            r0 = row0 + j * rows
            s0 = (r0 % _SUB) // 2
            x = x_v[pl.ds(r0, rows), :].astype(_F32)
            dep = None
            if throttle and j > 0:
                dep = rep(zero_of_bits(stage[pl.ds(zero8, 8), pl.ds(0, _G)]), rows // 8)
            m, rstd = ln_stats(x, dep, throttle)[:2]
            mb = jnp.broadcast_to(m, (rows, _G))
            for c in range(n_cb):
                xc = x_v[pl.ds(pl.multiple_of(r0 + zero * rows, rows), rows), cols(c)].astype(_F32)
                xn = _pack(((xc - jnp.concatenate([mb] * (_CB // _G), axis=1)) * rstd).astype(_BF16))
                stage[pl.ds(s0, rows // 2), cols(c)] = xn
                if throttle and c + 1 < n_cb:
                    mb = mb + rep(zero_of_bits(stage[pl.ds(zero8, 8), pl.ds(0, _G)]), rows // 8)

    sub_iota = jax.lax.broadcasted_iota(jnp.int32, (8, 1), 0)

    def ln_pair(pair, dst, dep, half=_SUB, full=True, stages=_STAGES):
        wr = None
        if full:
            wr8 = wr_v[...].astype(_F32)
            wr = jnp.concatenate([wr8[g:g + 1, :] for g in range(n_groups)], axis=1)
            wr = (wr, jnp.sum(wr, axis=-1, keepdims=True))
            best = best_v[...]
        n_u = half // 16
        base = pair * (2 * half)
        x1 = x_v.at[pl.ds(pl.multiple_of(base, 2 * half), 2 * half)]
        x2 = x_v.at[pl.ds(pl.multiple_of(base + zero * 16, 16), 2 * half)]
        res = res_v.at[pl.ds(pl.multiple_of(pair * half, half), half)]
        rev_iota = ((S - 1 - base) - sub_iota).astype(_U32)
        r0 = [[t * half + j * 16 for t in range(2)] for j in range(n_u)]
        st = {}
        for j in range(-1, n_u):
            if j + 1 < n_u:
                d = dep
                for t in range(2):
                    x = x1[pl.ds(r0[j + 1][t], 16), :].astype(_F32)
                    ms, rs = [], []
                    for q in range(2):
                        m, rstd, r, d = ln_stats(x[q * 8:(q + 1) * 8], d, True, wr)
                        ms.append(jnp.broadcast_to(m, (8, _G)))
                        rs.append(jnp.broadcast_to(rstd, (8, _G)))
                        if full:
                            key = pltpu.bitcast(r, _U32) | (rev_iota - (r0[j + 1][t] + q * 8))
                            best = jnp.maximum(best, pltpu.bitcast(key, _F32))
                    st[j + 1, t] = (jnp.concatenate(ms, axis=0), jnp.concatenate(rs, axis=0))
            if j < 0:
                continue
            for g in range(hd // _G):
                xn = {}
                for blocks, outs in stages:
                    for t, h in blocks:
                        csl = pl.ds(h * hd + g * _G, _G)
                        xc = x2[pl.ds(r0[j][t], 16), csl].astype(_F32)
                        mb = st[j, t][0]
                        mb = jnp.concatenate([mb[:8] + dep, mb[8:]], axis=0)
                        xn[t, h] = (xc - mb) * st[j, t][1]
                        if full:
                            res[pl.ds(r0[j][t] // 2, 8), csl] = _pack((xc + xn[t, h]).astype(_BF16))
                    for b in outs:
                        dst.at[b][pl.ds(j * 8, 8), pl.ds(g * _G, _G)] = _pack(_SEVEN[b](xn).astype(_BF16))
                    dep = zero_of_bits(dst[0, pl.ds(zero8, 8), pl.ds(0, _G)])
        if full:
            best_v[...] = best
        return dep

    def seven_rows(load, dst, dst_row, n_units, dep, gs=range(hd // _G)):
        for j in range(n_units):
            for g in gs:
                w = {(a, b): load(a, b, j, g).astype(_F32) for a in range(2) for b in range(2)}
                for gate, outs in (((0, 0), (0, 1, 2, 4)), ((1, 0), (3, 5, 6))):
                    w[gate] = jnp.concatenate([w[gate][:8] + dep, w[gate][8:]], axis=0)
                    for b in outs:
                        dst.at[b][pl.ds(dst_row + j * 8, 8), pl.ds(g * _G, _G)] = _pack(_SEVEN[b](w).astype(_BF16))
                    dep = zero_of_bits(dst[0, pl.ds(dst_row + zero8, 8), pl.ds(gs[0] * _G, _G)])
        return dep

    g_home = {(0, 0): 6, (0, 1): 2, (1, 0): 1, (1, 1): 5}

    def staged(stage, part):
        return _unpack(stage[...] if part is None else stage[pl.ds(part * hs // 2, hs // 2), :])

    def k_job(stage, c, first=False, part=None):
        p = _phi(_dot(staged(stage, part), wk_v[:, cols(c)]))
        zs = jnp.sum(p.reshape(p.shape[0] // 8, 8, _CB), axis=0)
        if first:
            z_v[:, cols(c)] = zs
        else:
            z_v[:, cols(c)] += zs
        return p.astype(_BF16)

    def g_job(pk, stage, c, first=False, part=None):
        upd = _dot_tn(pk, staged(stage, part))
        a, j = divmod(c, n_sl)
        halves = [upd[:, :hd], upd[:, hd:]]
        if a == 1:
            assert first
            halves[1] = halves[1] + halves[0] - gm_v[g_home[0, 1], cols(j), :]
        for b in range(2):
            if first:
                gm_v[g_home[a, b], cols(j), :] = halves[b]
            else:
                gm_v[g_home[a, b], cols(j), :] += halves[b]

    def store_tr(blocks, j):
        n = blocks[0].shape[0]
        for b, v in enumerate(_seven(*blocks)):
            tr_v.at[b][:, pl.ds(j * _CB, n)] = _pack(v.astype(_BF16).T)
        return zero_of_bits(tr_v[0, pl.ds(zero8, 8), pl.ds(0, _G)])

    def kg_strassen(cur, pin, side, fresh=()):
        n = cur(0).shape[0]
        pins = []
        for j in range(n_sl):
            def prod(m):
                p = _dot(cur(_A_IDX[m]), _unpack(wks_v[_B_IDX[m], :, cols(j)]))
                if pin is not None and m == 1:
                    p = p + jnp.concatenate([pin[0:1, :]] * (_CB // _G), axis=1)
                return p

            p11, p12, p21, p22 = map(_phi, _strassen(prod))
            z_v[:, cols(j)] += jnp.sum((p11 + p21).reshape(n // 8, 8, _CB), axis=0)
            z_v[:, cols(n_sl + j)] += jnp.sum((p12 + p22).reshape(n // 8, 8, _CB), axis=0)
            pin = store_tr((p11, p21, p12, p22), j)
            pins.append(pin)
        side(pins)
        for j in range(n_sl):
            for m in range(7):
                upd = _dot(_unpack(tr_v[_A_IDX[m], :, pl.ds(j * _CB, n)]), cur(_B_IDX[m]))
                if m in fresh:
                    gm_v[m, cols(j), :] = upd
                else:
                    gm_v[m, cols(j), :] += upd

    def wk_load(j0):
        return lambda a, b, j, g: wk_v[pl.ds(a * hd + (j0 + j) * 16, 16), pl.ds(b * hd + g * _G, _G)]

    n_wu = hd // 16
    zero_v = jnp.zeros((8, _G), _F32)
    wait("x0a")
    ln_plain(0, _SUB // 2, sb_v, 16, False)
    wait("k0")
    p0a = k_job(sb_v, 0, True, part=0)
    wait("x0b")
    ln_plain(_SUB // 2, _SUB // 2, sb_v, 16, False)
    g_job(p0a, sb_v, 0, True, part=0)
    p0b = k_job(sb_v, 0, part=1)
    wait("k1")
    gps = _CB // _G
    seven_rows(wk_load(0), wks_v, 0, n_wu, zero_v, range(0, gps))
    p2 = k_job(sb_v, 2, True)
    g_job(p0b, sb_v, 0, part=1)
    g_job(p2, sb_v, 2, True)
    wait("k2x1")
    ln_pair(1, xh_v, zero_v, half=_SUB // 2, full=False)
    p1 = k_job(sb_v, 1, True)
    p3 = k_job(sb_v, 3, True)
    after_p3 = zero_like(p3[_SUB - 16:, _CB - _G:].astype(_F32)[8:])
    seven_rows(wk_load(0), wks_v, 0, n_wu, after_p3, range(gps, 2 * gps))
    g_job(p1, sb_v, 1, True)
    g_job(p3, sb_v, 3, True)
    wait("x23")
    kg_strassen(lambda b: _unpack(xh_v[b]), None,
                lambda pins: ln_pair(1, xs_v.at[0], pins[0], stages=_STAGES3), fresh=(0, 3, 4))
    wait("x45q")

    def phase1(i, carry):
        @pl.when(i == 1)
        def _():
            wait("x67")

        win = xs_v.at[pl.ds(i, 2)]
        cur = lambda b: _unpack(win[0, b, :, hcols])

        for u in range(2):
            s = jnp.minimum(2 * i + u, hd // _G - 1)
            for b in range(2):
                f0 = pl.multiple_of(b * hd + s * _G, _G)
                for c in range(n_cb):
                    wqt_v[u, b, :, cols(c)] = _pack(wq_v[cols(c), pl.ds(f0, _G)].T)
        wq_pin = zero_of_bits(wqt_v[0, 0, pl.ds(zero8, 8), pl.ds(0, _G)])
        dep = zero_v
        for u in range(2):
            s = jnp.minimum(2 * i + u, hd // _G - 1)
            load = lambda a, b, j, g, u=u: _unpack(
                wqt_v[u, b, pl.ds(pl.multiple_of(j * 8 + zero8, 8), 8), pl.ds(a * hd + g * _G, _G)])
            dep = seven_rows(load, wqs_v, pl.multiple_of(s * (_G // 2), _G // 2), _G // 16, dep)
        kg_strassen(cur, wq_pin, lambda pins: ln_pair((i + 2) & (n_pair - 1), win.at[1], pins[-1]))
        return carry

    jax.lax.fori_loop(0, n_pair - 1, phase1, 0)
    wait("vo")

    key = pltpu.bitcast(jnp.max(best_v[...], axis=0, keepdims=True), jnp.int32)
    rmax = pltpu.bitcast(key & jnp.int32(-65536), _F32)
    idx = (S - 1) - jnp.max(key & (S - 1))
    idx_pair = idx // (2 * _SUB)
    gate_r = jax.nn.sigmoid(rmax)

    xs = x_v[pl.ds(pl.multiple_of((idx >> 4) * 16, 16), 16), :].astype(_F32)
    m, rstd = ln_stats(xs, None, False)[:2]
    xs = ((xs - m) * rstd).astype(_BF16).astype(_F32)
    sel = jax.lax.broadcasted_iota(jnp.int32, (16, D), 0) == (idx & 15)
    xs = jnp.sum(jnp.where(sel, xs, 0.0), axis=0, keepdims=True)
    for g in range(n_groups):
        xcol_v[pl.ds(g * _G, _G), :] = _col_bcast(xs[:, gsl(g)])
    res_row = pl.ds(pl.multiple_of((idx >> 4) * 8, 8), 8)
    for g in range(n_groups):
        z = jnp.sum(z_v[:, pl.ds(g * _G, _G)], axis=0, keepdims=True)
        zcol_v[pl.ds(g * _G, _G), :] = _col_bcast(z)

    rr = jax.lax.broadcasted_iota(jnp.int32, (_G, _G), 0) // dh
    cc = jax.lax.broadcasted_iota(jnp.int32, (_G, _G), 1) // dh
    same_head = rr == cc
    n_hg = hd // _G
    kvb = {}
    col_pins = {2: zero_like(zcol_v[pl.ds(zero8, 1), :]), 3: zero_like(xcol_v[pl.ds(zero8, 1), :])}

    def kv_job(g):
        gm = lambda m: gm_v[m, pl.ds((g % n_hg) * _G, _G), :]
        if g < n_hg:
            row = [gm(0) + gm(3) - gm(4) + gm(6), gm(2) + gm(4)]
        else:
            row = [gm(1) + gm(3), gm(0) - gm(1) + gm(2) + gm(5)]
        kv = _dot(jnp.concatenate(row, axis=1).astype(_BF16), wv_v[:, pl.ds(g * _G, _G)])
        if g in col_pins:
            kv = kv + col_pins[g]
        kvb[g] = jnp.where(same_head, kv, 0.0).astype(_BF16)

    def m_job(g):
        top, bot = [_dot(kvb.pop(q), wo_v[pl.ds(q * _G, _G), dcols]) for q in (g, g + n_hg)]
        for b, v in enumerate(_seven(top[:, :hd], top[:, hd:], bot[:, :hd], bot[:, hd:])):
            ms_v.at[b][pl.ds(g * _G // 2, _G // 2), :] = _pack(v.astype(_BF16))

    for g in range(n_hg):
        kv_job(g)
        kv_job(g + n_hg)
        if g > 0:
            m_job(g - 1)
    m_job(n_hg - 1)
    wait("f0")

    def chain_matvec(w_ref, lead, cb, col_ref, acc0):
        n = col_ref.shape[0] // 8
        acc = [acc0[:, :_G], acc0[:, _G:]]
        link = None
        for k0 in range(0, n, _BLK):
            rows = pl.ds(k0 * 8, _BLK * 8)
            w = w_ref[lead, rows, cols(cb)].astype(_F32)
            colv = col_ref[rows, :]
            for h in range(2):
                prod = (w[:, h * _G:(h + 1) * _G] * colv).reshape(_BLK, 8, _G)
                first = acc[h] if link is None else acc[h] + link
                acc[h] = jnp.sum(jnp.concatenate([first[None], prod], axis=0), axis=0)
                link = zero_like(acc[h])
        return jnp.concatenate(acc, axis=1)

    def phase2(i, carry):
        @pl.when(i == 1)
        def _():
            wait("f1")

        slot = (idx_pair + i) & (n_pair - 1)
        pair = (slot + 1) & (n_pair - 1)
        prows = pl.ds(pl.multiple_of(pair * (2 * _SUB), 2 * _SUB), 2 * _SUB)
        out_w, hbm_w = out_v.at[prows], out_hbm.at[prows]
        res_w = res_v.at[pl.ds(pl.multiple_of(pair * _SUB, _SUB), _SUB)]
        win = xs_v.at[slot]
        cur = lambda b: _unpack(win[b, :, hcols])

        ys, accs, pins = [], [], {}
        n_gu = 2 * fc // _CB

        def ffn_part(first, last, dep):
            for n in range(first, last):
                if n < n_cb:
                    ys.append(chain_matvec(wd_v, jnp.maximum(i - 1, 0), n, hcol_v, y_v[:, cols(n)] + dep))
                    dep = zero_link(ys[-1])
                else:
                    accs.append(chain_matvec(gu_v, jnp.minimum(i, n_fc - 1), n - n_cb, xcol_v, dep))
                    dep = zero_link(accs[-1])
            return dep

        def normalise(p, c):
            zc = jnp.concatenate([zcol_v[cols(c), :]] * (_SUB // _G), axis=1)
            p3 = p.reshape(_CB // dh, dh, _SUB)
            den = jnp.sum(p3 * zc.reshape(_CB // dh, dh, _SUB), axis=1, keepdims=True) + _DEN_EPS
            return (p3 * pl.reciprocal(den, approx=True)).reshape(_CB, _SUB)

        def qs_job(j, pin):
            def prod(m):
                p = _dot_nt(_unpack(wqs_v[_B_IDX[m], pl.ds(j * _CB // 2, _CB // 2), :]), cur(_A_IDX[m]))
                if (j, m) in pins:
                    p = p + pins[j, m]
                return p + pin if pin is not None and m == 4 else p

            p11, p12, p21, p22 = map(_phi, _strassen(prod))
            o = [normalise(p11, j), normalise(p12, n_sl + j), normalise(p21, j), normalise(p22, n_sl + j)]
            return jnp.concatenate([store_tr(o, j)] * (_CB // _G), axis=1)


        def finish(cs, j):
            order = (1, 3, 2, 0)
            for q in order:
                t, b = divmod(q, 2)
                c = b * n_sl + j
                rows = pl.ds(t * _SUB, _SUB)
                res = cs[q] + _unpack(res_w[pl.ds(t * hs, hs), cols(c)]).astype(_F32)
                out_w[rows, cols(c)] = res.astype(_BF16)
                pltpu.make_async_copy(out_w.at[rows, cols(c)], hbm_w.at[rows, cols(c)], sem_o).start()

        wide = lambda d: jnp.concatenate([d] * (_CB // _G), axis=1)
        h = h_v[...].astype(_BF16).astype(_F32)
        for f in range(fc // _G):
            hcol_v[pl.ds(f * _G, _G), :] = _col_bcast(h[:, gsl(f)])
        dep = ffn_part(0, 2, wide(zero_like(hcol_v[pl.ds(zero8, 8), :])))
        pins[0, 6] = dep[0:1, :]
        rel = qs_job(0, None)
        dep = ffn_part(2, n_cb, dep + rel)
        pins[1, 6] = dep[0:1, :]
        qs_job(1, rel[0:1, :])
        ffn_part(n_cb, n_cb + n_gu, dep)

        yacc = jnp.concatenate(ys, axis=1)
        y_v[...] = yacc
        yrow = jnp.sum(yacc, axis=0, keepdims=True) * gate_r
        hit = jax.lax.broadcasted_iota(jnp.int32, (16, D), 0) == jnp.where(i == n_pair - 1, idx & 15, -1)
        upd = _unpack(res_v[res_row, :]).astype(_F32) + jnp.where(hit, yrow, 0.0)
        res_v[res_row, :] = _pack(upd.astype(_BF16))
        gu = jnp.sum(jnp.concatenate(accs, axis=1), axis=0, keepdims=True)
        g, u = gu[:, :fc], gu[:, fc:]
        hnext = (g * jax.nn.sigmoid(g) * u).astype(_BF16).astype(_F32)
        lane = jax.lax.broadcasted_iota(jnp.int32, (1, fc), 1)
        h_v[...] = jnp.where(lane < jnp.where(i > 0, f_dup, 0), 0.0, hnext)

        for j in range(n_sl):
            cs = _strassen_late22(lambda m: _dot(_unpack(tr_v[_A_IDX[m]]), _unpack(ms_v[_B_IDX[m], :, cols(j)])))
            finish(cs, j)
        return carry

    jax.lax.fori_loop(0, n_pair, phase2, 0)
    pltpu.make_async_copy(out_v, out_hbm, sem_o).wait()


@jax.jit
def pallas_parallel_sum__linear_attn_block__moe_arch_mod__prompt_kernel(
    A_x: jax.Array,
    A_wqkv: jax.Array,
    A_wo: jax.Array,
    B_x: jax.Array,
    B_w_r: jax.Array,
    B_w_gate: jax.Array,
    B_w_up: jax.Array,
    B_w_down: jax.Array,
):
    del B_x
    B, S, D = A_x.shape
    assert B == 1
    F = B_w_gate.shape[1]
    n_pair = S // _SUB // 2
    n_fc = n_pair - 1
    fc = _ffn_chunks(F, n_fc)[0]
    hd = D // 2
    any_spec = pl.BlockSpec(memory_space=pl.ANY)
    out = pl.pallas_call(
        functools.partial(_kernel, S=S, D=D, F=F),
        out_shape=jax.ShapeDtypeStruct((S, D), A_x.dtype),
        in_specs=[any_spec] * 7,
        out_specs=any_spec,
        scratch_shapes=[
            pltpu.VMEM((S, D), _BF16),
            pltpu.VMEM((D, D + _PAD), _BF16),
            pltpu.VMEM((D, D + _PAD), _BF16),
            pltpu.VMEM((D, D + _PAD), _BF16),
            pltpu.VMEM((D, D + _PAD), _BF16),
            pltpu.VMEM((D // _G, _G), _BF16),
            pltpu.VMEM((n_fc, D, 2 * fc), _BF16),
            pltpu.VMEM((n_fc, fc, D + _PAD), _BF16),
            pltpu.VMEM((7, _SUB // 4, hd), _U32),
            pltpu.VMEM((_SUB // 2, D), _U32),
            pltpu.VMEM((n_pair, 7, _SUB // 2, hd + _PAD), _U32),
            pltpu.VMEM((S // 2, D), _U32),
            pltpu.VMEM((7, hd // 2, hd), _U32),
            pltpu.VMEM((2, 2, _G // 2, D), _U32),
            pltpu.VMEM((7, hd // 2, hd), _U32),
            pltpu.VMEM((7, hd, hd), _F32),
            pltpu.VMEM((8, D), _F32),
            pltpu.VMEM((8, 1), _F32),
            pltpu.VMEM((D, _G), _F32),
            pltpu.VMEM((D, _G), _F32),
            pltpu.VMEM((1, fc), _F32),
            pltpu.VMEM((fc, _G), _F32),
            pltpu.VMEM((8, D), _F32),
            pltpu.VMEM((7, _SUB // 2, hd), _U32),
            pltpu.VMEM((7, hd // 2, hd), _U32),
            pltpu.VMEM((S, D), _BF16),
            pltpu.SemaphoreType.DMA((11,)),
            pltpu.SemaphoreType.DMA,
            pltpu.SemaphoreType.REGULAR,
        ],
        compiler_params=pltpu.CompilerParams(
            vmem_limit_bytes=110 * 1024 * 1024,
            disable_bounds_checks=not _RUNTIME_CHECKS,
            disable_semaphore_checks=not _RUNTIME_CHECKS,
        ),
    )(A_x.reshape(S, D), A_wqkv, A_wo, B_w_r.reshape(D // _G, _G), B_w_gate, B_w_up, B_w_down)
    return out.reshape(B, S, D)
```

```python
import functools

import jax
import jax.numpy as jnp
import jax.experimental.pallas as pl
import jax.experimental.pallas.tpu as pltpu

_H = 32
_LN_EPS = 1e-5
_PHI_EPS = 1e-6
_DEN_EPS = 1e-6
_SUB = 256
_CB = 256
_G = 128
_BLK = 16
_PAD = 128

_RUNTIME_CHECKS = False

_F32 = jnp.float32
_BF16 = jnp.bfloat16
_U32 = jnp.uint32


def _dot(a, b):
    return jnp.dot(a, b, preferred_element_type=_F32)


def _dot_tn(a, b):
    return jax.lax.dot_general(a, b, (((0,), (0,)), ((), ())), preferred_element_type=_F32)


def _dot_nt(a, b):
    return jax.lax.dot_general(a, b, (((1,), (1,)), ((), ())), preferred_element_type=_F32)


def _phi(t):
    return jnp.where(t > 0, t + 1.0, jnp.exp(t)) + _PHI_EPS


def _pack(v):
    return pltpu.bitcast(v, _U32)


def _unpack(v):
    return pltpu.bitcast(v, _BF16)


def _col_bcast(row):
    return jnp.broadcast_to(row, (_G, _G)).T


_A_IDX = (2, 3, 0, 1, 4, 5, 6)
_B_IDX = (2, 0, 6, 5, 1, 4, 3)


def _seven(a11, a12, a21, a22):
    return [a11, a22, a11 + a22, a21 + a22, a11 + a12, a21 - a11, a12 - a22]


_SEVEN = (
    lambda a: a[0, 0],
    lambda a: a[1, 1],
    lambda a: a[0, 0] + a[1, 1],
    lambda a: a[1, 0] + a[1, 1],
    lambda a: a[0, 0] + a[0, 1],
    lambda a: a[1, 0] - a[0, 0],
    lambda a: a[0, 1] - a[1, 1],
)
_STAGES3 = ((((0, 0), (1, 1)), (0, 1, 2)), (((0, 1),), (4, 6)), (((1, 0),), (3, 5)))
_STAGES = ((((0, 0),), (0,)), (((1, 1),), (1, 2)), (((0, 1),), (4, 6)), (((1, 0),), (3, 5)))


def _add(a, b):
    return tuple(x + y for x, y in zip(a, b)) if isinstance(a, tuple) else a + b


def _sub(a, b):
    return tuple(x - y for x, y in zip(a, b)) if isinstance(a, tuple) else a - b


def _strassen(prod):
    m1 = prod(0)
    m4 = prod(3)
    c11 = _add(m1, m4)
    m2 = prod(1)
    c21 = _add(m2, m4)
    c22 = _sub(m1, m2)
    m5 = prod(4)
    c11 = _sub(c11, m5)
    c11 = _add(c11, prod(6))
    m3 = prod(2)
    c12 = _add(m3, m5)
    c22 = _add(c22, m3)
    c22 = _add(c22, prod(5))
    return c11, c12, c21, c22


def _seven2(blk, a):
    sub = {}
    for a2 in range(2):
        for b2 in range(2):
            sub[a2, b2] = _SEVEN[a](_Lazy(lambda A, B: blk(A, B, a2, b2)))
    return sub


class _Lazy:
    def __init__(self, f):
        self._f = f

    def __getitem__(self, k):
        return self._f(*k)


def _strassen_late22(prod):
    m6 = prod(5)
    m3 = prod(2)
    c22 = m6 + m3
    m5 = prod(4)
    c12 = m3 + m5
    m1 = prod(0)
    c11 = m1 - m5
    c22 = c22 + m1
    m2 = prod(1)
    c22 = c22 - m2
    m4 = prod(3)
    c21 = m2 + m4
    c11 = c11 + m4
    c11 = c11 + prod(6)
    return c11, c12, c21, c22


def _ffn_chunks(F, n):
    nb = F // _G
    per = -(-nb // n)
    step = (nb - per) // (n - 1)
    assert step * (n - 1) == nb - per
    return per * _G, [j * step * _G for j in range(n)], (per - step) * _G


def _kernel(x_hbm, wqkv_hbm, wo_hbm, wr_hbm, wg_hbm, wu_hbm, wd_hbm, out_hbm,
            x_v, wq_v, wk_v, wv_v, wo_v, wr_v, gu_v, wd_v,
            xh_v, sb_v, xs_v, x2_v, res_v, wks_v, wqt_v, wq2_v, gm_v, z_v, best_v,
            zcol_v, xcol_v, h_v, hcol_v, y_v, tr_v, ms_v, out_v,
            sem_i, sem_o, sem_b, *, S, D, F):
    n_sub = S // _SUB
    n_cb = D // _CB
    n_groups = D // _G
    dh = D // _H
    n_pair = n_sub // 2
    n_fc = n_pair - 1
    fc, f_start, f_dup = _ffn_chunks(F, n_fc)
    hs = _SUB // 2
    hd = D // 2
    n_sl = hd // _CB

    cols = lambda c: pl.ds(c * _CB, _CB)
    dcols = pl.ds(0, D)
    hcols = pl.ds(0, hd)
    gsl = lambda g: slice(g * _G, (g + 1) * _G)

    def x_cp(a, b, s):
        sl = pl.ds(int(a * _SUB), int((b - a) * _SUB))
        return pltpu.make_async_copy(x_hbm.at[sl, :], x_v.at[sl, :], sem_i.at[s])

    def k_cp(a, b, s):
        return pltpu.make_async_copy(wqkv_hbm.at[:, pl.ds(D + a * _CB, (b - a) * _CB)],
                                     wk_v.at[:, pl.ds(a * _CB, (b - a) * _CB)], sem_i.at[s])

    def gu_cps(j, s):
        src = pl.ds(f_start[j], fc)
        return [pltpu.make_async_copy(wg_hbm.at[:, src], gu_v.at[j, :, pl.ds(0, fc)], sem_i.at[s]),
                pltpu.make_async_copy(wu_hbm.at[:, src], gu_v.at[j, :, pl.ds(fc, fc)], sem_i.at[s])]

    def d_cp(j, s):
        return pltpu.make_async_copy(wd_hbm.at[pl.ds(f_start[j], fc), :], wd_v.at[j, :, dcols], sem_i.at[s])

    groups = dict(
        x0a=[x_cp(0, 0.5, 0)],
        k0=[k_cp(0, 1, 1)],
        x0b=[x_cp(0.5, 1, 2)],
        k1=[k_cp(2, 3, 3)],
        k2x1=[k_cp(1, 2, 4), k_cp(3, 4, 4), x_cp(1, 2, 4)],
        x23=[x_cp(2, 4, 5), pltpu.make_async_copy(wr_hbm, wr_v, sem_i.at[5])],
        x45q=[x_cp(4, 6, 6),
              pltpu.make_async_copy(wqkv_hbm.at[:, pl.ds(0, D)], wq_v.at[:, dcols], sem_i.at[6])],
        x67=[x_cp(6, n_sub, 7)],
        vo=[pltpu.make_async_copy(wqkv_hbm.at[:, pl.ds(2 * D, D)], wv_v.at[:, dcols], sem_i.at[8]),
            pltpu.make_async_copy(wo_hbm, wo_v.at[:, dcols], sem_i.at[8])],
        f0=gu_cps(0, 9) + [d_cp(0, 9)],
        f1=sum([gu_cps(j, 10) + [d_cp(j, 10)] for j in range(1, n_fc)], []),
    )

    for grp in groups.values():
        for cp in grp:
            cp.start()
            pl.semaphore_signal(sem_b, 1)
            pl.semaphore_wait(sem_b, 1)

    def wait(name):
        for cp in groups[name]:
            cp.wait()

    zero = pl.semaphore_read(sem_b)
    zero8 = pl.multiple_of(zero * 8, 8)
    zero_u = zero.astype(_U32)

    def zero_of_bits(u):
        return pltpu.bitcast(u & zero_u, _F32)

    def zero_like(v):
        return zero_of_bits(pltpu.bitcast(v, _U32))

    def zero_link(v):
        d = pltpu.bitcast(v, _U32)
        d = zero_of_bits(d[:, :_G] | d[:, _G:])
        return jnp.concatenate([d, d], axis=1)

    def rep(d, n):
        return jnp.concatenate([d] * n, axis=0)

    h_v[...] = jnp.zeros_like(h_v)
    y_v[...] = jnp.zeros_like(y_v)
    best_v[...] = jnp.full(best_v.shape, -jnp.inf, _F32)

    def lane_partial(terms, dep):
        acc = terms[0] if dep is None else dep + terms[0]
        for t in terms[1:]:
            acc = acc + t
        return acc

    def ln_stats(x, dep, throttle, wr=None):
        s1 = lane_partial([x[:, gsl(g)] for g in range(n_groups)], dep)
        s2 = lane_partial([x[:, gsl(g)] * x[:, gsl(g)] for g in range(n_groups)],
                          zero_like(s1) if throttle else None)
        m = jnp.sum(s1, axis=-1, keepdims=True) * (1.0 / D)
        ex2 = jnp.sum(s2, axis=-1, keepdims=True) * (1.0 / D)
        rstd = jnp.exp2(-0.5 * jnp.log2(jnp.maximum(ex2 - m * m, 0.0) + _LN_EPS))
        if wr is None:
            return m, rstd, None, zero_like(s2)
        s3 = lane_partial([x[:, gsl(g)] * wr[0][:, gsl(g)] for g in range(n_groups)], zero_like(s2))
        r = (jnp.sum(s3, axis=-1, keepdims=True) - m * wr[1]) * rstd
        r = r.astype(_BF16).astype(_F32)
        return m, rstd + zero_like(r), r, zero_like(s3)

    def ln_plain(row0, n_rows, stage, rows, throttle):
        for j in range(n_rows // rows):
            r0 = row0 + j * rows
            s0 = (r0 % _SUB) // 2
            x = x_v[pl.ds(r0, rows), :].astype(_F32)
            dep = None
            if throttle and j > 0:
                dep = rep(zero_of_bits(stage[pl.ds(zero8, 8), pl.ds(0, _G)]), rows // 8)
            m, rstd = ln_stats(x, dep, throttle)[:2]
            mb = jnp.broadcast_to(m, (rows, _G))
            for c in range(n_cb):
                xc = x_v[pl.ds(pl.multiple_of(r0 + zero * rows, rows), rows), cols(c)].astype(_F32)
                xn = _pack(((xc - jnp.concatenate([mb] * (_CB // _G), axis=1)) * rstd).astype(_BF16))
                stage[pl.ds(s0, rows // 2), cols(c)] = xn
                if throttle and c + 1 < n_cb:
                    mb = mb + rep(zero_of_bits(stage[pl.ds(zero8, 8), pl.ds(0, _G)]), rows // 8)

    sub_iota = jax.lax.broadcasted_iota(jnp.int32, (8, 1), 0)

    def ln_pair(pair, dst, dep, half=_SUB, full=True, stages=_STAGES):
        wr = None
        if full:
            wr8 = wr_v[...].astype(_F32)
            wr = jnp.concatenate([wr8[g:g + 1, :] for g in range(n_groups)], axis=1)
            wr = (wr, jnp.sum(wr, axis=-1, keepdims=True))
            best = best_v[...]
        n_u = half // 16
        base = pair * (2 * half)
        x1 = x_v.at[pl.ds(pl.multiple_of(base, 2 * half), 2 * half)]
        x2 = x_v.at[pl.ds(pl.multiple_of(base + zero * 16, 16), 2 * half)]
        res = res_v.at[pl.ds(pl.multiple_of(pair * half, half), half)]
        rev_iota = ((S - 1 - base) - sub_iota).astype(_U32)
        r0 = [[t * half + j * 16 for t in range(2)] for j in range(n_u)]
        st = {}
        for j in range(-1, n_u):
            if j + 1 < n_u:
                d = dep
                for t in range(2):
                    x = x1[pl.ds(r0[j + 1][t], 16), :].astype(_F32)
                    ms, rs = [], []
                    for q in range(2):
                        m, rstd, r, d = ln_stats(x[q * 8:(q + 1) * 8], d, True, wr)
                        ms.append(jnp.broadcast_to(m, (8, _G)))
                        rs.append(jnp.broadcast_to(rstd, (8, _G)))
                        if full:
                            key = pltpu.bitcast(r, _U32) | (rev_iota - (r0[j + 1][t] + q * 8))
                            best = jnp.maximum(best, pltpu.bitcast(key, _F32))
                    st[j + 1, t] = (jnp.concatenate(ms, axis=0), jnp.concatenate(rs, axis=0))
            if j < 0:
                continue
            for g in range(hd // _G):
                xn = {}
                for blocks, outs in stages:
                    for t, h in blocks:
                        csl = pl.ds(h * hd + g * _G, _G)
                        xc = x2[pl.ds(r0[j][t], 16), csl].astype(_F32)
                        mb = st[j, t][0]
                        mb = jnp.concatenate([mb[:8] + dep, mb[8:]], axis=0)
                        xn[t, h] = (xc - mb) * st[j, t][1]
                        if full:
                            res[pl.ds(r0[j][t] // 2, 8), csl] = _pack((xc + xn[t, h]).astype(_BF16))
                    for b in outs:
                        dst.at[b][pl.ds(j * 8, 8), pl.ds(g * _G, _G)] = _pack(_SEVEN[b](xn).astype(_BF16))
                    dep = zero_of_bits(dst[0, pl.ds(zero8, 8), pl.ds(0, _G)])
        if full:
            best_v[...] = best
        return dep

    def seven_rows(load, dst, dst_row, n_units, dep, gs=range(hd // _G)):
        for j in range(n_units):
            for g in gs:
                w = {(a, b): load(a, b, j, g).astype(_F32) for a in range(2) for b in range(2)}
                for gate, outs in (((0, 0), (0, 1, 2, 4)), ((1, 0), (3, 5, 6))):
                    w[gate] = jnp.concatenate([w[gate][:8] + dep, w[gate][8:]], axis=0)
                    for b in outs:
                        dst.at[b][pl.ds(dst_row + j * 8, 8), pl.ds(g * _G, _G)] = _pack(_SEVEN[b](w).astype(_BF16))
                    dep = zero_of_bits(dst[0, pl.ds(dst_row + zero8, 8), pl.ds(gs[0] * _G, _G)])
        return dep

    qd = D // 4

    def level2_rows(blk, dst, dst_row, n_units, dep, first, groups=range(7), stages=2):
        n_out = 7 - first
        plan = (((0, 0), (0, 1, 2, 4)), ((1, 0), (3, 5, 6))) if stages == 2 else (((0, 0), range(7)),)
        for a in groups:
            for j in range(n_units):
                for g in range(qd // _G):
                    w = blk(a, j, g)
                    for gate, outs in plan:
                        w[gate] = jnp.concatenate([w[gate][:8] + dep, w[gate][8:]], axis=0)
                        for b in outs:
                            if b >= first:
                                dst.at[a * n_out + b - first][pl.ds(dst_row + j * 8, 8), pl.ds(g * _G, _G)] = (
                                    _pack(_SEVEN[b](w).astype(_BF16)))
                        dep = zero_of_bits(dst[a * n_out, pl.ds(dst_row + zero8, 8), pl.ds(0, _G)])
        return dep

    def xn_level2(src, dst, dep, stages=2):
        blk = lambda a, j, g: {
            (a2, b2): _unpack(src[a, pl.ds(a2 * (hs // 2) + j * 8, 8), pl.ds(b2 * qd + g * _G, _G)]).astype(_F32)
            for a2 in range(2) for b2 in range(2)}
        return level2_rows(blk, dst, 0, _SUB // 32, dep, 2, stages=stages)

    g_home = {(0, 0): 6, (0, 1): 2, (1, 0): 1, (1, 1): 5}

    def staged(stage, part):
        return _unpack(stage[...] if part is None else stage[pl.ds(part * hs // 2, hs // 2), :])

    def k_job(stage, c, first=False, part=None):
        p = _phi(_dot(staged(stage, part), wk_v[:, cols(c)]))
        zs = jnp.sum(p.reshape(p.shape[0] // 8, 8, _CB), axis=0)
        if first:
            z_v[:, cols(c)] = zs
        else:
            z_v[:, cols(c)] += zs
        return p.astype(_BF16)

    def g_job(pk, stage, c, first=False, part=None):
        upd = _dot_tn(pk, staged(stage, part))
        a, j = divmod(c, n_sl)
        halves = [upd[:, :hd], upd[:, hd:]]
        if a == 1:
            assert first
            halves[1] = halves[1] + halves[0] - gm_v[g_home[0, 1], cols(j), :]
        for b in range(2):
            if first:
                gm_v[g_home[a, b], cols(j), :] = halves[b]
            else:
                gm_v[g_home[a, b], cols(j), :] += halves[b]

    def store_tr(blocks, j):
        n = blocks[0].shape[0]
        for b, v in enumerate(_seven(*blocks)):
            tr_v.at[b][:, pl.ds(j * _CB, n)] = _pack(v.astype(_BF16).T)
        return zero_of_bits(tr_v[0, pl.ds(zero8, 8), pl.ds(0, _G)])

    def kg_strassen(cur, pin, side, fresh=()):
        n = cur(0).shape[0]
        pins = []
        for j in range(n_sl):
            def prod(m):
                p = _dot(cur(_A_IDX[m]), _unpack(wks_v[_B_IDX[m], :, cols(j)]))
                if pin is not None and m == 1:
                    p = p + jnp.concatenate([pin[0:1, :]] * (_CB // _G), axis=1)
                return p

            p11, p12, p21, p22 = map(_phi, _strassen(prod))
            z_v[:, cols(j)] += jnp.sum((p11 + p21).reshape(n // 8, 8, _CB), axis=0)
            z_v[:, cols(n_sl + j)] += jnp.sum((p12 + p22).reshape(n // 8, 8, _CB), axis=0)
            pin = store_tr((p11, p21, p12, p22), j)
            pins.append(pin)
        side(pins)
        for j in range(n_sl):
            for m in range(7):
                upd = _dot(_unpack(tr_v[_A_IDX[m], :, pl.ds(j * _CB, n)]), cur(_B_IDX[m]))
                if m in fresh:
                    gm_v[m, cols(j), :] = upd
                else:
                    gm_v[m, cols(j), :] += upd

    def wk_load(j0):
        return lambda a, b, j, g: wk_v[pl.ds(a * hd + (j0 + j) * 16, 16), pl.ds(b * hd + g * _G, _G)]

    n_wu = hd // 16
    zero_v = jnp.zeros((8, _G), _F32)
    wait("x0a")
    ln_plain(0, _SUB // 2, sb_v, 16, False)
    wait("k0")
    p0a = k_job(sb_v, 0, True, part=0)
    wait("x0b")
    ln_plain(_SUB // 2, _SUB // 2, sb_v, 16, False)
    g_job(p0a, sb_v, 0, True, part=0)
    p0b = k_job(sb_v, 0, part=1)
    wait("k1")
    gps = _CB // _G
    seven_rows(wk_load(0), wks_v, 0, n_wu, zero_v, range(0, gps))
    p2 = k_job(sb_v, 2, True)
    g_job(p0b, sb_v, 0, part=1)
    g_job(p2, sb_v, 2, True)
    wait("k2x1")
    ln_pair(1, xh_v, zero_v, half=_SUB // 2, full=False)
    p1 = k_job(sb_v, 1, True)
    p3 = k_job(sb_v, 3, True)
    after_p3 = zero_like(p3[_SUB - 16:, _CB - _G:].astype(_F32)[8:])
    seven_rows(wk_load(0), wks_v, 0, n_wu, after_p3, range(gps, 2 * gps))
    g_job(p1, sb_v, 1, True)
    g_job(p3, sb_v, 3, True)
    wait("x23")
    kg_strassen(lambda b: _unpack(xh_v[b]), None,
                lambda pins: ln_pair(1, xs_v.at[0], pins[0], stages=_STAGES3), fresh=(0, 3, 4))
    wait("x45q")

    def phase1(i, carry):
        @pl.when(i == 1)
        def _():
            wait("x67")

        win = xs_v.at[pl.ds(i, 2)]
        cur = lambda b: _unpack(win[0, b, :, hcols])

        sl = jnp.minimum(i, qd // _G - 1)
        for u in range(2):
            for b in range(2):
                f0 = pl.multiple_of(b * hd + u * qd + sl * _G, _G)
                for c in range(n_cb):
                    wqt_v[u, b, :, cols(c)] = _pack(wq_v[cols(c), pl.ds(f0, _G)].T)
        wq_pin = zero_of_bits(wqt_v[0, 0, pl.ds(zero8, 8), pl.ds(0, _G)])
        raw = lambda j, g: (lambda A, B, a2, b2: _unpack(
            wqt_v[b2, B, pl.ds(pl.multiple_of(j * 8 + zero8, 8), 8), pl.ds(A * hd + a2 * qd + g * _G, _G)]).astype(_F32))
        xn_level2(win.at[0], x2_v.at[i], zero_v, stages=1)
        level2_rows(lambda a, j, g: _seven2(raw(j, g), a), wq2_v, pl.multiple_of(sl * (_G // 2), _G // 2),
                    _G // 16, zero_v, 0)
        kg_strassen(cur, wq_pin, lambda pins: ln_pair((i + 2) & (n_pair - 1), win.at[1], pins[-1]))
        return carry

    jax.lax.fori_loop(0, n_pair - 1, phase1, 0)
    wait("vo")

    key = pltpu.bitcast(jnp.max(best_v[...], axis=0, keepdims=True), jnp.int32)
    rmax = pltpu.bitcast(key & jnp.int32(-65536), _F32)
    idx = (S - 1) - jnp.max(key & (S - 1))
    idx_pair = idx // (2 * _SUB)
    gate_r = jax.nn.sigmoid(rmax)

    xs = x_v[pl.ds(pl.multiple_of((idx >> 4) * 16, 16), 16), :].astype(_F32)
    m, rstd = ln_stats(xs, None, False)[:2]
    xs = ((xs - m) * rstd).astype(_BF16).astype(_F32)
    sel = jax.lax.broadcasted_iota(jnp.int32, (16, D), 0) == (idx & 15)
    xs = jnp.sum(jnp.where(sel, xs, 0.0), axis=0, keepdims=True)
    for g in range(n_groups):
        xcol_v[pl.ds(g * _G, _G), :] = _col_bcast(xs[:, gsl(g)])
    res_row = pl.ds(pl.multiple_of((idx >> 4) * 8, 8), 8)
    for g in range(n_groups):
        z = jnp.sum(z_v[:, pl.ds(g * _G, _G)], axis=0, keepdims=True)
        zcol_v[pl.ds(g * _G, _G), :] = _col_bcast(z)

    rr = jax.lax.broadcasted_iota(jnp.int32, (_G, _G), 0) // dh
    cc = jax.lax.broadcasted_iota(jnp.int32, (_G, _G), 1) // dh
    same_head = rr == cc
    n_hg = hd // _G
    kvb = {}
    col_pins = {2: zero_like(zcol_v[pl.ds(zero8, 1), :]), 3: zero_like(xcol_v[pl.ds(zero8, 1), :])}

    def kv_job(g):
        gm = lambda m: gm_v[m, pl.ds((g % n_hg) * _G, _G), :]
        if g < n_hg:
            row = [gm(0) + gm(3) - gm(4) + gm(6), gm(2) + gm(4)]
        else:
            row = [gm(1) + gm(3), gm(0) - gm(1) + gm(2) + gm(5)]
        kv = _dot(jnp.concatenate(row, axis=1).astype(_BF16), wv_v[:, pl.ds(g * _G, _G)])
        if g in col_pins:
            kv = kv + col_pins[g]
        kvb[g] = jnp.where(same_head, kv, 0.0).astype(_BF16)

    def m_job(g):
        top, bot = [_dot(kvb.pop(q), wo_v[pl.ds(q * _G, _G), dcols]) for q in (g, g + n_hg)]
        for b, v in enumerate(_seven(top[:, :hd], top[:, hd:], bot[:, :hd], bot[:, hd:])):
            ms_v.at[b][pl.ds(g * _G // 2, _G // 2), :] = _pack(v.astype(_BF16))

    xn_level2(xs_v.at[n_pair - 1], x2_v.at[n_pair - 1], zero_v)
    for g in range(n_hg):
        kv_job(g)
        kv_job(g + n_hg)
        if g > 0:
            m_job(g - 1)
    m_job(n_hg - 1)
    wait("f0")

    def chain_matvec(w_ref, lead, cb, col_ref, acc0):
        n = col_ref.shape[0] // 8
        acc = [acc0[:, :_G], acc0[:, _G:]]
        link = None
        for k0 in range(0, n, _BLK):
            rows = pl.ds(k0 * 8, _BLK * 8)
            w = w_ref[lead, rows, cols(cb)].astype(_F32)
            colv = col_ref[rows, :]
            for h in range(2):
                prod = (w[:, h * _G:(h + 1) * _G] * colv).reshape(_BLK, 8, _G)
                first = acc[h] if link is None else acc[h] + link
                acc[h] = jnp.sum(jnp.concatenate([first[None], prod], axis=0), axis=0)
                link = zero_like(acc[h])
        return jnp.concatenate(acc, axis=1)

    def phase2(i, carry):
        @pl.when(i == 1)
        def _():
            wait("f1")

        slot = (idx_pair + i) & (n_pair - 1)
        pair = (slot + 1) & (n_pair - 1)
        prows = pl.ds(pl.multiple_of(pair * (2 * _SUB), 2 * _SUB), 2 * _SUB)
        out_w, hbm_w = out_v.at[prows], out_hbm.at[prows]
        res_w = res_v.at[pl.ds(pl.multiple_of(pair * _SUB, _SUB), _SUB)]
        win = xs_v.at[slot]
        cur = lambda b: _unpack(win[b, :, hcols])

        ys, accs, pins = [], [], {}
        n_gu = 2 * fc // _CB

        def ffn_part(first, last, dep):
            for n in range(first, last):
                if n < n_cb:
                    ys.append(chain_matvec(wd_v, jnp.maximum(i - 1, 0), n, hcol_v, y_v[:, cols(n)] + dep))
                    dep = zero_link(ys[-1])
                else:
                    accs.append(chain_matvec(gu_v, jnp.minimum(i, n_fc - 1), n - n_cb, xcol_v, dep))
                    dep = zero_link(accs[-1])
            return dep

        x2w = x2_v.at[slot]

        def xop(a, b):
            if b < 2:
                return _unpack(win[a, pl.ds(b * (hs // 2), hs // 2), pl.ds(b * qd, qd)])
            return _unpack(x2w[a * 5 + b - 2])

        def normalise(p, fq):
            p3 = _phi(p).reshape(qd // dh, dh, _G)
            zc = zcol_v[pl.ds(fq * qd, qd), :].reshape(qd // dh, dh, _G)
            den = jnp.sum(p3 * zc, axis=1, keepdims=True) + _DEN_EPS
            return (p3 * pl.reciprocal(den, approx=True)).reshape(qd, _G)

        def q_phase():
            def prod(m1, m2):
                if (m1, m2) in hooks:
                    hooks[m1, m2]()
                p = _dot_nt(_unpack(wq2_v[_B_IDX[m1] * 7 + _B_IDX[m2]]), xop(_A_IDX[m1], _A_IDX[m2]))
                last[0] = p
                return p + pins[m1, m2][:, :_G] if (m1, m2) in pins else p

            q = _strassen(lambda m1: _strassen(lambda m2: prod(m1, m2)))
            for n in (2, 0, 1, 3):
                a2, b2 = divmod(n, 2)
                o = [normalise(q[k][n], 2 * (k % 2) + b2) for k in range(4)]
                for b, v in enumerate(_seven(*o)):
                    tr_v.at[b][pl.ds(a2 * (hs // 2), hs // 2), pl.ds(b2 * qd, qd)] = _pack(v.astype(_BF16).T)

        def finish(cs, j):
            order = (1, 3, 2, 0)
            for q in order:
                t, b = divmod(q, 2)
                c = b * n_sl + j
                rows = pl.ds(t * _SUB, _SUB)
                res = cs[q] + _unpack(res_w[pl.ds(t * hs, hs), cols(c)]).astype(_F32)
                out_w[rows, cols(c)] = res.astype(_BF16)
                pltpu.make_async_copy(out_w.at[rows, cols(c)], hbm_w.at[rows, cols(c)], sem_o).start()

        wide = lambda d: jnp.concatenate([d] * (_CB // _G), axis=1)
        h = h_v[...].astype(_BF16).astype(_F32)
        for f in range(fc // _G):
            hcol_v[pl.ds(f * _G, _G), :] = _col_bcast(h[:, gsl(f)])
        order = (0, 3, 1, 4, 6, 2, 5)
        at = lambda n: (order[n // 7], order[n % 7])
        hooks, last, st = {}, {}, {}
        st["dep"] = ffn_part(0, 3, wide(zero_like(hcol_v[pl.ds(zero8, 8), :])))
        pins[at(20)] = st["dep"][0:1, :]

        def seg2():
            st["dep"] = ffn_part(3, 4, st["dep"] + wide(zero_like(last[0][:8, :])))
            pins[at(32)] = st["dep"][0:1, :]

        hooks[at(22)] = seg2
        q_phase()

        yacc = jnp.concatenate(ys, axis=1)
        y_v[...] = yacc
        yrow = jnp.sum(yacc, axis=0, keepdims=True) * gate_r
        hit = jax.lax.broadcasted_iota(jnp.int32, (16, D), 0) == jnp.where(i == n_pair - 1, idx & 15, -1)
        upd = _unpack(res_v[res_row, :]).astype(_F32) + jnp.where(hit, yrow, 0.0)
        res_v[res_row, :] = _pack(upd.astype(_BF16))
        cnt = [0]

        def oprod(m, j):
            p = _dot(_unpack(tr_v[_A_IDX[m]]), _unpack(ms_v[_B_IDX[m], :, cols(j)]))
            if cnt[0] == 3:
                ffn_part(n_cb, n_cb + n_gu, st["dep"] + wide(zero_like(p[:8, :_G])))
            cnt[0] += 1
            return p

        for j in range(n_sl):
            finish(_strassen_late22(lambda m: oprod(m, j)), j)
        gu = jnp.sum(jnp.concatenate(accs, axis=1), axis=0, keepdims=True)
        g, u = gu[:, :fc], gu[:, fc:]
        hnext = (g * jax.nn.sigmoid(g) * u).astype(_BF16).astype(_F32)
        lane = jax.lax.broadcasted_iota(jnp.int32, (1, fc), 1)
        h_v[...] = jnp.where(lane < jnp.where(i > 0, f_dup, 0), 0.0, hnext)
        return carry

    jax.lax.fori_loop(0, n_pair, phase2, 0)
    pltpu.make_async_copy(out_v, out_hbm, sem_o).wait()


@jax.jit
def pallas_parallel_sum__linear_attn_block__moe_arch_mod__prompt_kernel(
    A_x: jax.Array,
    A_wqkv: jax.Array,
    A_wo: jax.Array,
    B_x: jax.Array,
    B_w_r: jax.Array,
    B_w_gate: jax.Array,
    B_w_up: jax.Array,
    B_w_down: jax.Array,
):
    del B_x
    B, S, D = A_x.shape
    assert B == 1
    F = B_w_gate.shape[1]
    n_pair = S // _SUB // 2
    n_fc = n_pair - 1
    fc = _ffn_chunks(F, n_fc)[0]
    hd = D // 2
    qd = D // 4
    any_spec = pl.BlockSpec(memory_space=pl.ANY)
    out = pl.pallas_call(
        functools.partial(_kernel, S=S, D=D, F=F),
        out_shape=jax.ShapeDtypeStruct((S, D), A_x.dtype),
        in_specs=[any_spec] * 7,
        out_specs=any_spec,
        scratch_shapes=[
            pltpu.VMEM((S, D), _BF16),
            pltpu.VMEM((D, D + _PAD), _BF16),
            pltpu.VMEM((D, D + _PAD), _BF16),
            pltpu.VMEM((D, D + _PAD), _BF16),
            pltpu.VMEM((D, D + _PAD), _BF16),
            pltpu.VMEM((D // _G, _G), _BF16),
            pltpu.VMEM((n_fc, D, 2 * fc), _BF16),
            pltpu.VMEM((n_fc, fc, D + _PAD), _BF16),
            pltpu.VMEM((7, _SUB // 4, hd), _U32),
            pltpu.VMEM((_SUB // 2, D), _U32),
            pltpu.VMEM((n_pair, 7, _SUB // 2, hd + _PAD), _U32),
            pltpu.VMEM((n_pair, 35, _SUB // 4, qd), _U32),
            pltpu.VMEM((S // 2, D), _U32),
            pltpu.VMEM((7, hd // 2, hd), _U32),
            pltpu.VMEM((2, 2, _G // 2, D), _U32),
            pltpu.VMEM((49, qd // 2, qd), _U32),
            pltpu.VMEM((7, hd, hd), _F32),
            pltpu.VMEM((8, D), _F32),
            pltpu.VMEM((8, 1), _F32),
            pltpu.VMEM((D, _G), _F32),
            pltpu.VMEM((D, _G), _F32),
            pltpu.VMEM((1, fc), _F32),
            pltpu.VMEM((fc, _G), _F32),
            pltpu.VMEM((8, D), _F32),
            pltpu.VMEM((7, _SUB // 2, hd), _U32),
            pltpu.VMEM((7, hd // 2, hd), _U32),
            pltpu.VMEM((S, D), _BF16),
            pltpu.SemaphoreType.DMA((11,)),
            pltpu.SemaphoreType.DMA,
            pltpu.SemaphoreType.REGULAR,
        ],
        compiler_params=pltpu.CompilerParams(
            vmem_limit_bytes=120 * 1024 * 1024,
            disable_bounds_checks=not _RUNTIME_CHECKS,
            disable_semaphore_checks=not _RUNTIME_CHECKS,
        ),
    )(A_x.reshape(S, D), A_wqkv, A_wo, B_w_r.reshape(D // _G, _G), B_w_gate, B_w_up, B_w_down)
    return out.reshape(B, S, D)
```

```python
import functools

import jax
import jax.numpy as jnp
import jax.experimental.pallas as pl
import jax.experimental.pallas.tpu as pltpu

_H = 32
_LN_EPS = 1e-5
_PHI_EPS = 1e-6
_DEN_EPS = 1e-6
_SUB = 256
_CB = 256
_G = 128
_BLK = 16
_PAD = 128

_RUNTIME_CHECKS = False

_F32 = jnp.float32
_BF16 = jnp.bfloat16
_U32 = jnp.uint32


def _dot(a, b):
    return jnp.dot(a, b, preferred_element_type=_F32)


def _dot_tn(a, b):
    return jax.lax.dot_general(a, b, (((0,), (0,)), ((), ())), preferred_element_type=_F32)


def _dot_nt(a, b):
    return jax.lax.dot_general(a, b, (((1,), (1,)), ((), ())), preferred_element_type=_F32)


def _phi(t):
    return jnp.where(t > 0, t + 1.0, jnp.exp(t)) + _PHI_EPS


def _pack(v):
    return pltpu.bitcast(v, _U32)


def _unpack(v):
    return pltpu.bitcast(v, _BF16)


def _col_bcast(row):
    return jnp.broadcast_to(row, (_G, _G)).T


_A_IDX = (2, 3, 0, 1, 4, 5, 6)
_B_IDX = (2, 0, 6, 5, 1, 4, 3)


def _seven(a11, a12, a21, a22):
    return [a11, a22, a11 + a22, a21 + a22, a11 + a12, a21 - a11, a12 - a22]


_SEVEN = (
    lambda a: a[0, 0],
    lambda a: a[1, 1],
    lambda a: a[0, 0] + a[1, 1],
    lambda a: a[1, 0] + a[1, 1],
    lambda a: a[0, 0] + a[0, 1],
    lambda a: a[1, 0] - a[0, 0],
    lambda a: a[0, 1] - a[1, 1],
)
_STAGES3 = ((((0, 0), (1, 1)), (0, 1, 2)), (((0, 1),), (4, 6)), (((1, 0),), (3, 5)))
_STAGES = ((((0, 0),), (0,)), (((1, 1),), (1, 2)), (((0, 1),), (4, 6)), (((1, 0),), (3, 5)))


def _add(a, b):
    return tuple(x + y for x, y in zip(a, b)) if isinstance(a, tuple) else a + b


def _sub(a, b):
    return tuple(x - y for x, y in zip(a, b)) if isinstance(a, tuple) else a - b


def _strassen(prod):
    m1 = prod(0)
    m4 = prod(3)
    c11 = _add(m1, m4)
    m2 = prod(1)
    c21 = _add(m2, m4)
    c22 = _sub(m1, m2)
    m5 = prod(4)
    c11 = _sub(c11, m5)
    c11 = _add(c11, prod(6))
    m3 = prod(2)
    c12 = _add(m3, m5)
    c22 = _add(c22, m3)
    c22 = _add(c22, prod(5))
    return c11, c12, c21, c22


def _strassen_even(prod):
    m2 = prod(1)
    m4 = prod(3)
    c21 = _add(m2, m4)
    m3 = prod(2)
    c22 = _sub(m3, m2)
    m5 = prod(4)
    c12 = _add(m3, m5)
    c11 = _sub(m4, m5)
    m1 = prod(0)
    c11 = _add(c11, m1)
    c22 = _add(c22, m1)
    c11 = _add(c11, prod(6))
    c22 = _add(c22, prod(5))
    return c11, c12, c21, c22


_ORD = ((0, 3, 1, 4, 6, 2, 5), (1, 3, 2, 4, 0, 6, 5))


def _seven2(blk, a):
    sub = {}
    for a2 in range(2):
        for b2 in range(2):
            sub[a2, b2] = _SEVEN[a](_Lazy(lambda A, B: blk(A, B, a2, b2)))
    return sub


class _Lazy:
    def __init__(self, f):
        self._f = f

    def __getitem__(self, k):
        return self._f(*k)


def _strassen_late22(prod):
    m6 = prod(5)
    m3 = prod(2)
    c22 = m6 + m3
    m5 = prod(4)
    c12 = m3 + m5
    m1 = prod(0)
    c11 = m1 - m5
    c22 = c22 + m1
    m2 = prod(1)
    c22 = c22 - m2
    m4 = prod(3)
    c21 = m2 + m4
    c11 = c11 + m4
    c11 = c11 + prod(6)
    return c11, c12, c21, c22


def _ffn_chunks(F, n):
    nb = F // _G
    per = -(-nb // n)
    step = (nb - per) // (n - 1)
    assert step * (n - 1) == nb - per
    return per * _G, [j * step * _G for j in range(n)], (per - step) * _G


def _kernel(x_hbm, wqkv_hbm, wo_hbm, wr_hbm, wg_hbm, wu_hbm, wd_hbm, out_hbm,
            x_v, wq_v, wk_v, wv_v, wo_v, wr_v, gu_v, wd_v,
            xh_v, sb_v, xs_v, x2_v, res_v, wks_v, wqt_v, wq2_v, gm_v, z_v, best_v,
            zcol_v, xcol_v, h_v, hcol_v, y_v, tr_v, of_v, ms_v, out_v,
            sem_i, sem_o, sem_b, *, S, D, F):
    n_sub = S // _SUB
    n_cb = D // _CB
    n_groups = D // _G
    dh = D // _H
    n_pair = n_sub // 2
    n_fc = n_pair - 1
    fc, f_start, f_dup = _ffn_chunks(F, n_fc)
    hs = _SUB // 2
    hd = D // 2
    n_sl = hd // _CB

    cols = lambda c: pl.ds(c * _CB, _CB)
    dcols = pl.ds(0, D)
    hcols = pl.ds(0, hd)
    gsl = lambda g: slice(g * _G, (g + 1) * _G)

    def x_cp(a, b, s):
        sl = pl.ds(int(a * _SUB), int((b - a) * _SUB))
        return pltpu.make_async_copy(x_hbm.at[sl, :], x_v.at[sl, :], sem_i.at[s])

    def k_cp(a, b, s):
        return pltpu.make_async_copy(wqkv_hbm.at[:, pl.ds(D + a * _CB, (b - a) * _CB)],
                                     wk_v.at[:, pl.ds(a * _CB, (b - a) * _CB)], sem_i.at[s])

    def gu_cps(j, s):
        src = pl.ds(f_start[j], fc)
        return [pltpu.make_async_copy(wg_hbm.at[:, src], gu_v.at[j, :, pl.ds(0, fc)], sem_i.at[s]),
                pltpu.make_async_copy(wu_hbm.at[:, src], gu_v.at[j, :, pl.ds(fc, fc)], sem_i.at[s])]

    def d_cp(j, s):
        return pltpu.make_async_copy(wd_hbm.at[pl.ds(f_start[j], fc), :], wd_v.at[j, :, dcols], sem_i.at[s])

    groups = dict(
        x0a=[x_cp(0, 0.5, 0)],
        k0=[k_cp(0, 1, 1)],
        x0b=[x_cp(0.5, 1, 2)],
        k1=[k_cp(2, 3, 3)],
        k2x1=[k_cp(1, 2, 4), k_cp(3, 4, 4), x_cp(1, 2, 4)],
        x23=[x_cp(2, 4, 5), pltpu.make_async_copy(wr_hbm, wr_v, sem_i.at[5])],
        x45q=[x_cp(4, 6, 6),
              pltpu.make_async_copy(wqkv_hbm.at[:, pl.ds(0, D)], wq_v.at[:, dcols], sem_i.at[6])],
        x67=[x_cp(6, n_sub, 7)],
        vo=[pltpu.make_async_copy(wqkv_hbm.at[:, pl.ds(2 * D, D)], wv_v.at[:, dcols], sem_i.at[8]),
            pltpu.make_async_copy(wo_hbm, wo_v.at[:, dcols], sem_i.at[8])],
        f0=gu_cps(0, 9) + [d_cp(0, 9)],
        f1=sum([gu_cps(j, 10) + [d_cp(j, 10)] for j in range(1, n_fc)], []),
    )

    for grp in groups.values():
        for cp in grp:
            cp.start()
            pl.semaphore_signal(sem_b, 1)
            pl.semaphore_wait(sem_b, 1)

    def wait(name):
        for cp in groups[name]:
            cp.wait()

    zero = pl.semaphore_read(sem_b)
    zero8 = pl.multiple_of(zero * 8, 8)
    zero_u = zero.astype(_U32)

    def zero_of_bits(u):
        return pltpu.bitcast(u & zero_u, _F32)

    def zero_like(v):
        return zero_of_bits(pltpu.bitcast(v, _U32))

    def zero_link(v):
        d = pltpu.bitcast(v, _U32)
        d = zero_of_bits(d[:, :_G] | d[:, _G:])
        return jnp.concatenate([d, d], axis=1)

    class Clock:
        def __init__(self):
            self.t, self.marks = 0, []

        def mark(self, dt, v):
            self.marks.append((self.t, v[:8, :_G]))
            self.t += dt

        def every(self, t0, period):
            used = set()

            def tick(n):
                if not period:
                    return None
                past = [k for k, (t, _) in enumerate(self.marks) if t <= t0 + n * period]
                if not past or past[-1] in used:
                    return None
                used.add(past[-1])
                return self.marks[past[-1]][1]
            return tick

    no_tick = lambda n: None

    def rep(d, n):
        return jnp.concatenate([d] * n, axis=0)

    h_v[...] = jnp.zeros_like(h_v)
    y_v[...] = jnp.zeros_like(y_v)
    best_v[...] = jnp.full(best_v.shape, -jnp.inf, _F32)

    def lane_partial(terms, dep):
        acc = terms[0] if dep is None else dep + terms[0]
        for t in terms[1:]:
            acc = acc + t
        return acc

    def ln_stats(x, dep, throttle, wr=None):
        s1 = lane_partial([x[:, gsl(g)] for g in range(n_groups)], dep)
        s2 = lane_partial([x[:, gsl(g)] * x[:, gsl(g)] for g in range(n_groups)],
                          zero_like(s1) if throttle else None)
        m = jnp.sum(s1, axis=-1, keepdims=True) * (1.0 / D)
        ex2 = jnp.sum(s2, axis=-1, keepdims=True) * (1.0 / D)
        rstd = jnp.exp2(-0.5 * jnp.log2(jnp.maximum(ex2 - m * m, 0.0) + _LN_EPS))
        if wr is None:
            return m, rstd, None, zero_like(s2)
        s3 = lane_partial([x[:, gsl(g)] * wr[0][:, gsl(g)] for g in range(n_groups)], zero_like(s2))
        r = (jnp.sum(s3, axis=-1, keepdims=True) - m * wr[1]) * rstd
        r = r.astype(_BF16).astype(_F32)
        return m, rstd + zero_like(r), r, zero_like(s3)

    def ln_plain(row0, n_rows, stage, rows, throttle):
        for j in range(n_rows // rows):
            r0 = row0 + j * rows
            s0 = (r0 % _SUB) // 2
            x = x_v[pl.ds(r0, rows), :].astype(_F32)
            dep = None
            if throttle and j > 0:
                dep = rep(zero_of_bits(stage[pl.ds(zero8, 8), pl.ds(0, _G)]), rows // 8)
            m, rstd = ln_stats(x, dep, throttle)[:2]
            mb = jnp.broadcast_to(m, (rows, _G))
            for c in range(n_cb):
                xc = x_v[pl.ds(pl.multiple_of(r0 + zero * rows, rows), rows), cols(c)].astype(_F32)
                xn = _pack(((xc - jnp.concatenate([mb] * (_CB // _G), axis=1)) * rstd).astype(_BF16))
                stage[pl.ds(s0, rows // 2), cols(c)] = xn
                if throttle and c + 1 < n_cb:
                    mb = mb + rep(zero_of_bits(stage[pl.ds(zero8, 8), pl.ds(0, _G)]), rows // 8)

    sub_iota = jax.lax.broadcasted_iota(jnp.int32, (8, 1), 0)

    def ln_pair(pair, dst, dep, half=_SUB, full=True, stages=_STAGES, tick=no_tick):
        wr = None
        if full:
            wr8 = wr_v[...].astype(_F32)
            wr = jnp.concatenate([wr8[g:g + 1, :] for g in range(n_groups)], axis=1)
            wr = (wr, jnp.sum(wr, axis=-1, keepdims=True))
            best = best_v[...]
        n_u = half // 16
        base = pair * (2 * half)
        x1 = x_v.at[pl.ds(pl.multiple_of(base, 2 * half), 2 * half)]
        x2 = x_v.at[pl.ds(pl.multiple_of(base + zero * 16, 16), 2 * half)]
        res = res_v.at[pl.ds(pl.multiple_of(pair * half, half), half)]
        rev_iota = ((S - 1 - base) - sub_iota).astype(_U32)
        r0 = [[t * half + j * 16 for t in range(2)] for j in range(n_u)]
        st = {}
        for j in range(-1, n_u):
            tk = tick(j + 1)
            if tk is not None:
                dep = dep + zero_like(tk)
            if j + 1 < n_u:
                d = dep
                for t in range(2):
                    x = x1[pl.ds(r0[j + 1][t], 16), :].astype(_F32)
                    ms, rs = [], []
                    for q in range(2):
                        m, rstd, r, d = ln_stats(x[q * 8:(q + 1) * 8], d, True, wr)
                        ms.append(jnp.broadcast_to(m, (8, _G)))
                        rs.append(jnp.broadcast_to(rstd, (8, _G)))
                        if full:
                            key = pltpu.bitcast(r, _U32) | (rev_iota - (r0[j + 1][t] + q * 8))
                            best = jnp.maximum(best, pltpu.bitcast(key, _F32))
                    st[j + 1, t] = (jnp.concatenate(ms, axis=0), jnp.concatenate(rs, axis=0))
            if j < 0:
                continue
            for g in range(hd // _G):
                xn = {}
                for blocks, outs in stages:
                    for t, h in blocks:
                        csl = pl.ds(h * hd + g * _G, _G)
                        xc = x2[pl.ds(r0[j][t], 16), csl].astype(_F32)
                        mb = st[j, t][0]
                        mb = jnp.concatenate([mb[:8] + dep, mb[8:]], axis=0)
                        xn[t, h] = (xc - mb) * st[j, t][1]
                        if full:
                            res[pl.ds(r0[j][t] // 2, 8), csl] = _pack((xc + xn[t, h]).astype(_BF16))
                    for b in outs:
                        dst.at[b][pl.ds(j * 8, 8), pl.ds(g * _G, _G)] = _pack(_SEVEN[b](xn).astype(_BF16))
                    dep = zero_of_bits(dst[0, pl.ds(zero8, 8), pl.ds(0, _G)])
        if full:
            best_v[...] = best
        return dep

    def seven_rows(load, dst, dst_row, n_units, dep, gs=range(hd // _G), tick=no_tick):
        for j in range(n_units):
            tk = tick(j)
            if tk is not None:
                dep = dep + zero_like(tk)
            for g in gs:
                w = {(a, b): load(a, b, j, g).astype(_F32) for a in range(2) for b in range(2)}
                for gate, outs in (((0, 0), (0, 1, 2, 4)), ((1, 0), (3, 5, 6))):
                    w[gate] = jnp.concatenate([w[gate][:8] + dep, w[gate][8:]], axis=0)
                    for b in outs:
                        dst.at[b][pl.ds(dst_row + j * 8, 8), pl.ds(g * _G, _G)] = _pack(_SEVEN[b](w).astype(_BF16))
                    dep = zero_of_bits(dst[0, pl.ds(dst_row + zero8, 8), pl.ds(gs[0] * _G, _G)])
        return dep

    qd = D // 4

    def level2_rows(blk, dst, dst_row, n_units, dep, first, groups=range(7), stages=2, tick=no_tick):
        n_out = 7 - first
        plan = (((0, 0), (0, 1, 2, 4)), ((1, 0), (3, 5, 6))) if stages == 2 else (((0, 0), range(7)),)
        for n, a in enumerate(groups):
            for j in range(n_units):
                tk = tick(n * n_units + j)
                if tk is not None:
                    dep = dep + zero_like(tk)
                for g in range(qd // _G):
                    w = blk(a, j, g)
                    for gate, outs in plan:
                        w[gate] = jnp.concatenate([w[gate][:8] + dep, w[gate][8:]], axis=0)
                        for b in outs:
                            if b >= first:
                                dst.at[a * n_out + b - first][pl.ds(dst_row + j * 8, 8), pl.ds(g * _G, _G)] = (
                                    _pack(_SEVEN[b](w).astype(_BF16)))
                        dep = zero_of_bits(dst[a * n_out, pl.ds(dst_row + zero8, 8), pl.ds(0, _G)])
        return dep

    def xn_level2(src, dst, dep, stages=2, tick=no_tick):
        blk = lambda a, j, g: {
            (a2, b2): _unpack(src[a, pl.ds(a2 * (hs // 2) + j * 8, 8), pl.ds(b2 * qd + g * _G, _G)]).astype(_F32)
            for a2 in range(2) for b2 in range(2)}
        return level2_rows(blk, dst, 0, _SUB // 32, dep, 2, stages=stages, tick=tick)

    g_home = {(0, 0): 6, (0, 1): 2, (1, 0): 1, (1, 1): 5}

    def staged(stage, part):
        return _unpack(stage[...] if part is None else stage[pl.ds(part * hs // 2, hs // 2), :])

    def k_job(stage, c, first=False, part=None, clk=None):
        p = _dot(staged(stage, part), wk_v[:, cols(c)])
        if clk is not None:
            clk.t += p.shape[0]
            clk.mark(2 * p.shape[0], p)
            clk.mark(p.shape[0], p[:, _G:])
        p = _phi(p)
        zs = jnp.sum(p.reshape(p.shape[0] // 8, 8, _CB), axis=0)
        if first:
            z_v[:, cols(c)] = zs
        else:
            z_v[:, cols(c)] += zs
        return p.astype(_BF16)

    def g_job(pk, stage, c, first=False, part=None, clk=None):
        upd = _dot_tn(pk, staged(stage, part))
        if clk is not None:
            for q in range(n_cb):
                clk.mark(pk.shape[0], upd[:, q * _CB:])
        a, j = divmod(c, n_sl)
        halves = [upd[:, :hd], upd[:, hd:]]
        if a == 1:
            assert first
            halves[1] = halves[1] + halves[0] - gm_v[g_home[0, 1], cols(j), :]
        for b in range(2):
            if first:
                gm_v[g_home[a, b], cols(j), :] = halves[b]
            else:
                gm_v[g_home[a, b], cols(j), :] += halves[b]

    def store_tr(blocks, j):
        n = blocks[0].shape[0]
        for b, v in enumerate(_seven(*blocks)):
            tr_v.at[b][:, pl.ds(j * _CB, n)] = _pack(v.astype(_BF16).T)
        return zero_of_bits(tr_v[0, pl.ds(zero8, 8), pl.ds(0, _G)])

    def kg_strassen(cur, pin, side, fresh=()):
        n = cur(0).shape[0]
        pins, clk = [], Clock()
        for j in range(n_sl):
            def prod(m):
                p = _dot(cur(_A_IDX[m]), _unpack(wks_v[_B_IDX[m], :, cols(j)]))
                clk.mark(n, p)
                clk.mark(n, p[:, _G:])
                if pin is not None and m == (1 if j == 0 else 1):
                    p = p + jnp.concatenate([pin[0:1, :]] * (_CB // _G), axis=1)
                return p

            p11, p12, p21, p22 = map(_phi, [_strassen, _strassen_even][0](prod))
            z_v[:, cols(j)] += jnp.sum((p11 + p21).reshape(n // 8, 8, _CB), axis=0)
            z_v[:, cols(n_sl + j)] += jnp.sum((p12 + p22).reshape(n // 8, 8, _CB), axis=0)
            pin = store_tr((p11, p21, p12, p22), j)
            pins.append(pin)
        for j in range(n_sl):
            for m in range(7):
                upd = _dot(_unpack(tr_v[_A_IDX[m], :, pl.ds(j * _CB, n)]), cur(_B_IDX[m]))
                clk.mark(n, upd)
                clk.mark(n, upd[:, hd - _G:])
                if m in fresh:
                    gm_v[m, cols(j), :] = upd
                else:
                    gm_v[m, cols(j), :] += upd
        side(pins, clk)

    def wk_load(j0):
        return lambda a, b, j, g: wk_v[pl.ds(a * hd + (j0 + j) * 16, 16), pl.ds(b * hd + g * _G, _G)]

    n_wu = hd // 16
    zero_v = jnp.zeros((8, _G), _F32)
    wait("x0a")
    ln_plain(0, _SUB // 2, sb_v, 16, False)
    wait("k0")
    p0a = k_job(sb_v, 0, True, part=0)
    wait("x0b")
    ln_plain(_SUB // 2, _SUB // 2, sb_v, 16, False)
    g_job(p0a, sb_v, 0, True, part=0)
    p0b = k_job(sb_v, 0, part=1)
    wait("k1")
    gps = _CB // _G
    clk = Clock()
    p2 = k_job(sb_v, 2, True, clk=clk)
    g_job(p0b, sb_v, 0, part=1, clk=clk)
    g_job(p2, sb_v, 2, True, clk=clk)
    seven_rows(wk_load(0), wks_v, 0, n_wu, zero_v, range(0, gps), tick=clk.every(0, 75))
    wait("k2x1")
    clk = Clock()
    p1 = k_job(sb_v, 1, True, clk=clk)
    p3 = k_job(sb_v, 3, True, clk=clk)
    g_job(p1, sb_v, 1, True, clk=clk)
    g_job(p3, sb_v, 3, True, clk=clk)
    ln_pair(1, xh_v, zero_v, half=_SUB // 2, full=False, tick=clk.every(0, 330))
    seven_rows(wk_load(0), wks_v, 0, n_wu, zero_v, range(gps, 2 * gps), tick=clk.every(1500, 78))
    wait("x23")
    kg_strassen(lambda b: _unpack(xh_v[b]), None,
                lambda pins, clk: ln_pair(1, xs_v.at[0], [zero_v, pins[0]][1], stages=[_STAGES, _STAGES3][1],
                                          tick=clk.every(0, 0)), fresh=(0, 3, 4))
    wait("x45q")

    def phase1(i, carry):
        @pl.when(i == 1)
        def _():
            wait("x67")

        win = xs_v.at[pl.ds(i, 2)]
        cur = lambda b: _unpack(win[0, b, :, hcols])

        sl = jnp.minimum(i, qd // _G - 1)
        for u in range(2):
            for b in range(2):
                f0 = pl.multiple_of(b * hd + u * qd + sl * _G, _G)
                for c in range(n_cb):
                    wqt_v[u, b, :, cols(c)] = _pack(wq_v[cols(c), pl.ds(f0, _G)].T)
        wq_pin = zero_of_bits(wqt_v[0, 0, pl.ds(zero8, 8), pl.ds(0, _G)])
        raw = lambda j, g: (lambda A, B, a2, b2: _unpack(
            wqt_v[b2, B, pl.ds(pl.multiple_of(j * 8 + zero8, 8), 8), pl.ds(A * hd + a2 * qd + g * _G, _G)]).astype(_F32))

        def side(pins, clk):
            xn_level2(win.at[0], x2_v.at[i], zero_v, stages=1, tick=clk.every(0, 0))
            level2_rows(lambda a, j, g: _seven2(raw(j, g), a), wq2_v, pl.multiple_of(sl * (_G // 2), _G // 2),
                        _G // 16, zero_v, 0, stages=2, tick=clk.every(1500, 0))
            ln_pair((i + 2) & (n_pair - 1), win.at[1], pins[-1], tick=clk.every(7680, 384))

        kg_strassen(cur, wq_pin, side)
        return carry

    jax.lax.fori_loop(0, n_pair - 1, phase1, 0)
    wait("vo")

    key = pltpu.bitcast(jnp.max(best_v[...], axis=0, keepdims=True), jnp.int32)
    rmax = pltpu.bitcast(key & jnp.int32(-65536), _F32)
    idx = (S - 1) - jnp.max(key & (S - 1))
    idx_pair = idx // (2 * _SUB)
    gate_r = jax.nn.sigmoid(rmax)

    xs = x_v[pl.ds(pl.multiple_of((idx >> 4) * 16, 16), 16), :].astype(_F32)
    m, rstd = ln_stats(xs, None, False)[:2]
    xs = ((xs - m) * rstd).astype(_BF16).astype(_F32)
    sel = jax.lax.broadcasted_iota(jnp.int32, (16, D), 0) == (idx & 15)
    xs = jnp.sum(jnp.where(sel, xs, 0.0), axis=0, keepdims=True)
    for g in range(n_groups):
        xcol_v[pl.ds(g * _G, _G), :] = _col_bcast(xs[:, gsl(g)])
    res_row = pl.ds(pl.multiple_of((idx >> 4) * 8, 8), 8)
    for g in range(n_groups):
        z = jnp.sum(z_v[:, pl.ds(g * _G, _G)], axis=0, keepdims=True)
        zcol_v[pl.ds(g * _G, _G), :] = _col_bcast(z)

    rr = jax.lax.broadcasted_iota(jnp.int32, (_G, _G), 0) // dh
    cc = jax.lax.broadcasted_iota(jnp.int32, (_G, _G), 1) // dh
    same_head = rr == cc
    n_hg = hd // _G
    kvb = {}
    col_pins = {2: zero_like(zcol_v[pl.ds(zero8, 1), :]), 3: zero_like(xcol_v[pl.ds(zero8, 1), :])}

    def kv_job(g):
        gm = lambda m: gm_v[m, pl.ds((g % n_hg) * _G, _G), :]
        if g < n_hg:
            row = [gm(0) + gm(3) - gm(4) + gm(6), gm(2) + gm(4)]
        else:
            row = [gm(1) + gm(3), gm(0) - gm(1) + gm(2) + gm(5)]
        kv = _dot(jnp.concatenate(row, axis=1).astype(_BF16), wv_v[:, pl.ds(g * _G, _G)])
        clk.t += _G
        clk.mark(_G, kv)
        if g in col_pins:
            kv = kv + col_pins[g]
        kvb[g] = jnp.where(same_head, kv, 0.0).astype(_BF16)

    def m_job(g):
        top, bot = [_dot(kvb.pop(q), wo_v[pl.ds(q * _G, _G), dcols]) for q in (g, g + n_hg)]
        clk.mark(2 * _G, top)
        clk.mark(2 * _G, bot)
        for b, v in enumerate(_seven(top[:, :hd], top[:, hd:], bot[:, :hd], bot[:, hd:])):
            ms_v.at[b][pl.ds(g * _G // 2, _G // 2), :] = _pack(v.astype(_BF16))

    clk = Clock()
    for g in range(n_hg):
        kv_job(g)
        kv_job(g + n_hg)
        if g > 0:
            m_job(g - 1)
    m_job(n_hg - 1)
    xn_level2(xs_v.at[n_pair - 1], x2_v.at[n_pair - 1], zero_v, stages=2, tick=clk.every(0, 0))
    wait("f0")

    def chain_matvec(w_ref, lead, cb, col_ref, acc0):
        n = col_ref.shape[0] // 8
        acc = [acc0[:, :_G], acc0[:, _G:]]
        link = None
        for k0 in range(0, n, _BLK):
            rows = pl.ds(k0 * 8, _BLK * 8)
            w = w_ref[lead, rows, cols(cb)].astype(_F32)
            colv = col_ref[rows, :]
            for h in range(2):
                prod = (w[:, h * _G:(h + 1) * _G] * colv).reshape(_BLK, 8, _G)
                first = acc[h] if link is None else acc[h] + link
                acc[h] = jnp.sum(jnp.concatenate([first[None], prod], axis=0), axis=0)
                link = zero_like(acc[h])
        return jnp.concatenate(acc, axis=1)

    def phase2(i, carry):
        @pl.when(i == 1)
        def _():
            wait("f1")

        slot = (idx_pair + i) & (n_pair - 1)
        pair = (slot + 1) & (n_pair - 1)
        prows = pl.ds(pl.multiple_of(pair * (2 * _SUB), 2 * _SUB), 2 * _SUB)
        out_w, hbm_w = out_v.at[prows], out_hbm.at[prows]
        res_w = res_v.at[pl.ds(pl.multiple_of(pair * _SUB, _SUB), _SUB)]
        win = xs_v.at[slot]
        cur = lambda b: _unpack(win[b, :, hcols])

        ys, accs, pins, ticks = [], [], {}, []
        n_gu = 2 * fc // _CB
        d0, ds, nq, g0 = 3, 6, 0, 2
        plan = [d0 + ds * n for n in range(n_cb + nq)] + [49 + g0 + (n * 9) // 8 for n in range(n_gu - nq)]

        def ffn_part(first, last, dep):
            for n in range(first, last):
                if plan[n] >= 0:
                    dep = dep + wide(zero_like(ticks[plan[n]]))
                if n < n_cb:
                    ys.append(chain_matvec(wd_v, jnp.maximum(i - 1, 0), n, hcol_v, y_v[:, cols(n)] + dep))
                    dep = zero_link(ys[-1])
                else:
                    accs.append(chain_matvec(gu_v, jnp.minimum(i, n_fc - 1), n - n_cb, xcol_v, dep))
                    dep = zero_link(accs[-1])
            return dep

        x2w = x2_v.at[slot]

        def xop(a, b):
            if b < 2:
                return _unpack(win[a, pl.ds(b * (hs // 2), hs // 2), pl.ds(b * qd, qd)])
            return _unpack(x2w[a * 5 + b - 2])

        def normalise(p, fq):
            p3 = _phi(p).reshape(qd // dh, dh, _G)
            zc = zcol_v[pl.ds(fq * qd, qd), :].reshape(qd // dh, dh, _G)
            den = jnp.sum(p3 * zc, axis=1, keepdims=True) + _DEN_EPS
            return (p3 * pl.reciprocal(den, approx=True)).reshape(qd, _G)

        def q_phase():
            def prod(m1, m2):
                if (m1, m2) in hooks:
                    hooks[m1, m2]()
                w, x = _unpack(wq2_v[_B_IDX[m1] * 7 + _B_IDX[m2]]), xop(_A_IDX[m1], _A_IDX[m2])
                if (m1, m2) == at(48):
                    p = jnp.concatenate([_dot_nt(w[:qd // 2], x), _dot_nt(w[qd // 2:], x)], axis=0)
                else:
                    p = _dot_nt(w, x)
                ticks.append(p[:8, :_G])
                return p + pins[m1, m2][:, :_G] if (m1, m2) in pins else p

            inner = lambda m1: _strassen_even(lambda m2: prod(m1, m2))

            def early(k, c, at_prod):
                for n in (2, 1, 0, 3):
                    of_v[4 * k + n] = normalise(c[n], 2 * (k % 2) + n % 2)
                if at_prod < 49:
                    pins[at(at_prod)] = zero_like(of_v[4 * k + 2, pl.ds(zero8, 1), :])

            m2 = inner(1)
            m4 = inner(3)
            early(2, _add(m2, m4), 19)
            m3 = inner(2)
            m5 = inner(4)
            early(1, _add(m3, m5), 33)
            m1 = inner(0)
            early(0, _add(_add(_sub(m4, m5), m1), inner(6)), 99)
            c22 = _add(_add(_sub(m3, m2), m1), inner(5))
            for n in (2, 1, 0, 3):
                a2, b2 = divmod(n, 2)
                o = [of_v[4 * k + n] for k in range(3)] + [normalise(c22[n], 2 + b2)]
                for b, v in enumerate(_seven(*o)):
                    tr_v.at[b][pl.ds(a2 * (hs // 2), hs // 2), pl.ds(b2 * qd, qd)] = _pack(v.astype(_BF16).T)

        def finish(cs, j):
            order = (1, 3, 2, 0)
            for q in order:
                t, b = divmod(q, 2)
                c = b * n_sl + j
                rows = pl.ds(t * _SUB, _SUB)
                res = cs[q] + _unpack(res_w[pl.ds(t * hs, hs), cols(c)]).astype(_F32)
                out_w[rows, cols(c)] = res.astype(_BF16)
                pltpu.make_async_copy(out_w.at[rows, cols(c)], hbm_w.at[rows, cols(c)], sem_o).start()

        wide = lambda d: jnp.concatenate([d] * (_CB // _G), axis=1)
        h = h_v[...].astype(_BF16).astype(_F32)
        for f in range(fc // _G):
            hcol_v[pl.ds(f * _G, _G), :] = _col_bcast(h[:, gsl(f)])
        order = (0, 3, 1, 4, 6, 2, 5)
        at = lambda n: (_ORD[1][n // 7], _ORD[1][n % 7])
        hooks, last, st = {}, {}, {}
        hrel = wide(zero_like(hcol_v[pl.ds(zero8, 8), :]))
        q_phase()

        st['dep'] = ffn_part(0, n_cb + nq, hrel)
        yacc = jnp.concatenate(ys, axis=1)
        y_v[...] = yacc
        yrow = jnp.sum(yacc, axis=0, keepdims=True) * gate_r
        hit = jax.lax.broadcasted_iota(jnp.int32, (16, D), 0) == jnp.where(i == n_pair - 1, idx & 15, -1)
        upd = _unpack(res_v[res_row, :]).astype(_F32) + jnp.where(hit, yrow, 0.0)
        res_v[res_row, :] = _pack(upd.astype(_BF16))
        cnt = [0]

        def oprod(m, j):
            p = _dot(_unpack(tr_v[_A_IDX[m]]), _unpack(ms_v[_B_IDX[m], :, cols(j)]))
            ticks.append(p[:8, :_G])
            cnt[0] += 1
            return p

        for j in range(n_sl):
            finish(_strassen_late22(lambda m: oprod(m, j)), j)
        ffn_part(n_cb + nq, n_cb + n_gu, st["dep"])
        gu = jnp.sum(jnp.concatenate(accs, axis=1), axis=0, keepdims=True)
        g, u = gu[:, :fc], gu[:, fc:]
        hnext = (g * jax.nn.sigmoid(g) * u).astype(_BF16).astype(_F32)
        lane = jax.lax.broadcasted_iota(jnp.int32, (1, fc), 1)
        h_v[...] = jnp.where(lane < jnp.where(i > 0, f_dup, 0), 0.0, hnext)
        return carry

    jax.lax.fori_loop(0, n_pair, phase2, 0)
    pltpu.make_async_copy(out_v, out_hbm, sem_o).wait()


@jax.jit
def pallas_parallel_sum__linear_attn_block__moe_arch_mod__prompt_kernel(
    A_x: jax.Array,
    A_wqkv: jax.Array,
    A_wo: jax.Array,
    B_x: jax.Array,
    B_w_r: jax.Array,
    B_w_gate: jax.Array,
    B_w_up: jax.Array,
    B_w_down: jax.Array,
):
    del B_x
    B, S, D = A_x.shape
    assert B == 1
    F = B_w_gate.shape[1]
    n_pair = S // _SUB // 2
    n_fc = n_pair - 1
    fc = _ffn_chunks(F, n_fc)[0]
    hd = D // 2
    qd = D // 4
    any_spec = pl.BlockSpec(memory_space=pl.ANY)
    out = pl.pallas_call(
        functools.partial(_kernel, S=S, D=D, F=F),
        out_shape=jax.ShapeDtypeStruct((S, D), A_x.dtype),
        in_specs=[any_spec] * 7,
        out_specs=any_spec,
        scratch_shapes=[
            pltpu.VMEM((S, D), _BF16),
            pltpu.VMEM((D, D + _PAD), _BF16),
            pltpu.VMEM((D, D + _PAD), _BF16),
            pltpu.VMEM((D, D + _PAD), _BF16),
            pltpu.VMEM((D, D + _PAD), _BF16),
            pltpu.VMEM((D // _G, _G), _BF16),
            pltpu.VMEM((n_fc, D, 2 * fc), _BF16),
            pltpu.VMEM((n_fc, fc, D + _PAD), _BF16),
            pltpu.VMEM((7, _SUB // 4, hd), _U32),
            pltpu.VMEM((_SUB // 2, D), _U32),
            pltpu.VMEM((n_pair, 7, _SUB // 2, hd + _PAD), _U32),
            pltpu.VMEM((n_pair, 35, _SUB // 4, qd), _U32),
            pltpu.VMEM((S // 2, D), _U32),
            pltpu.VMEM((7, hd // 2, hd), _U32),
            pltpu.VMEM((2, 2, _G // 2, D), _U32),
            pltpu.VMEM((49, qd // 2, qd), _U32),
            pltpu.VMEM((7, hd, hd), _F32),
            pltpu.VMEM((8, D), _F32),
            pltpu.VMEM((8, 1), _F32),
            pltpu.VMEM((D, _G), _F32),
            pltpu.VMEM((D, _G), _F32),
            pltpu.VMEM((1, fc), _F32),
            pltpu.VMEM((fc, _G), _F32),
            pltpu.VMEM((8, D), _F32),
            pltpu.VMEM((7, _SUB // 2, hd), _U32),
            pltpu.VMEM((12, qd, _G), _F32),
            pltpu.VMEM((7, hd // 2, hd), _U32),
            pltpu.VMEM((S, D), _BF16),
            pltpu.SemaphoreType.DMA((11,)),
            pltpu.SemaphoreType.DMA,
            pltpu.SemaphoreType.REGULAR,
        ],
        compiler_params=pltpu.CompilerParams(
            vmem_limit_bytes=120 * 1024 * 1024,
            disable_bounds_checks=not _RUNTIME_CHECKS,
            disable_semaphore_checks=not _RUNTIME_CHECKS,
        ),
    )(A_x.reshape(S, D), A_wqkv, A_wo, B_w_r.reshape(D // _G, _G), B_w_gate, B_w_up, B_w_down)
    return out.reshape(B, S, D)
```
